```python
import jax
import jax.numpy as jnp

def _softmax(x, axis=-1):
    return jax.nn.softmax(x, axis=axis)

def _gelu(x):
    return jax.nn.gelu(x, approximate=True)

def _silu(x):
    return jax.nn.silu(x)

def _sigmoid(x):
    return jax.nn.sigmoid(x)

def _layernorm(x, axis=-1, eps=1e-05):
    m = jnp.mean(x, axis=axis, keepdims=True)
    v = jnp.var(x, axis=axis, keepdims=True)
    return (x - m) / jnp.sqrt(v + eps)

def _scatter_add(tgt, idx, src, axis=0):
    return tgt.at[idx].add(src)

def _segment_sum(src, seg, n):
    return jax.ops.segment_sum(src, seg, n)

class _Rng:

    def __init__(self, key):
        self._k = key

    def _next(self):
        self._k, sub = jax.random.split(self._k)
        return sub

    def normal(self, shape):
        return jax.random.normal(self._next(), shape, dtype=jnp.bfloat16)

    def randint(self, lo, hi, shape):
        return jax.random.randint(self._next(), shape, lo, hi, dtype=jnp.int32)

    def uniform(self, shape, lo=0.0, hi=1.0):
        return jax.random.uniform(self._next(), shape, jnp.bfloat16, lo, hi)

    def permutation(self, n):
        return jax.random.permutation(self._next(), n)
kernel_name = 'sequential_preLN__memory_aug_recurrent_mem_tr__mixer_s_mlp__prompt'

def setup_inputs():
    _rng = _Rng(jax.random.key(int.from_bytes(__import__("os").urandom(4), "little")))
    _w = lambda a: (lambda t: t.astype(jnp.bfloat16) if jnp.issubdtype(t.dtype, jnp.floating) else t)(jnp.asarray(a))

    def _A_setup():
        B, S, Dm = (1, 2048, 1024)
        H, Dh = (32, 128)
        M, seg = (8, 32)
        seg = min(seg, S)
        S = S // seg * seg
        return {'x': _w((lambda *s: _rng.normal(s) * 0.05)(B, S, Dm)), 'mem0': _w((lambda *s: _rng.normal(s) * 0.05)(B, M, Dm)), 'Wq': _w((lambda *s: _rng.normal(s) * 0.05)(Dm, H, Dh) * Dm ** (-0.5)), 'Wk': _w((lambda *s: _rng.normal(s) * 0.05)(Dm, H, Dh) * Dm ** (-0.5)), 'Wv': _w((lambda *s: _rng.normal(s) * 0.05)(Dm, H, Dh) * Dm ** (-0.5)), 'Wo': _w((lambda *s: _rng.normal(s) * 0.05)(H, Dh, Dm) * (H * Dh) ** (-0.5)), 'seg_len': seg}
    _A_in = _A_setup()

    def _B_setup():
        B, S, D, F = (1, 2048, 1024, 3584)
        return {'x': _w((lambda *s: _rng.normal(s) * 0.05)(B, S, D)), 'w1': _w((lambda *s: _rng.normal(s) * 0.05)(D, D) * D ** (-0.5)), 'w2': _w((lambda *s: _rng.normal(s) * 0.05)(D, D) * D ** (-0.5)), 'w3': _w((lambda *s: _rng.normal(s) * 0.05)(D, F) * D ** (-0.5)), 'w4': _w((lambda *s: _rng.normal(s) * 0.05)(F, D) * F ** (-0.5))}
    _B_in = _B_setup()
    return {'A_x': _A_in['x'], 'A_mem0': _A_in['mem0'], 'A_Wq': _A_in['Wq'], 'A_Wk': _A_in['Wk'], 'A_Wv': _A_in['Wv'], 'A_Wo': _A_in['Wo'], 'A_seg_len': _A_in['seg_len'], 'B_x': _B_in['x'], 'B_w1': _B_in['w1'], 'B_w2': _B_in['w2'], 'B_w3': _B_in['w3'], 'B_w4': _B_in['w4']}

def reference(A_x, A_mem0, A_Wq, A_Wk, A_Wv, A_Wo, A_seg_len, B_x, B_w1, B_w2, B_w3, B_w4):

    def _A_ref(x, mem0, Wq, Wk, Wv, Wo, seg_len):
        B, S, Dm = x.shape
        H, Dh = (Wq.shape[1], Wq.shape[2])
        M = mem0.shape[1]
        scale = Dh ** (-0.5)
        n_seg = S // seg_len
        L = M + seg_len
        idx = jnp.arange(L)
        mask = (idx[:, None] < M) | (idx[:, None] >= idx[None, :])
        mem = mem0
        outs = []
        for s in range(n_seg):
            xs = x[:, s * seg_len:(s + 1) * seg_len, :].copy()
            h = jnp.concatenate([mem, xs], axis=1)
            q = jnp.einsum('btd,dhe->bhte', h, Wq)
            k = jnp.einsum('btd,dhe->bhte', h, Wk)
            v = jnp.einsum('btd,dhe->bhte', h, Wv)
            scores = jnp.einsum('bhqe,bhke->bhqk', q, k) * scale
            scores = jnp.where(mask[None, None], scores, -1000000000.0)
            p = _softmax(scores, axis=-1)
            o = jnp.einsum('bhqk,bhke->bhqe', p, v)
            o = jnp.einsum('bhte,hed->btd', o, Wo)
            mem = o[:, :M, :].copy()
            outs.append(o[:, M:, :])
        return jnp.concatenate(outs, axis=1)

    def _B_ref(x, w1, w2, w3, w4):
        B, S, D = x.shape
        h = _gelu(_layernorm(x, axis=-1) @ w1)
        c = D // 4
        g0 = jnp.pad(h[:, :, 0 * c:1 * c], ((0, 0), (1, 0), (0, 0)))[:, :S, :]
        g1 = jnp.pad(h[:, :, 1 * c:2 * c], ((0, 0), (0, 1), (0, 0)))[:, 1:, :]
        g2 = jnp.pad(h[:, :, 2 * c:3 * c], ((0, 0), (2, 0), (0, 0)))[:, :S, :]
        g3 = jnp.pad(h[:, :, 3 * c:], ((0, 0), (0, 2), (0, 0)))[:, 2:, :]
        hs = jnp.concatenate([g0, g1, g2, g3], axis=-1) @ w2
        x1 = x + hs
        h2 = _gelu(_layernorm(x1, axis=-1) @ w3) @ w4
        return x1 + h2
    x = A_x
    h = x + _A_ref(_layernorm(x, axis=-1), A_mem0, A_Wq, A_Wk, A_Wv, A_Wo, A_seg_len)
    h2 = h + _B_ref(_layernorm(h, axis=-1), B_w1, B_w2, B_w3, B_w4)
    return h2
```

```python
import functools

import numpy as np
import jax
import jax.numpy as jnp
from jax import lax
import jax.experimental.pallas as pl
import jax.experimental.pallas.tpu as pltpu

F32 = jnp.float32
BF16 = jnp.bfloat16
U32 = jnp.uint32
LANE = 128
EPS = 1e-5


def _bf(w_u32):
    return pltpu.bitcast(w_u32, BF16)


def _ln(x):
    m = jnp.mean(x, axis=-1, keepdims=True)
    d = x - m
    v = jnp.mean(d * d, axis=-1, keepdims=True)
    return d * lax.rsqrt(v + EPS)


def _gelu(x):
    c0 = np.float32(np.sqrt(2.0 / np.pi))
    c1 = np.float32(np.sqrt(2.0 / np.pi) * 0.044715)
    t = jnp.tanh(x * (c0 + c1 * (x * x)))
    hx = 0.5 * x
    return hx + hx * t


def _cat(xs, axis):
    return xs[0] if len(xs) == 1 else jnp.concatenate(xs, axis=axis)


def _make_kernel(S, D, H, DH, M, SEG, F, TB):
    NSEG = S // SEG
    TOK = SEG - M
    P = S - NSEG * TOK
    R = SEG * TOK * -(-(P + SEG) // (SEG * TOK))
    KD = D // LANE
    KF = F // LANE
    NPAIR = H // 2
    NB = S // TB
    HALO = 16
    scale = np.float32(DH ** (-0.5))
    PT = P // SEG
    LNS = NSEG // NPAIR

    def kernel(x_hbm, mem0_ref, wq_hbm, wk_hbm, wv_hbm, wo_hbm, w1_hbm, w2_hbm, w3_hbm, w4_hbm,
               out_hbm,
               wq_s, wk_s, wv_s, wo_s, w1_s, w2_s, w3_s, w4_s,
               xs, xl, rq, rk, rv, o2, hs, h1s, ostage,
               sem_x, sem_w, sem_wo, sem_b, sem_o):
        def x_copy(j):
            return pltpu.make_async_copy(x_hbm.at[:, j * LANE:(j + 1) * LANE], xs.at[j], sem_x.at[j])

        def pair_copies(j):
            cps = []
            for w_hbm, w_s in ((wq_hbm, wq_s), (wk_hbm, wk_s), (wv_hbm, wv_s)):
                wb = w_hbm.bitcast(U32)
                for p in range(2):
                    cps.append(pltpu.make_async_copy(wb.at[:, p, j, :], w_s.at[2 * j + p], sem_w.at[j]))
            return cps

        def col_copy(w_hbm, w_s, j, sem):
            return pltpu.make_async_copy(w_hbm.bitcast(U32).at[:, pl.ds(j * LANE, LANE)], w_s.at[j], sem)

        def b_copies():
            cps = []
            for i, (w_hbm, w_s) in enumerate(((w1_hbm, w1_s), (w2_hbm, w2_s), (w3_hbm, w3_s), (w4_hbm, w4_s))):
                for j in range(w_s.shape[0]):
                    cps.append(col_copy(w_hbm, w_s, j, sem_b.at[i]))
            return cps

        for j in range(KD):
            x_copy(j).start()
        for j in range(2):
            for c in pair_copies(j):
                c.start()

        for k in range(KD):
            xl[k, P:P + M, :] = mem0_ref[:, k * LANE:(k + 1) * LANE]
        for j in range(KD):
            x_copy(j).wait()

        def ln_rows(src_row, dst_row, n):
            xf = _cat([xs[k, pl.ds(src_row, n), :] for k in range(KD)], 1).astype(F32)
            xn = _ln(xf).astype(BF16)
            for k in range(KD):
                xl[k, pl.ds(dst_row, n), :] = xn[:, k * LANE:(k + 1) * LANE]

        def ln0_body(i, c):
            r = pl.multiple_of(i * 64, 64)
            ln_rows(r, r, 64)
            return c
        lax.fori_loop(0, P // 64, ln0_body, 0)

        def pro_body(j, c):
            @pl.when(j + 2 < NPAIR)
            def _():
                for cp in pair_copies(j + 2):
                    cp.start()

            @pl.when(j < KD)
            def _():
                col_copy(wo_hbm, wo_s, j, sem_wo.at[j]).start()

            for cp in pair_copies(j):
                cp.wait()
            lhs = _cat([xl[k, 0:P, :] for k in range(KD)], 1)
            for w_s, r_s in ((wq_s, rq), (wk_s, rk), (wv_s, rv)):
                a = w_s[2 * j]
                b = w_s[2 * j + 1]
                lo = (a & np.uint32(0xFFFF)) | (b << 16)
                hi = (a >> 16) | (b & np.uint32(0xFFFF0000))
                w_s[2 * j] = lo
                w_s[2 * j + 1] = hi
                r_s[2 * j, 0:P, :] = jnp.dot(lhs, _bf(lo), preferred_element_type=F32).astype(BF16)
                r_s[2 * j + 1, 0:P, :] = jnp.dot(lhs, _bf(hi), preferred_element_type=F32).astype(BF16)
            for i in range(LNS):
                s = j * LNS + i
                ln_rows(pl.multiple_of(P + s * TOK, 8), pl.multiple_of(P + s * SEG + M, 8), TOK)
            return c
        lax.fori_loop(0, NPAIR, pro_body, 0)

        for cp in b_copies():
            cp.start()
        for j in range(KD):
            col_copy(wo_hbm, wo_s, j, sem_wo.at[j]).wait()

        def step(s, c):
            srow = pl.multiple_of(s * SEG, SEG)
            lhs = _cat([xl[k, pl.ds(P + srow, SEG), :] for k in range(KD)], 1)
            wr = [pl.multiple_of(lax.rem(P + s * TOK + 8 * i, R), 8) for i in range(TOK // 8)]
            rr = pl.multiple_of(lax.rem(srow, R), SEG)
            orow = []
            for i in range(SEG // 8):
                p = s * (SEG // 8) + i
                a = (p // (TOK // 8)) * SEG + M + (p % (TOK // 8)) * 8
                b = (s + PT) * SEG + 8 * i
                orow.append(pl.multiple_of(jnp.where(s < NSEG - PT, a, b), 8))
            L = SEG + M
            qi = lax.broadcasted_iota(jnp.int32, (L, L), 0)
            kj = lax.broadcasted_iota(jnp.int32, (L, L), 1)
            mask = (qi >= SEG) | (kj >= SEG) | (kj <= qi)

            mems = {}

            def proj(h):
                vals = []
                for w_s, r_s in ((wq_s, rq), (wk_s, rk), (wv_s, rv)):
                    y = jnp.dot(lhs, _bf(w_s[h]), preferred_element_type=F32)
                    for i in range(TOK // 8):
                        r_s[h, pl.ds(wr[i], 8), :] = y[M + 8 * i:M + 8 * i + 8, :].astype(BF16)
                    vals.append(y[0:M, :].astype(BF16))
                mems[h] = vals

            def attend(h):
                qm, km, vm = mems.pop(h)
                q = _cat([rq[h, pl.ds(rr, SEG), :], qm], 0)
                k = _cat([rk[h, pl.ds(rr, SEG), :], km], 0)
                v = _cat([rv[h, pl.ds(rr, SEG), :], vm], 0)
                sc = lax.dot_general(q, k, (((1,), (1,)), ((), ())), preferred_element_type=F32)
                sc = jnp.where(mask, sc * scale, np.float32(-1e9))
                mx = jnp.max(sc, axis=-1, keepdims=True)
                e = jnp.exp(sc - mx)
                l = jnp.sum(e, axis=-1, keepdims=True)
                p = (e / l).astype(BF16)
                o = jnp.dot(p, v, preferred_element_type=F32)
                for i in range(SEG // 8):
                    o2[h, pl.ds(orow[i], 8), :] = o[8 * i:8 * i + 8, :].astype(BF16)
                o2[h, pl.ds(srow, M), :] = o[SEG:SEG + M, :].astype(BF16)

            G = 8
            NG = H // G
            for h in range(G):
                proj(h)
            for g in range(1, NG):
                for i in range(G):
                    proj(g * G + i)
                    attend((g - 1) * G + i)

            def wo_part(hs_):
                lo_ = _cat([o2[h, pl.ds(srow, SEG), :] for h in hs_], 1)
                outs = []
                for j in range(KD):
                    w = wo_s[j, hs_[0] * (DH // 2):(hs_[-1] + 1) * (DH // 2), :]
                    outs.append(jnp.dot(lo_, _bf(w), preferred_element_type=F32))
                return outs

            for i in range(G):
                attend((NG - 1) * G + i)
            accs = wo_part(list(range(H)))
            hrow = pl.multiple_of(s * TOK, 8)
            for j in range(KD):
                acc = accs[j]
                xl[j, pl.ds(P + srow + SEG, M), :] = acc[0:M, :].astype(BF16)
                hs[j, pl.ds(hrow, TOK), :] = (xs[j, pl.ds(hrow, TOK), :].astype(F32) + acc[M:SEG, :]).astype(BF16)
            return c
        lax.fori_loop(0, NSEG, step, 0)

        TE = 128

        def epi_body(i, c):
            r = pl.multiple_of(NSEG * SEG + i * TE, TE)
            t = pl.multiple_of(NSEG * TOK + i * TE, TE)
            lo_ = _cat([o2[h, pl.ds(r, TE), :] for h in range(H)], 1)
            for j in range(KD):
                acc = jnp.dot(lo_, _bf(wo_s[j]), preferred_element_type=F32)
                hs[j, pl.ds(t, TE), :] = (xs[j, pl.ds(t, TE), :].astype(F32) + acc).astype(BF16)
            return c
        lax.fori_loop(0, P // TE, epi_body, 0)

        for cp in b_copies():
            cp.wait()
        zero_halo = jnp.zeros((HALO, LANE), BF16)
        for j in range(KD):
            h1s[j, 0:HALO, :] = zero_halo
            h1s[j, HALO + S:HALO + S + HALO, :] = zero_halo

        def load_h(r):
            return _cat([hs[k, pl.ds(r, TB), :] for k in range(KD)], 1).astype(F32)

        def b1_body(i, c):
            r = pl.multiple_of(i * TB, TB)
            a = _ln(_ln(load_h(r))).astype(BF16)
            for j in range(KD):
                z = jnp.dot(a, _bf(w1_s[j]), preferred_element_type=F32)
                h1s[j, pl.ds(HALO + r, TB), :] = _gelu(z).astype(BF16)
            return c
        lax.fori_loop(0, NB, b1_body, 0)

        shifts = (-1, 1, -2, 2)

        def out_copy(i, slot):
            return pltpu.make_async_copy(ostage.at[slot], out_hbm.at[pl.ds(i * TB, TB), :], sem_o.at[slot])

        def b2_body(i, c):
            r = pl.multiple_of(i * TB, TB)
            slot = lax.rem(i, 2)
            cols = []
            for j in range(KD):
                d = shifts[j // (KD // 4)]
                win = h1s[j, pl.ds(r, TB + 2 * HALO), :].astype(F32)
                cols.append(win[HALO + d:HALO + d + TB, :].astype(BF16))
            g = _cat(cols, 1)
            hf = load_h(r)
            xb = _ln(hf)
            x1 = _cat([jnp.dot(g, _bf(w2_s[j]), preferred_element_type=F32) for j in range(KD)], 1) + xb
            a = _ln(x1).astype(BF16)
            u = _cat([_gelu(jnp.dot(a, _bf(w3_s[f]), preferred_element_type=F32)).astype(BF16)
                      for f in range(KF)], 1)
            res = hf + x1

            @pl.when(i >= 2)
            def _():
                out_copy(i - 2, slot).wait()
            for j in range(KD):
                y = jnp.dot(u, _bf(w4_s[j]), preferred_element_type=F32)
                ostage[slot, :, j * LANE:(j + 1) * LANE] = (res[:, j * LANE:(j + 1) * LANE] + y).astype(BF16)
            out_copy(i, slot).start()
            return c
        lax.fori_loop(0, NB, b2_body, 0)
        for i in range(NB - 2, NB):
            out_copy(i, i % 2).wait()

    scratch = [
        pltpu.VMEM((H, D // 2, LANE), U32),
        pltpu.VMEM((H, D // 2, LANE), U32),
        pltpu.VMEM((H, D // 2, LANE), U32),
        pltpu.VMEM((KD, H * DH // 2, LANE), U32),
        pltpu.VMEM((KD, D // 2, LANE), U32),
        pltpu.VMEM((KD, D // 2, LANE), U32),
        pltpu.VMEM((KF, D // 2, LANE), U32),
        pltpu.VMEM((KD, F // 2, LANE), U32),
        pltpu.VMEM((KD, S, LANE), BF16),
        pltpu.VMEM((KD, P + (NSEG + 1) * SEG, LANE), BF16),
        pltpu.VMEM((H, R, LANE), BF16),
        pltpu.VMEM((H, R, LANE), BF16),
        pltpu.VMEM((H, R, LANE), BF16),
        pltpu.VMEM((H, NSEG * SEG + P, LANE), BF16),
        pltpu.VMEM((KD, S, LANE), BF16),
        pltpu.VMEM((KD, S + 2 * HALO, LANE), BF16),
        pltpu.VMEM((2, TB, D), BF16),
        pltpu.SemaphoreType.DMA((KD,)),
        pltpu.SemaphoreType.DMA((NPAIR,)),
        pltpu.SemaphoreType.DMA((KD,)),
        pltpu.SemaphoreType.DMA((4,)),
        pltpu.SemaphoreType.DMA((2,)),
    ]
    return kernel, scratch


@functools.partial(jax.jit, static_argnames=("A_seg_len",))
def pallas_sequential_preLN__memory_aug_recurrent_mem_tr__mixer_s_mlp__prompt_kernel(
    A_x, A_mem0, A_Wq, A_Wk, A_Wv, A_Wo, A_seg_len, B_x, B_w1, B_w2, B_w3, B_w4,
):
    del B_x
    B, S, D = A_x.shape
    M = A_mem0.shape[1]
    H, DH = A_Wq.shape[1], A_Wq.shape[2]
    F = B_w3.shape[1]
    SEG = int(A_seg_len)
    assert B == 1 and DH == LANE and M == 8 and SEG == 32 and H % 8 == 0 and D == 4 * 2 * LANE
    kernel, scratch = _make_kernel(S, D, H, DH, M, SEG, F, TB=256)
    any_spec = pl.BlockSpec(memory_space=pl.ANY)
    out = pl.pallas_call(
        kernel,
        out_shape=jax.ShapeDtypeStruct((S, D), A_x.dtype),
        in_specs=[any_spec, pl.BlockSpec()] + [any_spec] * 8,
        out_specs=any_spec,
        scratch_shapes=scratch,
        compiler_params=pltpu.CompilerParams(vmem_limit_bytes=120 * 1024 * 1024),
    )(
        A_x.reshape(S, D),
        A_mem0.reshape(M, D),
        A_Wq.reshape(D // 2, 2, H, DH),
        A_Wk.reshape(D // 2, 2, H, DH),
        A_Wv.reshape(D // 2, 2, H, DH),
        A_Wo.reshape(H * DH, D),
        B_w1, B_w2, B_w3, B_w4,
    )
    return out.reshape(B, S, D)
```

```python
import functools

import numpy as np
import jax
import jax.numpy as jnp
from jax import lax
import jax.experimental.pallas as pl
import jax.experimental.pallas.tpu as pltpu

F32 = jnp.float32
BF16 = jnp.bfloat16
U32 = jnp.uint32
LANE = 128
EPS = 1e-5
CFG = dict(L1=1, L2=5, HS=24)


def _bf(w_u32):
    return pltpu.bitcast(w_u32, BF16)


def _ln(x):
    m = jnp.mean(x, axis=-1, keepdims=True)
    d = x - m
    v = jnp.mean(d * d, axis=-1, keepdims=True)
    return d * lax.rsqrt(v + EPS)


def _gelu(x):
    c0 = np.float32(np.sqrt(2.0 / np.pi))
    c1 = np.float32(np.sqrt(2.0 / np.pi) * 0.044715)
    t = jnp.tanh(x * (c0 + c1 * (x * x)))
    hx = 0.5 * x
    return hx + hx * t


def _cat(xs, axis):
    return xs[0] if len(xs) == 1 else jnp.concatenate(xs, axis=axis)


def _make_kernel(S, D, H, DH, M, SEG, F, TB):
    NSEG = S // SEG
    TOK = SEG - M
    P = S - NSEG * TOK
    R = SEG * TOK * -(-(P + SEG) // (SEG * TOK))
    KD = D // LANE
    KF = F // LANE
    NPAIR = H // 2
    NB = S // TB
    HALO = 16
    scale = np.float32(DH ** (-0.5))
    PT = P // SEG
    LNS = NSEG // NPAIR

    def kernel(x_hbm, mem0_ref, wq_hbm, wk_hbm, wv_hbm, wo_hbm, w1_hbm, w2_hbm, w3_hbm, w4_hbm,
               out_hbm,
               wq_s, wk_s, wv_s, wo_s, w1_s, w2_s, w3_s, w4_s,
               xs, xl, rq, rk, rv, o2, hs, h1s, ostage,
               sem_x, sem_w, sem_wo, sem_b, sem_o):
        def x_copy(j):
            return pltpu.make_async_copy(x_hbm.at[:, j * LANE:(j + 1) * LANE], xs.at[j], sem_x.at[j])

        def pair_copies(j):
            cps = []
            for w_hbm, w_s in ((wq_hbm, wq_s), (wk_hbm, wk_s), (wv_hbm, wv_s)):
                wb = w_hbm.bitcast(U32)
                for p in range(2):
                    cps.append(pltpu.make_async_copy(wb.at[:, p, j, :], w_s.at[2 * j + p], sem_w.at[j]))
            return cps

        def col_copy(w_hbm, w_s, j, sem):
            return pltpu.make_async_copy(w_hbm.bitcast(U32).at[:, pl.ds(j * LANE, LANE)], w_s.at[j], sem)

        def b_copies():
            cps = []
            for i, (w_hbm, w_s) in enumerate(((w1_hbm, w1_s), (w2_hbm, w2_s), (w3_hbm, w3_s), (w4_hbm, w4_s))):
                for j in range(w_s.shape[0]):
                    cps.append(col_copy(w_hbm, w_s, j, sem_b.at[i]))
            return cps

        for j in range(KD):
            x_copy(j).start()
        for j in range(2):
            for c in pair_copies(j):
                c.start()

        for k in range(KD):
            xl[k, P:P + M, :] = mem0_ref[:, k * LANE:(k + 1) * LANE]
        for j in range(KD):
            x_copy(j).wait()

        def ln_rows(src_row, dst_row, n):
            xf = _cat([xs[k, pl.ds(src_row, n), :] for k in range(KD)], 1).astype(F32)
            xn = _ln(xf).astype(BF16)
            for k in range(KD):
                xl[k, pl.ds(dst_row, n), :] = xn[:, k * LANE:(k + 1) * LANE]

        def ln0_body(i, c):
            r = pl.multiple_of(i * 64, 64)
            ln_rows(r, r, 64)
            return c
        lax.fori_loop(0, P // 64, ln0_body, 0)

        def pro_body(j, c):
            @pl.when(j + 2 < NPAIR)
            def _():
                for cp in pair_copies(j + 2):
                    cp.start()

            @pl.when(j < KD)
            def _():
                col_copy(wo_hbm, wo_s, j, sem_wo.at[j]).start()

            for cp in pair_copies(j):
                cp.wait()
            lhs = _cat([xl[k, 0:P, :] for k in range(KD)], 1)
            for w_s, r_s in ((wq_s, rq), (wk_s, rk), (wv_s, rv)):
                a = w_s[2 * j]
                b = w_s[2 * j + 1]
                lo = (a & np.uint32(0xFFFF)) | (b << 16)
                hi = (a >> 16) | (b & np.uint32(0xFFFF0000))
                w_s[2 * j] = lo
                w_s[2 * j + 1] = hi
                r_s[0][j, 0:P, :] = jnp.dot(lhs, _bf(lo), preferred_element_type=F32).astype(BF16)
                r_s[1][j, 0:P, :] = jnp.dot(lhs, _bf(hi), preferred_element_type=F32).astype(BF16)
            for i in range(LNS):
                s = j * LNS + i
                ln_rows(pl.multiple_of(P + s * TOK, 8), pl.multiple_of(P + s * SEG + M, 8), TOK)
            return c
        lax.fori_loop(0, NPAIR, pro_body, 0)

        for cp in b_copies():
            cp.start()
        for j in range(KD):
            col_copy(wo_hbm, wo_s, j, sem_wo.at[j]).wait()

        def step(s, c):
            srow = pl.multiple_of(s * SEG, SEG)
            lhs = _cat([xl[k, pl.ds(P + srow, SEG), :] for k in range(KD)], 1)
            wr = [pl.multiple_of(lax.rem(P + s * TOK + 8 * i, R), 8) for i in range(TOK // 8)]
            rr = pl.multiple_of(lax.rem(srow, R), SEG)
            orow = []
            for i in range(SEG // 8):
                p = s * (SEG // 8) + i
                a = (p // (TOK // 8)) * SEG + M + (p % (TOK // 8)) * 8
                b = (s + PT) * SEG + 8 * i
                orow.append(pl.multiple_of(jnp.where(s < NSEG - PT, a, b), 8))
            L = SEG + M
            qi = lax.broadcasted_iota(jnp.int32, (L, L), 0)
            kj = lax.broadcasted_iota(jnp.int32, (L, L), 1)
            mask = (qi >= SEG) | (kj >= SEG) | (kj <= qi)

            mems = {}

            def proj(h):
                vals = []
                for w_s, r_s in ((wq_s, rq), (wk_s, rk), (wv_s, rv)):
                    y = jnp.dot(lhs, _bf(w_s[h]), preferred_element_type=F32)
                    for i in range(TOK // 8):
                        r_s[h % 2][h // 2, pl.ds(wr[i], 8), :] = y[M + 8 * i:M + 8 * i + 8, :].astype(BF16)
                    vals.append(y[0:M, :].astype(BF16))
                mems[h] = vals

            probs = {}

            def score(h):
                qm, km, _ = mems[h]
                q = _cat([rq[h % 2][h // 2, pl.ds(rr, SEG), :], qm], 0)
                k = _cat([rk[h % 2][h // 2, pl.ds(rr, SEG), :], km], 0)
                sc = lax.dot_general(q, k, (((1,), (1,)), ((), ())), preferred_element_type=F32)
                sc = jnp.where(mask, sc * scale, np.float32(-1e9))
                mx = jnp.max(sc, axis=-1, keepdims=True)
                e = jnp.exp(sc - mx)
                l = jnp.sum(e, axis=-1, keepdims=True)
                probs[h] = (e * pl.reciprocal(l, approx=False)).astype(BF16)

            def pv(h):
                _, _, vm = mems.pop(h)
                v = _cat([rv[h % 2][h // 2, pl.ds(rr, SEG), :], vm], 0)
                o = jnp.dot(probs.pop(h), v, preferred_element_type=F32)
                for i in range(SEG // 8):
                    o2[h][pl.ds(orow[i], 8), :] = o[8 * i:8 * i + 8, :].astype(BF16)
                o2[h][pl.ds(srow, M), :] = o[SEG:SEG + M, :].astype(BF16)

            def wo_part(hs_):
                lo_ = _cat([o2[h][pl.ds(srow, SEG), :] for h in hs_], 1)
                outs = []
                for j in range(KD):
                    w = wo_s[j, hs_[0] * (DH // 2):(hs_[-1] + 1) * (DH // 2), :]
                    outs.append(jnp.dot(lo_, _bf(w), preferred_element_type=F32))
                return outs

            L1, L2 = CFG["L1"], CFG["L2"]
            HS = CFG["HS"]
            part_a = None
            for t in range(H + L2):
                if t < H:
                    proj(t)
                if t == H:
                    part_a = wo_part(list(range(HS)))
                if 0 <= t - L1 < H:
                    score(t - L1)
                if 0 <= t - L2 < H:
                    pv(t - L2)
            part_b = wo_part(list(range(HS, H)))
            accs = [a + b for a, b in zip(part_a, part_b)]
            hrow = pl.multiple_of(s * TOK, 8)
            for j in range(KD):
                acc = accs[j]
                xl[j, pl.ds(P + srow + SEG, M), :] = acc[0:M, :].astype(BF16)
                hs[j, pl.ds(hrow, TOK), :] = (xs[j, pl.ds(hrow, TOK), :].astype(F32) + acc[M:SEG, :]).astype(BF16)
            return c
        lax.fori_loop(0, NSEG, step, 0)

        TE = 128

        def epi_body(i, c):
            r = pl.multiple_of(NSEG * SEG + i * TE, TE)
            t = pl.multiple_of(NSEG * TOK + i * TE, TE)
            lo_ = _cat([o2[h][pl.ds(r, TE), :] for h in range(H)], 1)
            for j in range(KD):
                acc = jnp.dot(lo_, _bf(wo_s[j]), preferred_element_type=F32)
                hs[j, pl.ds(t, TE), :] = (xs[j, pl.ds(t, TE), :].astype(F32) + acc).astype(BF16)
            return c
        lax.fori_loop(0, P // TE, epi_body, 0)

        for cp in b_copies():
            cp.wait()
        zero_halo = jnp.zeros((HALO, LANE), BF16)
        for j in range(KD):
            h1s[j, 0:HALO, :] = zero_halo
            h1s[j, HALO + S:HALO + S + HALO, :] = zero_halo

        def load_h(r):
            return _cat([hs[k, pl.ds(r, TB), :] for k in range(KD)], 1).astype(F32)

        def b1_body(i, c):
            r = pl.multiple_of(i * TB, TB)
            a = _ln(_ln(load_h(r))).astype(BF16)
            for j in range(KD):
                z = jnp.dot(a, _bf(w1_s[j]), preferred_element_type=F32)
                h1s[j, pl.ds(HALO + r, TB), :] = _gelu(z).astype(BF16)
            return c
        lax.fori_loop(0, NB, b1_body, 0)

        shifts = (-1, 1, -2, 2)

        def out_copy(i, slot):
            return pltpu.make_async_copy(ostage.at[slot], out_hbm.at[pl.ds(i * TB, TB), :], sem_o.at[slot])

        def b2_body(i, c):
            r = pl.multiple_of(i * TB, TB)
            slot = lax.rem(i, 2)
            cols = []
            for j in range(KD):
                d = shifts[j // (KD // 4)]
                win = h1s[j, pl.ds(r, TB + 2 * HALO), :].astype(F32)
                cols.append(win[HALO + d:HALO + d + TB, :].astype(BF16))
            g = _cat(cols, 1)
            hf = load_h(r)
            xb = _ln(hf)
            x1 = _cat([jnp.dot(g, _bf(w2_s[j]), preferred_element_type=F32) for j in range(KD)], 1) + xb
            a = _ln(x1).astype(BF16)
            u = _cat([_gelu(jnp.dot(a, _bf(w3_s[f]), preferred_element_type=F32)).astype(BF16)
                      for f in range(KF)], 1)
            res = hf + x1

            @pl.when(i >= 2)
            def _():
                out_copy(i - 2, slot).wait()
            for j in range(KD):
                y = jnp.dot(u, _bf(w4_s[j]), preferred_element_type=F32)
                ostage[slot, :, j * LANE:(j + 1) * LANE] = (res[:, j * LANE:(j + 1) * LANE] + y).astype(BF16)
            out_copy(i, slot).start()
            return c
        lax.fori_loop(0, NB, b2_body, 0)
        for i in range(NB - 2, NB):
            out_copy(i, i % 2).wait()

    scratch = [
        pltpu.VMEM((H, D // 2, LANE), U32),
        pltpu.VMEM((H, D // 2, LANE), U32),
        pltpu.VMEM((H, D // 2, LANE), U32),
        pltpu.VMEM((KD, H * DH // 2, LANE), U32),
        pltpu.VMEM((KD, D // 2, LANE), U32),
        pltpu.VMEM((KD, D // 2, LANE), U32),
        pltpu.VMEM((KF, D // 2, LANE), U32),
        pltpu.VMEM((KD, F // 2, LANE), U32),
        pltpu.VMEM((KD, S, LANE), BF16),
        pltpu.VMEM((KD, P + (NSEG + 1) * SEG, LANE), BF16),
        [pltpu.VMEM((H // 2, R, LANE), BF16) for _ in range(2)],
        [pltpu.VMEM((H // 2, R, LANE), BF16) for _ in range(2)],
        [pltpu.VMEM((H // 2, R, LANE), BF16) for _ in range(2)],
        [pltpu.VMEM((NSEG * SEG + P, LANE), BF16) for _ in range(H)],
        pltpu.VMEM((KD, S, LANE), BF16),
        pltpu.VMEM((KD, S + 2 * HALO, LANE), BF16),
        pltpu.VMEM((2, TB, D), BF16),
        pltpu.SemaphoreType.DMA((KD,)),
        pltpu.SemaphoreType.DMA((NPAIR,)),
        pltpu.SemaphoreType.DMA((KD,)),
        pltpu.SemaphoreType.DMA((4,)),
        pltpu.SemaphoreType.DMA((2,)),
    ]
    return kernel, scratch


@functools.partial(jax.jit, static_argnames=("A_seg_len",))
def pallas_sequential_preLN__memory_aug_recurrent_mem_tr__mixer_s_mlp__prompt_kernel(
    A_x, A_mem0, A_Wq, A_Wk, A_Wv, A_Wo, A_seg_len, B_x, B_w1, B_w2, B_w3, B_w4,
):
    del B_x
    B, S, D = A_x.shape
    M = A_mem0.shape[1]
    H, DH = A_Wq.shape[1], A_Wq.shape[2]
    F = B_w3.shape[1]
    SEG = int(A_seg_len)
    assert B == 1 and DH == LANE and M == 8 and SEG == 32 and H % 8 == 0 and D == 4 * 2 * LANE
    kernel, scratch = _make_kernel(S, D, H, DH, M, SEG, F, TB=256)
    any_spec = pl.BlockSpec(memory_space=pl.ANY)
    out = pl.pallas_call(
        kernel,
        out_shape=jax.ShapeDtypeStruct((S, D), A_x.dtype),
        in_specs=[any_spec, pl.BlockSpec()] + [any_spec] * 8,
        out_specs=any_spec,
        scratch_shapes=scratch,
        compiler_params=pltpu.CompilerParams(vmem_limit_bytes=120 * 1024 * 1024),
    )(
        A_x.reshape(S, D),
        A_mem0.reshape(M, D),
        A_Wq.reshape(D // 2, 2, H, DH),
        A_Wk.reshape(D // 2, 2, H, DH),
        A_Wv.reshape(D // 2, 2, H, DH),
        A_Wo.reshape(H * DH, D),
        B_w1, B_w2, B_w3, B_w4,
    )
    return out.reshape(B, S, D)
```

```python
import functools

import numpy as np
import jax
import jax.numpy as jnp
from jax import lax
import jax.experimental.pallas as pl
import jax.experimental.pallas.tpu as pltpu

F32 = jnp.float32
BF16 = jnp.bfloat16
U32 = jnp.uint32
LANE = 128
EPS = 1e-5
CFG = dict(LG=0, PVK=2, PVE=1)


def _bf(w_u32):
    return pltpu.bitcast(w_u32, BF16)


def _ln(x):
    m = jnp.mean(x, axis=-1, keepdims=True)
    d = x - m
    v = jnp.mean(d * d, axis=-1, keepdims=True)
    return d * lax.rsqrt(v + EPS)


def _gelu(x):
    c0 = np.float32(np.sqrt(2.0 / np.pi))
    c1 = np.float32(np.sqrt(2.0 / np.pi) * 0.044715)
    t = jnp.tanh(x * (c0 + c1 * (x * x)))
    hx = 0.5 * x
    return hx + hx * t


def _cat(xs, axis):
    return xs[0] if len(xs) == 1 else jnp.concatenate(xs, axis=axis)


def _make_kernel(S, D, H, DH, M, SEG, F, TB):
    NSEG = S // SEG
    TOK = SEG - M
    P = S - NSEG * TOK
    R = SEG * TOK * -(-(P + SEG) // (SEG * TOK))
    KD = D // LANE
    KF = F // LANE
    NPAIR = H // 2
    NB = S // TB
    HALO = 16
    scale = np.float32(DH ** (-0.5))
    PT = P // SEG
    LNS = NSEG // NPAIR

    def kernel(x_hbm, mem0_ref, wq_hbm, wk_hbm, wv_hbm, wo_hbm, w1_hbm, w2_hbm, w3_hbm, w4_hbm,
               out_hbm,
               wq_s, wk_s, wv_s, wo_s, w1_s, w2_s, w3_s, w4_s,
               xs, xl, rq, rk, rv, o2, ps, wacc, hs, h1s, ostage,
               sem_x, sem_w, sem_wo, sem_b, sem_o):
        def x_copy(j):
            return pltpu.make_async_copy(x_hbm.at[:, j * LANE:(j + 1) * LANE], xs.at[j], sem_x.at[j])

        def pair_copies(j):
            cps = []
            for w_hbm, w_s in ((wq_hbm, wq_s), (wk_hbm, wk_s), (wv_hbm, wv_s)):
                wb = w_hbm.bitcast(U32)
                for p in range(2):
                    cps.append(pltpu.make_async_copy(wb.at[:, p, j, :], w_s.at[2 * j + p], sem_w.at[j]))
            return cps

        def col_copy(w_hbm, w_s, j, sem):
            return pltpu.make_async_copy(w_hbm.bitcast(U32).at[:, pl.ds(j * LANE, LANE)], w_s.at[j], sem)

        def b_copies():
            cps = []
            for i, (w_hbm, w_s) in enumerate(((w1_hbm, w1_s), (w2_hbm, w2_s), (w3_hbm, w3_s), (w4_hbm, w4_s))):
                for j in range(w_s.shape[0]):
                    cps.append(col_copy(w_hbm, w_s, j, sem_b.at[i]))
            return cps

        for j in range(KD):
            x_copy(j).start()
        for j in range(2):
            for c in pair_copies(j):
                c.start()

        for k in range(KD):
            xl[k, P:P + M, :] = mem0_ref[:, k * LANE:(k + 1) * LANE]
        for j in range(KD):
            x_copy(j).wait()

        def ln_rows(src_row, dst_row, n):
            xf = _cat([xs[k, pl.ds(src_row, n), :] for k in range(KD)], 1).astype(F32)
            xn = _ln(xf).astype(BF16)
            for k in range(KD):
                xl[k, pl.ds(dst_row, n), :] = xn[:, k * LANE:(k + 1) * LANE]

        def ln0_body(i, c):
            r = pl.multiple_of(i * 64, 64)
            ln_rows(r, r, 64)
            return c
        lax.fori_loop(0, P // 64, ln0_body, 0)

        def pro_body(i, c):
            @pl.when(2 * i + 2 < NPAIR)
            def _():
                for j in (2 * i + 2, 2 * i + 3):
                    for cp in pair_copies(j):
                        cp.start()

            col_copy(wo_hbm, wo_s, i, sem_wo.at[i]).start()
            lhs = _cat([xl[k, 0:P, :] for k in range(KD)], 1)
            for cls in range(2):
                j = 2 * i + cls
                for cp in pair_copies(j):
                    cp.wait()
                for w_s, r_s in ((wq_s, rq), (wk_s, rk), (wv_s, rv)):
                    a = w_s[2 * j]
                    b = w_s[2 * j + 1]
                    lo = (a & np.uint32(0xFFFF)) | (b << 16)
                    hi = (a >> 16) | (b & np.uint32(0xFFFF0000))
                    w_s[2 * j] = lo
                    w_s[2 * j + 1] = hi
                    r_s[cls][i, 0, 0:P, :] = jnp.dot(lhs, _bf(lo), preferred_element_type=F32).astype(BF16)
                    r_s[cls][i, 1, 0:P, :] = jnp.dot(lhs, _bf(hi), preferred_element_type=F32).astype(BF16)
            for t in range(2 * LNS):
                s = i * 2 * LNS + t
                ln_rows(pl.multiple_of(P + s * TOK, 8), pl.multiple_of(P + s * SEG + M, 8), TOK)
            return c
        lax.fori_loop(0, NPAIR // 2, pro_body, 0)

        for cp in b_copies():
            cp.start()
        for j in range(KD):
            col_copy(wo_hbm, wo_s, j, sem_wo.at[j]).wait()

        def step(s, c):
            srow = pl.multiple_of(s * SEG, SEG)
            lhs = _cat([xl[k, pl.ds(P + srow, SEG), :] for k in range(KD)], 1)
            wr = [pl.multiple_of(lax.rem(P + s * TOK + 8 * i, R), 8) for i in range(TOK // 8)]
            rr = pl.multiple_of(lax.rem(srow, R), SEG)
            orow = []
            for i in range(SEG // 8):
                p = s * (SEG // 8) + i
                a = (p // (TOK // 8)) * SEG + M + (p % (TOK // 8)) * 8
                b = (s + PT) * SEG + 8 * i
                orow.append(pl.multiple_of(jnp.where(s < NSEG - PT, a, b), 8))
            L = 2 * (SEG + M)
            ri = lax.broadcasted_iota(jnp.int32, (L, L), 0)
            ci = lax.broadcasted_iota(jnp.int32, (L, L), 1)

            def head_of(i):
                return ((i >= SEG) & (i < 2 * SEG)) | (i >= 2 * SEG + M)
            same = head_of(ri) == head_of(ci)
            allowed = same & ((ri >= 2 * SEG) | (ci >= 2 * SEG) | ((ci & (SEG - 1)) <= (ri & (SEG - 1))))
            fill = jnp.where(same, np.float32(-1e9), np.float32(-1e30))

            def slab(r_s, h):
                j = h // 2
                return r_s[j % 2].at[j // 2, h % 2]

            def proj(w_s, r_s, h):
                y = jnp.dot(lhs, _bf(w_s[h]), preferred_element_type=F32)
                dst = slab(r_s, h)
                dst[R:R + M, :] = y[0:M, :].astype(BF16)
                for i in range(TOK // 8):
                    dst[pl.ds(wr[i], 8), :] = y[M + 8 * i:M + 8 * i + 8, :].astype(BF16)

            def stack(r_s, j):
                s0, s1 = slab(r_s, 2 * j), slab(r_s, 2 * j + 1)
                return _cat([s0[pl.ds(rr, SEG), :], s1[pl.ds(rr, SEG), :], s0[R:R + M, :], s1[R:R + M, :]], 0)

            def proj_qk(j):
                for w_s, r_s in ((wq_s, rq), (wk_s, rk)):
                    proj(w_s, r_s, 2 * j)
                    proj(w_s, r_s, 2 * j + 1)

            def proj_v(j):
                proj(wv_s, rv, 2 * j)
                proj(wv_s, rv, 2 * j + 1)

            def score(j):
                q = stack(rq, j)
                k = stack(rk, j)
                sc = lax.dot_general(q, k, (((1,), (1,)), ((), ())), preferred_element_type=F32)
                sc = jnp.where(allowed, sc * scale, fill)
                mx = jnp.max(sc, axis=-1, keepdims=True)
                e = jnp.exp(sc - mx)
                l = jnp.sum(e, axis=-1, keepdims=True)
                r = pl.reciprocal(l, approx=True)
                r = r * (2.0 - l * r)
                ps[j][...] = (e * r).astype(BF16)

            def pv(j):
                o = jnp.dot(ps[j][...], stack(rv, j), preferred_element_type=F32)
                for hh in range(2):
                    dst = o2[2 * j + hh]
                    for i in range(SEG // 8):
                        dst[pl.ds(orow[i], 8), :] = o[hh * SEG + 8 * i:hh * SEG + 8 * i + 8, :].astype(BF16)
                    dst[pl.ds(srow, M), :] = o[2 * SEG + hh * M:2 * SEG + (hh + 1) * M, :].astype(BF16)

            def wo_tile(par, j):
                pairs = range(par, NPAIR, 2)
                lo_ = _cat([o2[2 * pj + hh][pl.ds(srow, SEG), :] for pj in pairs for hh in range(2)], 1)
                w = _cat([wo_s[j, pj * DH:(pj + 1) * DH, :] for pj in pairs], 0)
                return jnp.dot(lo_, _bf(w), preferred_element_type=F32)

            NH = NPAIR // 2
            accs = [None] * KD

            def wo_a(j):
                wacc[j] = wo_tile(0, j)

            def wo_b(j):
                accs[j] = wacc[j] + wo_tile(1, j)
                finish(j)

            hrow = pl.multiple_of(s * TOK, 8)

            def finish(j):
                acc = accs[j]
                xl[j, pl.ds(P + srow + SEG, M), :] = acc[0:M, :].astype(BF16)
                hs[j, pl.ds(hrow, TOK), :] = (xs[j, pl.ds(hrow, TOK), :].astype(F32) + acc[M:SEG, :]).astype(BF16)

            main = ([(proj_qk, 2 * i) for i in range(NH)] + [(proj_qk, 2 * i + 1) for i in range(NH)]
                    + [(proj_v, 2 * i) for i in range(NH)] + [(proj_v, 2 * i + 1) for i in range(NH)]
                    + [(wo_a, j) for j in range(KD)] + [(wo_b, j) for j in range(KD)])
            extra = {}
            LG, PVK = CFG["LG"], CFG["PVK"]
            for i in range(NH):
                extra.setdefault(NH + i + LG, []).append((score, 2 * i))
                extra.setdefault(2 * NH + i + LG, []).append((score, 2 * i + 1))
                extra.setdefault(3 * NH + i // CFG["PVE"] + LG, []).append((pv, 2 * i))
                extra.setdefault(4 * NH + LG + i // PVK, []).append((pv, 2 * i + 1))
            for t, (fn, arg) in enumerate(main):
                fn(arg)
                for fn2, arg2 in extra.get(t, []):
                    fn2(arg2)
            return c
        lax.fori_loop(0, NSEG, step, 0)
        TE = 128

        def epi_body(i, c):
            r = pl.multiple_of(NSEG * SEG + i * TE, TE)
            t = pl.multiple_of(NSEG * TOK + i * TE, TE)
            lo_ = _cat([o2[h][pl.ds(r, TE), :] for h in range(H)], 1)
            for j in range(KD):
                acc = jnp.dot(lo_, _bf(wo_s[j]), preferred_element_type=F32)
                hs[j, pl.ds(t, TE), :] = (xs[j, pl.ds(t, TE), :].astype(F32) + acc).astype(BF16)
            return c
        lax.fori_loop(0, P // TE, epi_body, 0)

        for cp in b_copies():
            cp.wait()
        zero_halo = jnp.zeros((HALO, LANE), BF16)
        for j in range(KD):
            h1s[j, 0:HALO, :] = zero_halo
            h1s[j, HALO + S:HALO + S + HALO, :] = zero_halo

        def load_h(r):
            return _cat([hs[k, pl.ds(r, TB), :] for k in range(KD)], 1).astype(F32)

        def b1_body(i, c):
            r = pl.multiple_of(i * TB, TB)
            a = _ln(_ln(load_h(r))).astype(BF16)
            for j in range(KD):
                z = jnp.dot(a, _bf(w1_s[j]), preferred_element_type=F32)
                h1s[j, pl.ds(HALO + r, TB), :] = _gelu(z).astype(BF16)
            return c
        lax.fori_loop(0, NB, b1_body, 0)

        shifts = (-1, 1, -2, 2)

        def out_copy(i, slot):
            return pltpu.make_async_copy(ostage.at[slot], out_hbm.at[pl.ds(i * TB, TB), :], sem_o.at[slot])

        def b2_body(i, c):
            r = pl.multiple_of(i * TB, TB)
            slot = lax.rem(i, 2)
            cols = []
            for j in range(KD):
                d = shifts[j // (KD // 4)]
                win = h1s[j, pl.ds(r, TB + 2 * HALO), :].astype(F32)
                cols.append(win[HALO + d:HALO + d + TB, :].astype(BF16))
            g = _cat(cols, 1)
            hf = load_h(r)
            xb = _ln(hf)
            x1 = _cat([jnp.dot(g, _bf(w2_s[j]), preferred_element_type=F32) for j in range(KD)], 1) + xb
            a = _ln(x1).astype(BF16)
            u = _cat([_gelu(jnp.dot(a, _bf(w3_s[f]), preferred_element_type=F32)).astype(BF16)
                      for f in range(KF)], 1)
            res = hf + x1

            @pl.when(i >= 2)
            def _():
                out_copy(i - 2, slot).wait()
            for j in range(KD):
                y = jnp.dot(u, _bf(w4_s[j]), preferred_element_type=F32)
                ostage[slot, :, j * LANE:(j + 1) * LANE] = (res[:, j * LANE:(j + 1) * LANE] + y).astype(BF16)
            out_copy(i, slot).start()
            return c
        lax.fori_loop(0, NB, b2_body, 0)
        for i in range(NB - 2, NB):
            out_copy(i, i % 2).wait()

    scratch = [
        pltpu.VMEM((H, D // 2, LANE), U32),
        pltpu.VMEM((H, D // 2, LANE), U32),
        pltpu.VMEM((H, D // 2, LANE), U32),
        pltpu.VMEM((KD, H * DH // 2, LANE), U32),
        pltpu.VMEM((KD, D // 2, LANE), U32),
        pltpu.VMEM((KD, D // 2, LANE), U32),
        pltpu.VMEM((KF, D // 2, LANE), U32),
        pltpu.VMEM((KD, F // 2, LANE), U32),
        pltpu.VMEM((KD, S, LANE), BF16),
        pltpu.VMEM((KD, P + (NSEG + 1) * SEG, LANE), BF16),
        [pltpu.VMEM((NPAIR // 2, 2, R + 16, LANE), BF16) for _ in range(2)],
        [pltpu.VMEM((NPAIR // 2, 2, R + 16, LANE), BF16) for _ in range(2)],
        [pltpu.VMEM((NPAIR // 2, 2, R + 16, LANE), BF16) for _ in range(2)],
        [pltpu.VMEM((NSEG * SEG + P, LANE), BF16) for _ in range(H)],
        [pltpu.VMEM((2 * (SEG + M), 2 * (SEG + M)), BF16) for _ in range(NPAIR)],
        pltpu.VMEM((KD, SEG, LANE), F32),
        pltpu.VMEM((KD, S, LANE), BF16),
        pltpu.VMEM((KD, S + 2 * HALO, LANE), BF16),
        pltpu.VMEM((2, TB, D), BF16),
        pltpu.SemaphoreType.DMA((KD,)),
        pltpu.SemaphoreType.DMA((NPAIR,)),
        pltpu.SemaphoreType.DMA((KD,)),
        pltpu.SemaphoreType.DMA((4,)),
        pltpu.SemaphoreType.DMA((2,)),
    ]
    return kernel, scratch


@functools.partial(jax.jit, static_argnames=("A_seg_len",))
def pallas_sequential_preLN__memory_aug_recurrent_mem_tr__mixer_s_mlp__prompt_kernel(
    A_x, A_mem0, A_Wq, A_Wk, A_Wv, A_Wo, A_seg_len, B_x, B_w1, B_w2, B_w3, B_w4,
):
    del B_x
    B, S, D = A_x.shape
    M = A_mem0.shape[1]
    H, DH = A_Wq.shape[1], A_Wq.shape[2]
    F = B_w3.shape[1]
    SEG = int(A_seg_len)
    assert B == 1 and DH == LANE and M == 8 and SEG == 32 and H % 8 == 0 and D == 4 * 2 * LANE
    kernel, scratch = _make_kernel(S, D, H, DH, M, SEG, F, TB=256)
    any_spec = pl.BlockSpec(memory_space=pl.ANY)
    out = pl.pallas_call(
        kernel,
        out_shape=jax.ShapeDtypeStruct((S, D), A_x.dtype),
        in_specs=[any_spec, pl.BlockSpec()] + [any_spec] * 8,
        out_specs=any_spec,
        scratch_shapes=scratch,
        compiler_params=pltpu.CompilerParams(vmem_limit_bytes=120 * 1024 * 1024),
    )(
        A_x.reshape(S, D),
        A_mem0.reshape(M, D),
        A_Wq.reshape(D // 2, 2, H, DH),
        A_Wk.reshape(D // 2, 2, H, DH),
        A_Wv.reshape(D // 2, 2, H, DH),
        A_Wo.reshape(H * DH, D),
        B_w1, B_w2, B_w3, B_w4,
    )
    return out.reshape(B, S, D)
```

```python
import functools

import numpy as np
import jax
import jax.numpy as jnp
from jax import lax
import jax.experimental.pallas as pl
import jax.experimental.pallas.tpu as pltpu

F32 = jnp.float32
BF16 = jnp.bfloat16
U32 = jnp.uint32
LANE = 128
EPS = 1e-5
CFG = dict(LG=0, PVK=2, PVE=1, LA=2, WOF=2, WON=4, CH=64, ORDER='b0 a0 c0 b1 a1 c1 d0 b2 a2 c2 d1 b3 a3 c3 d2 d3',
           ORDER2='b0 b1 b2 b3 c0 c1 c2 c3 d0 d1 d2 d3', FLAGS=None)


def _bf(w_u32):
    return pltpu.bitcast(w_u32, BF16)


def _rows(ref, idx, start, n):
    w = ref.bitcast(U32)
    if isinstance(start, int):
        words = w[(*idx, slice(start // 2, (start + n) // 2), slice(None))]
    else:
        words = w[(*idx, pl.ds(pl.multiple_of(start // 2, 8), n // 2), slice(None))]
    return pltpu.bitcast(words, BF16)


def _ln(x):
    m = jnp.mean(x, axis=-1, keepdims=True)
    d = x - m
    v = jnp.mean(d * d, axis=-1, keepdims=True)
    return d * lax.rsqrt(v + EPS)


def _gelu(x):
    c0 = np.float32(np.sqrt(2.0 / np.pi))
    c1 = np.float32(np.sqrt(2.0 / np.pi) * 0.044715)
    t = jnp.tanh(x * (c0 + c1 * (x * x)))
    hx = 0.5 * x
    return hx + hx * t


def _cat(xs, axis):
    return xs[0] if len(xs) == 1 else jnp.concatenate(xs, axis=axis)


def _make_kernel(S, D, H, DH, M, SEG, F, TB):
    NSEG = S // SEG
    TOK = SEG - M
    P = S - NSEG * TOK
    R = SEG * TOK * -(-(P + SEG) // (SEG * TOK))
    KD = D // LANE
    KF = F // LANE
    NPAIR = H // 2
    NB = S // TB
    HALO = 16
    YB = 4
    scale = np.float32(DH ** (-0.5))
    PT = P // SEG
    LNS = NSEG // NPAIR

    def kernel(x_hbm, mem0_ref, wq_hbm, wk_hbm, wv_hbm, wo_hbm, w1_hbm, w2_hbm, w3_hbm, w4_hbm,
               out_hbm,
               wq_s, wk_s, wv_s, wo_s, w1_s, w2_s, w3_s, w4_s,
               xs, xn0, xl, rq, rk, rv, o2, ps, wacc, hs, h1s, a1, gs, ys, x1s, a3, us, ostage,
               sem_x, sem_w, sem_b, sem_o):
        wqkv = ((wq_hbm, wq_s), (wk_hbm, wk_s), (wv_hbm, wv_s))

        def x_copies(lo, n, sem):
            return [pltpu.make_async_copy(x_hbm.at[pl.ds(lo, n), j * LANE:(j + 1) * LANE],
                                          xs.at[j, pl.ds(lo, n)], sem) for j in range(KD)]

        def pair_copies(j, m, src=None):
            w_hbm, w_s = wqkv[m]
            wb = w_hbm.bitcast(U32)
            src = j if src is None else src
            return [pltpu.make_async_copy(wb.at[:, p, src, :], w_s.at[2 * j + p], sem_w.at[3 * j + m])
                    for p in range(2)]

        def col_copies(w_hbm, w_s, sem):
            wb = w_hbm.bitcast(U32)
            return [pltpu.make_async_copy(wb.at[:, pl.ds(j * LANE, LANE)], w_s.at[j], sem)
                    for j in range(w_s.shape[0])]

        x_head = x_copies(0, P, sem_x.at[0])
        XC = (S - P) // (NPAIR // 2)
        XA = 2
        x_tail_a = x_copies(P, XA * XC, sem_x.at[1])
        x_tail_b = x_copies(P + XA * XC, S - P - XA * XC, sem_x.at[2])
        wo_copies = col_copies(wo_hbm, wo_s, sem_b.at[4])
        b_groups = [col_copies(wh, ws, sem_b.at[i])
                    for i, (wh, ws) in enumerate(((w1_hbm, w1_s), (w2_hbm, w2_s), (w3_hbm, w3_s), (w4_hbm, w4_s)))]
        b_copies = [c for g in b_groups for c in g]

        NI = NPAIR // 2

        def start(cps):
            for cp in cps:
                cp.start()

        def need(i):
            return [(2 * i, 1), (2 * i, 2), (2 * i + 1, 0), (2 * i + 1, 1), (2 * i + 1, 2), (2 * i + 2, 0)]

        def group_copies(j, m):
            return pair_copies(j, m, src=0) if j == NPAIR else pair_copies(j, m)

        def need_copies(i):
            return [c for j, m in need(i) for c in group_copies(j, m)]

        LA = CFG["LA"]
        wo_first, wo_n = CFG["WOF"], CFG["WON"]
        issue = [[] for _ in range(NI)]
        for k in range(1, NI):
            if k + LA < NI:
                issue[k] += need_copies(k + LA)
            if wo_first <= k < wo_first + wo_n:
                issue[k] += wo_copies[(k - wo_first) * KD // wo_n:(k - wo_first + 1) * KD // wo_n]
        start(x_head + pair_copies(0, 0) + pair_copies(0, 1))

        for k in range(KD):
            xl[k, 0:M, :] = mem0_ref[:, k * LANE:(k + 1) * LANE]
        for cp in x_head:
            cp.wait()
        start(pair_copies(0, 2) + pair_copies(1, 0) + x_tail_a)

        def ln_rows(dst, src_row, dst_row, n):
            xf = _cat([xs[k, pl.ds(src_row, n), :] for k in range(KD)], 1).astype(F32)
            xn = _ln(xf).astype(BF16)
            for k in range(KD):
                dst[k, pl.ds(dst_row, n), :] = xn[:, k * LANE:(k + 1) * LANE]

        def ln0_body(i, c):
            r = pl.multiple_of(i * 128, 128)
            ln_rows(xn0, r, r, 128)
            return c
        lax.fori_loop(0, P // 128, ln0_body, 0)

        def untangle(j, m):
            w_s = wqkv[m][1]
            a = w_s[2 * j]
            b = w_s[2 * j + 1]
            w_s[2 * j] = (a & np.uint32(0xFFFF)) | (b << 16)
            w_s[2 * j + 1] = (a >> 16) | (b & np.uint32(0xFFFF0000))

        for cp in pair_copies(0, 0):
            cp.wait()
        untangle(0, 0)

        def pro_body(i, inline_waits):
            groups = [(cls, m) for cls in range(2) for m in range(3)]
            nxt = need(i)
            if not inline_waits:
                for jn, mn in nxt:
                    for cp in pair_copies(jn, mn, src=0):
                        cp.wait()

                @pl.when(i == XA)
                def _():
                    for cp in x_tail_b:
                        cp.wait()
                for k in range(1, NI):
                    pl.when(i == k)(functools.partial(start, issue[k]))
            else:
                n1 = need_copies(1)
                rolling = [pair_copies(1, 1) + pair_copies(1, 2), pair_copies(2, 0) + n1[0:4], n1[4:8], n1[8:12],
                           x_tail_b, [c for k in range(2, LA + 1) for c in need_copies(k)]]
            for n, (cls, m) in enumerate(groups):
                j = 2 * i + cls
                jn, mn = nxt[n]
                if inline_waits:
                    if n == 1:
                        for cp in x_tail_a:
                            cp.wait()
                    start(rolling[n])
                    for cp in pair_copies(jn, mn, src=0):
                        cp.wait()
                untangle(jn, mn)
                r_s = (rq, rk, rv)[m]
                for hh in range(2):
                    lhs = _cat([_rows(xn0, (k,), 0, P) for k in range(KD)], 1)
                    w = _bf(wqkv[m][1][2 * j + hh])
                    r_s[cls][i, hh, 0:P, :] = jnp.dot(lhs, w, preferred_element_type=F32).astype(BF16)
                if 1 <= n <= LNS:
                    for t in range(2):
                        sg = i * 2 * LNS + 2 * (n - 1) + t
                        ln_rows(xl, pl.multiple_of(P + sg * TOK, 8), pl.multiple_of(sg * SEG + M, 8), TOK)

        pro_body(0, True)

        def pro_loop(i, c):
            pro_body(i, False)
            return c
        lax.fori_loop(1, NPAIR // 2, pro_loop, 0)

        for cp in wo_copies:
            cp.wait()
        start(b_copies)

        def step(s, c):
            srow = pl.multiple_of(s * SEG, SEG)
            lhs = _cat([_rows(xl, (k,), srow, SEG) for k in range(KD)], 1)
            wr = [pl.multiple_of(lax.rem(P + s * TOK + 8 * i, R), 8) for i in range(TOK // 8)]
            rr = pl.multiple_of(lax.rem(srow, R), SEG)
            orow = []
            for i in range(SEG // 8):
                p = s * (SEG // 8) + i
                a = (p // (TOK // 8)) * SEG + M + (p % (TOK // 8)) * 8
                b = (s + PT) * SEG + 8 * i
                orow.append(pl.multiple_of(jnp.where(s < NSEG - PT, a, b), 8))
            L = 2 * (SEG + M)
            ri = lax.broadcasted_iota(jnp.int32, (L, L), 0)
            ci = lax.broadcasted_iota(jnp.int32, (L, L), 1)

            def head_of(i):
                return ((i >= SEG) & (i < 2 * SEG)) | (i >= 2 * SEG + M)
            same = head_of(ri) == head_of(ci)
            allowed = same & ((ri >= 2 * SEG) | (ci >= 2 * SEG) | ((ci & (SEG - 1)) <= (ri & (SEG - 1))))
            fill = jnp.where(same, np.float32(-1e9), np.float32(-1e30))

            def proj(w_s, r_s, h):
                j, hh = h // 2, h % 2
                ring = r_s[j % 2]
                y = jnp.dot(lhs, _bf(w_s[h]), preferred_element_type=F32)
                ring[j // 2, 0, R + hh * M:R + (hh + 1) * M, :] = y[0:M, :].astype(BF16)
                for i in range(TOK // 8):
                    ring[j // 2, hh, pl.ds(wr[i], 8), :] = y[M + 8 * i:M + 8 * i + 8, :].astype(BF16)

            def stack(r_s, j):
                ring = r_s[j % 2]
                return _cat([_rows(ring, (j // 2, 0), rr, SEG), _rows(ring, (j // 2, 1), rr, SEG),
                             _rows(ring, (j // 2, 0), R, 2 * M)], 0)

            def proj_qk(j):
                for w_s, r_s in ((wq_s, rq), (wk_s, rk)):
                    proj(w_s, r_s, 2 * j)
                    proj(w_s, r_s, 2 * j + 1)

            def proj_v(j):
                proj(wv_s, rv, 2 * j)
                proj(wv_s, rv, 2 * j + 1)

            def score(j):
                q = stack(rq, j)
                k = stack(rk, j)
                sc = lax.dot_general(q, k, (((1,), (1,)), ((), ())), preferred_element_type=F32)
                sc = jnp.where(allowed, sc * scale, fill)
                mx = jnp.max(sc, axis=-1, keepdims=True)
                e = jnp.exp(sc - mx)
                l = jnp.sum(e, axis=-1, keepdims=True)
                r = pl.reciprocal(l, approx=True)
                r = r * (2.0 - l * r)
                ps[j][...] = (e * r).astype(BF16)

            def pv(j):
                o = jnp.dot(ps[j][...], stack(rv, j), preferred_element_type=F32)
                for hh in range(2):
                    dst = o2[2 * j + hh]
                    for i in range(SEG // 8):
                        dst[pl.ds(orow[i], 8), :] = o[hh * SEG + 8 * i:hh * SEG + 8 * i + 8, :].astype(BF16)
                    dst[pl.ds(srow, M), :] = o[2 * SEG + hh * M:2 * SEG + (hh + 1) * M, :].astype(BF16)

            def wo_tile(par, j):
                pairs = range(par, NPAIR, 2)
                lo_ = _cat([_rows(o2[2 * pj + hh], (), srow, SEG) for pj in pairs for hh in range(2)], 1)
                w = _cat([wo_s[j, pj * DH:(pj + 1) * DH, :] for pj in pairs], 0)
                return jnp.dot(lo_, _bf(w), preferred_element_type=F32)

            NH = NPAIR // 2
            accs = [None] * KD

            def wo_a(j):
                wacc[j] = wo_tile(0, j)

            def wo_b(j):
                accs[j] = wacc[j] + wo_tile(1, j)
                finish(j)

            hrow = pl.multiple_of(s * TOK, 8)

            def finish(j):
                acc = accs[j]
                xl[j, pl.ds(srow + SEG, M), :] = acc[0:M, :].astype(BF16)
                hs[j, pl.ds(hrow, TOK), :] = (xs[j, pl.ds(hrow, TOK), :].astype(F32) + acc[M:SEG, :]).astype(BF16)

            main = ([(proj_qk, 2 * i) for i in range(NH)] + [(proj_qk, 2 * i + 1) for i in range(NH)]
                    + [(proj_v, 2 * i) for i in range(NH)] + [(proj_v, 2 * i + 1) for i in range(NH)]
                    + [(wo_a, j) for j in range(KD)] + [(wo_b, j) for j in range(KD)])
            extra = {}
            LG, PVK = CFG["LG"], CFG["PVK"]
            for i in range(NH):
                extra.setdefault(NH + i + LG, []).append((score, 2 * i))
                extra.setdefault(2 * NH + i + LG, []).append((score, 2 * i + 1))
                extra.setdefault(3 * NH + i // CFG["PVE"] + LG, []).append((pv, 2 * i))
                extra.setdefault(4 * NH + LG + i // PVK, []).append((pv, 2 * i + 1))
            for t, (fn, arg) in enumerate(main):
                fn(arg)
                for fn2, arg2 in extra.get(t, []):
                    fn2(arg2)
            return c
        lax.fori_loop(0, NSEG, step, 0)
        for cp in b_copies:
            cp.wait()
        zero_halo = jnp.zeros((HALO, LANE), BF16)
        for j in range(KD):
            h1s[j, 0:HALO, :] = zero_halo
            h1s[j, HALO + S:HALO + S + HALO, :] = zero_halo

        CH = CFG["CH"]

        def load_h(r, n):
            return _cat([hs[k, pl.ds(r, n), :] for k in range(KD)], 1).astype(F32)

        def put_cols(dst, row, val):
            for k in range(KD):
                dst[k, row:row + val.shape[0], :] = val[:, k * LANE:(k + 1) * LANE]

        def mix1_pre(r, q):
            y = _ln(load_h(r + q, CH))
            yr = pl.multiple_of(lax.rem(r, YB * TB) + q, CH)
            for k in range(KD):
                ys[k, pl.ds(yr, CH), :] = y[:, k * LANE:(k + 1) * LANE]
            put_cols(a1, q, _ln(y).astype(BF16))

        def mix1_dot(r, q):
            for j in range(KD):
                a = _cat([_rows(a1, (k,), q, CH) for k in range(KD)], 1)
                z = jnp.dot(a, _bf(w1_s[j]), preferred_element_type=F32)
                h1s[j, pl.ds(HALO + r + q, CH), :] = _gelu(z).astype(BF16)

        def mix1(r, q):
            mix1_pre(r, q)
            mix1_dot(r, q)

        shifts = (-1, 1, -2, 2)

        TE = 128
        assert (P // TE) * TE == 2 * TB

        def epi_body(i, c):
            r = pl.multiple_of(NSEG * SEG + i * TE, TE)
            t = pl.multiple_of(NSEG * TOK + i * TE, TE)
            r1 = pl.multiple_of(i * TE, TE)
            for q in range(0, TE, CH):
                mix1_pre(r1, q)
            for j in range(KD):
                lo_ = _cat([_rows(o2[h], (), r, TE) for h in range(H)], 1)
                acc = jnp.dot(lo_, _bf(wo_s[j]), preferred_element_type=F32)
                hs[j, pl.ds(t, TE), :] = (xs[j, pl.ds(t, TE), :].astype(F32) + acc).astype(BF16)
            for q in range(0, TE, CH):
                mix1_dot(r1, q)
            return c
        lax.fori_loop(0, P // TE, epi_body, 0)

        def out_copy(i, slot):
            return pltpu.make_async_copy(ostage.at[slot], out_hbm.at[pl.ds(i * TB, TB), :], sem_o.at[slot])

        def b2_body(i, with_mix1):
            r = pl.multiple_of(i * TB, TB)
            slot = lax.rem(i, 2)

            @pl.when(i >= 2)
            def _():
                out_copy(i - 2, slot).wait()

            def mix2(q):
                for j in range(KD):
                    d = shifts[j // (KD // 4)]
                    win = h1s[j, pl.ds(r + q, CH + 2 * HALO), :].astype(F32)
                    gs[j, q:q + CH, :] = win[HALO + d:HALO + d + CH, :].astype(BF16)
                yr = pl.multiple_of(lax.rem(r, YB * TB) + q, CH)
                for j in range(KD):
                    g = _cat([_rows(gs, (k,), q, CH) for k in range(KD)], 1)
                    x1s[j, q:q + CH, :] = (jnp.dot(g, _bf(w2_s[j]), preferred_element_type=F32)
                                           + ys[j, pl.ds(yr, CH), :])

            def up(q):
                put_cols(a3, q, _ln(_cat([x1s[k, q:q + CH, :] for k in range(KD)], 1)).astype(BF16))
                for f in range(KF):
                    a = _cat([_rows(a3, (k,), q, CH) for k in range(KD)], 1)
                    us[f, q:q + CH, :] = _gelu(jnp.dot(a, _bf(w3_s[f]), preferred_element_type=F32)).astype(BF16)

            def down(q):
                for j in range(KD):
                    u = _cat([_rows(us, (f,), q, CH) for f in range(KF)], 1)
                    y = jnp.dot(u, _bf(w4_s[j]), preferred_element_type=F32)
                    res = hs[j, pl.ds(r + q, CH), :].astype(F32) + x1s[j, q:q + CH, :]
                    ostage[slot, q:q + CH, j * LANE:(j + 1) * LANE] = (res + y).astype(BF16)

            r2 = pl.multiple_of((i + 2) * TB, TB)
            stage = {"a": lambda q: mix1(r2, q), "b": mix2, "c": up, "d": down}
            for name in CFG["ORDER" if with_mix1 else "ORDER2"].split():
                stage[name[0]](int(name[1:]) * CH)
            out_copy(i, slot).start()

        def b2_main(i, c):
            b2_body(i, True)
            return c

        def b2_tail(i, c):
            b2_body(i, False)
            return c
        lax.fori_loop(0, NB - 2, b2_main, 0)
        lax.fori_loop(NB - 2, NB, b2_tail, 0)
        for i in range(NB - 2, NB):
            out_copy(i, i % 2).wait()

    scratch = [
        pltpu.VMEM((H + 2, D // 2, LANE), U32),
        pltpu.VMEM((H, D // 2, LANE), U32),
        pltpu.VMEM((H, D // 2, LANE), U32),
        pltpu.VMEM((KD, H * DH // 2, LANE), U32),
        pltpu.VMEM((KD, D // 2, LANE), U32),
        pltpu.VMEM((KD, D // 2, LANE), U32),
        pltpu.VMEM((KF, D // 2, LANE), U32),
        pltpu.VMEM((KD, F // 2, LANE), U32),
        pltpu.VMEM((KD, S, LANE), BF16),
        pltpu.VMEM((KD, P, LANE), BF16),
        pltpu.VMEM((KD, (NSEG + 1) * SEG, LANE), BF16),
        [pltpu.VMEM((NPAIR // 2, 2, R + 16, LANE), BF16) for _ in range(2)],
        [pltpu.VMEM((NPAIR // 2, 2, R + 16, LANE), BF16) for _ in range(2)],
        [pltpu.VMEM((NPAIR // 2, 2, R + 16, LANE), BF16) for _ in range(2)],
        [pltpu.VMEM((NSEG * SEG + P, LANE), BF16) for _ in range(H)],
        [pltpu.VMEM((2 * (SEG + M), 2 * (SEG + M)), BF16) for _ in range(NPAIR)],
        pltpu.VMEM((KD, SEG, LANE), F32),
        pltpu.VMEM((KD, S, LANE), BF16),
        pltpu.VMEM((KD, S + 2 * HALO, LANE), BF16),
        pltpu.VMEM((KD, TB, LANE), BF16),
        pltpu.VMEM((KD, TB, LANE), BF16),
        pltpu.VMEM((KD, YB * TB, LANE), F32),
        pltpu.VMEM((KD, TB, LANE), F32),
        pltpu.VMEM((KD, TB, LANE), BF16),
        pltpu.VMEM((KF, TB, LANE), BF16),
        pltpu.VMEM((2, TB, D), BF16),
        pltpu.SemaphoreType.DMA((3,)),
        pltpu.SemaphoreType.DMA((3 * NPAIR + 1,)),
        pltpu.SemaphoreType.DMA((5,)),
        pltpu.SemaphoreType.DMA((2,)),
    ]
    return kernel, scratch


@functools.partial(jax.jit, static_argnames=("A_seg_len",))
def pallas_sequential_preLN__memory_aug_recurrent_mem_tr__mixer_s_mlp__prompt_kernel(
    A_x, A_mem0, A_Wq, A_Wk, A_Wv, A_Wo, A_seg_len, B_x, B_w1, B_w2, B_w3, B_w4,
):
    del B_x
    B, S, D = A_x.shape
    M = A_mem0.shape[1]
    H, DH = A_Wq.shape[1], A_Wq.shape[2]
    F = B_w3.shape[1]
    SEG = int(A_seg_len)
    assert B == 1 and DH == LANE and M == 8 and SEG == 32 and H % 8 == 0 and D == 4 * 2 * LANE
    kernel, scratch = _make_kernel(S, D, H, DH, M, SEG, F, TB=256)
    any_spec = pl.BlockSpec(memory_space=pl.ANY)
    out = pl.pallas_call(
        kernel,
        out_shape=jax.ShapeDtypeStruct((S, D), A_x.dtype),
        in_specs=[any_spec, pl.BlockSpec()] + [any_spec] * 8,
        out_specs=any_spec,
        scratch_shapes=scratch,
        compiler_params=pltpu.CompilerParams(vmem_limit_bytes=120 * 1024 * 1024, flags=CFG["FLAGS"]),
    )(
        A_x.reshape(S, D),
        A_mem0.reshape(M, D),
        A_Wq.reshape(D // 2, 2, H, DH),
        A_Wk.reshape(D // 2, 2, H, DH),
        A_Wv.reshape(D // 2, 2, H, DH),
        A_Wo.reshape(H * DH, D),
        B_w1, B_w2, B_w3, B_w4,
    )
    return out.reshape(B, S, D)
```

```python
import functools

import numpy as np
import jax
import jax.numpy as jnp
from jax import lax
import jax.experimental.pallas as pl
import jax.experimental.pallas.tpu as pltpu

F32 = jnp.float32
BF16 = jnp.bfloat16
U32 = jnp.uint32
LANE = 128
EPS = 1e-5
CFG = dict(TB=128, LG=0, PVK=2, PVE=1, LA=2, WOF=2, WON=4, CH=64, ORDER='b0 a0 c0 b1 a1 c1 d0 d1',
           ORDER2='b0 b1 c0 c1 d0 d1', FLAGS=None)


def _bf(w_u32):
    return pltpu.bitcast(w_u32, BF16)


def _rows(ref, idx, start, n):
    w = ref.bitcast(U32)
    if isinstance(start, int):
        words = w[(*idx, slice(start // 2, (start + n) // 2), slice(None))]
    else:
        words = w[(*idx, pl.ds(pl.multiple_of(start // 2, 8), n // 2), slice(None))]
    return pltpu.bitcast(words, BF16)


def _ln(x):
    m = jnp.mean(x, axis=-1, keepdims=True)
    d = x - m
    v = jnp.mean(d * d, axis=-1, keepdims=True)
    return d * lax.rsqrt(v + EPS)


def _gelu(x):
    c0 = np.float32(np.sqrt(2.0 / np.pi))
    c1 = np.float32(np.sqrt(2.0 / np.pi) * 0.044715)
    t = jnp.tanh(x * (c0 + c1 * (x * x)))
    hx = 0.5 * x
    return hx + hx * t


def _cat(xs, axis):
    return xs[0] if len(xs) == 1 else jnp.concatenate(xs, axis=axis)


def _make_kernel(S, D, H, DH, M, SEG, F, TB):
    NSEG = S // SEG
    TOK = SEG - M
    P = S - NSEG * TOK
    R = SEG * TOK * -(-(P + SEG) // (SEG * TOK))
    KD = D // LANE
    KF = F // LANE
    NPAIR = H // 2
    NB = S // TB
    HALO = 16
    YB = 4
    scale = np.float32(DH ** (-0.5))
    PT = P // SEG
    LNS = NSEG // NPAIR

    def kernel(x_hbm, mem0_ref, wq_hbm, wk_hbm, wv_hbm, wo_hbm, w1_hbm, w2_hbm, w3_hbm, w4_hbm,
               out_hbm,
               wq_s, wk_s, wv_s, wo_s, w1_s, w2_s, w3_s, w4_s,
               xs, xn0, xl, rq, rk, rv, o2, ps, wacc, hs, h1s, a1, gs, ys, x1s, a3, us, ostage,
               sem_x, sem_w, sem_b, sem_o):
        wqkv = ((wq_hbm, wq_s), (wk_hbm, wk_s), (wv_hbm, wv_s))

        def x_copies(lo, n, sem):
            return [pltpu.make_async_copy(x_hbm.at[pl.ds(lo, n), j * LANE:(j + 1) * LANE],
                                          xs.at[j, pl.ds(lo, n)], sem) for j in range(KD)]

        def pair_copies(j, m, src=None):
            w_hbm, w_s = wqkv[m]
            wb = w_hbm.bitcast(U32)
            src = j if src is None else src
            return [pltpu.make_async_copy(wb.at[:, p, src, :], w_s.at[2 * j + p], sem_w.at[3 * j + m])
                    for p in range(2)]

        def col_copies(w_hbm, w_s, sem):
            wb = w_hbm.bitcast(U32)
            return [pltpu.make_async_copy(wb.at[:, pl.ds(j * LANE, LANE)], w_s.at[j], sem)
                    for j in range(w_s.shape[0])]

        x_head = x_copies(0, P, sem_x.at[0])
        XC = (S - P) // (NPAIR // 2)
        XA = 2
        x_tail_a = x_copies(P, XA * XC, sem_x.at[1])
        x_tail_b = x_copies(P + XA * XC, S - P - XA * XC, sem_x.at[2])
        wo_copies = col_copies(wo_hbm, wo_s, sem_b.at[4])
        b_groups = [col_copies(wh, ws, sem_b.at[i])
                    for i, (wh, ws) in enumerate(((w1_hbm, w1_s), (w2_hbm, w2_s), (w3_hbm, w3_s), (w4_hbm, w4_s)))]
        b_copies = [c for g in b_groups for c in g]

        NI = NPAIR // 2

        def start(cps):
            for cp in cps:
                cp.start()

        def need(i):
            return [(2 * i, 1), (2 * i, 2), (2 * i + 1, 0), (2 * i + 1, 1), (2 * i + 1, 2), (2 * i + 2, 0)]

        def group_copies(j, m):
            return pair_copies(j, m, src=0) if j == NPAIR else pair_copies(j, m)

        def need_copies(i):
            return [c for j, m in need(i) for c in group_copies(j, m)]

        LA = CFG["LA"]
        wo_first, wo_n = CFG["WOF"], CFG["WON"]
        issue = [[] for _ in range(NI)]
        for k in range(1, NI):
            if k + LA < NI:
                issue[k] += need_copies(k + LA)
            if wo_first <= k < wo_first + wo_n:
                issue[k] += wo_copies[(k - wo_first) * KD // wo_n:(k - wo_first + 1) * KD // wo_n]
        start(x_head + pair_copies(0, 0) + pair_copies(0, 1))

        for k in range(KD):
            xl[k, 0:M, :] = mem0_ref[:, k * LANE:(k + 1) * LANE]
        for cp in x_head:
            cp.wait()
        start(pair_copies(0, 2) + pair_copies(1, 0) + x_tail_a)

        def ln_rows(dst, src_row, dst_row, n):
            xf = _cat([xs[k, pl.ds(src_row, n), :] for k in range(KD)], 1).astype(F32)
            xn = _ln(xf).astype(BF16)
            for k in range(KD):
                dst[k, pl.ds(dst_row, n), :] = xn[:, k * LANE:(k + 1) * LANE]

        def ln0_body(i, c):
            r = pl.multiple_of(i * 128, 128)
            ln_rows(xn0, r, r, 128)
            return c
        lax.fori_loop(0, P // 128, ln0_body, 0)

        def untangle(j, m):
            w_s = wqkv[m][1]
            a = w_s[2 * j]
            b = w_s[2 * j + 1]
            w_s[2 * j] = (a & np.uint32(0xFFFF)) | (b << 16)
            w_s[2 * j + 1] = (a >> 16) | (b & np.uint32(0xFFFF0000))

        for cp in pair_copies(0, 0):
            cp.wait()
        untangle(0, 0)

        def pro_body(i, inline_waits):
            groups = [(cls, m) for cls in range(2) for m in range(3)]
            nxt = need(i)
            if not inline_waits:
                for jn, mn in nxt:
                    for cp in pair_copies(jn, mn, src=0):
                        cp.wait()

                @pl.when(i == XA)
                def _():
                    for cp in x_tail_b:
                        cp.wait()
                for k in range(1, NI):
                    pl.when(i == k)(functools.partial(start, issue[k]))
            else:
                n1 = need_copies(1)
                rolling = [pair_copies(1, 1) + pair_copies(1, 2), pair_copies(2, 0) + n1[0:4], n1[4:8], n1[8:12],
                           x_tail_b, [c for k in range(2, LA + 1) for c in need_copies(k)]]
            for n, (cls, m) in enumerate(groups):
                j = 2 * i + cls
                jn, mn = nxt[n]
                if inline_waits:
                    if n == 1:
                        for cp in x_tail_a:
                            cp.wait()
                    start(rolling[n])
                    for cp in pair_copies(jn, mn, src=0):
                        cp.wait()
                untangle(jn, mn)
                r_s = (rq, rk, rv)[m]
                for hh in range(2):
                    lhs = _cat([_rows(xn0, (k,), 0, P) for k in range(KD)], 1)
                    w = _bf(wqkv[m][1][2 * j + hh])
                    r_s[cls][i, hh, 0:P, :] = jnp.dot(lhs, w, preferred_element_type=F32).astype(BF16)
                if 1 <= n <= LNS:
                    for t in range(2):
                        sg = i * 2 * LNS + 2 * (n - 1) + t
                        ln_rows(xl, pl.multiple_of(P + sg * TOK, 8), pl.multiple_of(sg * SEG + M, 8), TOK)

        pro_body(0, True)

        def pro_loop(i, c):
            pro_body(i, False)
            return c
        lax.fori_loop(1, NPAIR // 2, pro_loop, 0)

        for cp in wo_copies:
            cp.wait()
        start(b_copies)

        def step(s, c):
            srow = pl.multiple_of(s * SEG, SEG)
            lhs = _cat([_rows(xl, (k,), srow, SEG) for k in range(KD)], 1)
            wr = [pl.multiple_of(lax.rem(P + s * TOK + 8 * i, R), 8) for i in range(TOK // 8)]
            rr = pl.multiple_of(lax.rem(srow, R), SEG)
            orow = []
            for i in range(SEG // 8):
                p = s * (SEG // 8) + i
                a = (p // (TOK // 8)) * SEG + M + (p % (TOK // 8)) * 8
                b = (s + PT) * SEG + 8 * i
                orow.append(pl.multiple_of(jnp.where(s < NSEG - PT, a, b), 8))
            L = 2 * (SEG + M)
            ri = lax.broadcasted_iota(jnp.int32, (L, L), 0)
            ci = lax.broadcasted_iota(jnp.int32, (L, L), 1)

            def head_of(i):
                return ((i >= SEG) & (i < 2 * SEG)) | (i >= 2 * SEG + M)
            same = head_of(ri) == head_of(ci)
            allowed = same & ((ri >= 2 * SEG) | (ci >= 2 * SEG) | ((ci & (SEG - 1)) <= (ri & (SEG - 1))))
            fill = jnp.where(same, np.float32(-1e9), np.float32(-1e30))

            def proj(w_s, r_s, h):
                j, hh = h // 2, h % 2
                ring = r_s[j % 2]
                y = jnp.dot(lhs, _bf(w_s[h]), preferred_element_type=F32)
                ring[j // 2, 0, R + hh * M:R + (hh + 1) * M, :] = y[0:M, :].astype(BF16)
                for i in range(TOK // 8):
                    ring[j // 2, hh, pl.ds(wr[i], 8), :] = y[M + 8 * i:M + 8 * i + 8, :].astype(BF16)

            def stack(r_s, j):
                ring = r_s[j % 2]
                return _cat([_rows(ring, (j // 2, 0), rr, SEG), _rows(ring, (j // 2, 1), rr, SEG),
                             _rows(ring, (j // 2, 0), R, 2 * M)], 0)

            def proj_qk(j):
                for w_s, r_s in ((wq_s, rq), (wk_s, rk)):
                    proj(w_s, r_s, 2 * j)
                    proj(w_s, r_s, 2 * j + 1)

            def proj_v(j):
                proj(wv_s, rv, 2 * j)
                proj(wv_s, rv, 2 * j + 1)

            def score(j):
                q = stack(rq, j)
                k = stack(rk, j)
                sc = lax.dot_general(q, k, (((1,), (1,)), ((), ())), preferred_element_type=F32)
                sc = jnp.where(allowed, sc * scale, fill)
                mx = jnp.max(sc, axis=-1, keepdims=True)
                e = jnp.exp(sc - mx)
                l = jnp.sum(e, axis=-1, keepdims=True)
                r = pl.reciprocal(l, approx=True)
                r = r * (2.0 - l * r)
                ps[j][...] = (e * r).astype(BF16)

            def pv(j):
                o = jnp.dot(ps[j][...], stack(rv, j), preferred_element_type=F32)
                for hh in range(2):
                    dst = o2[2 * j + hh]
                    for i in range(SEG // 8):
                        dst[pl.ds(orow[i], 8), :] = o[hh * SEG + 8 * i:hh * SEG + 8 * i + 8, :].astype(BF16)
                    dst[pl.ds(srow, M), :] = o[2 * SEG + hh * M:2 * SEG + (hh + 1) * M, :].astype(BF16)

            def wo_tile(par, j):
                pairs = range(par, NPAIR, 2)
                lo_ = _cat([_rows(o2[2 * pj + hh], (), srow, SEG) for pj in pairs for hh in range(2)], 1)
                w = _cat([wo_s[j, pj * DH:(pj + 1) * DH, :] for pj in pairs], 0)
                return jnp.dot(lo_, _bf(w), preferred_element_type=F32)

            NH = NPAIR // 2
            accs = [None] * KD

            def wo_a(j):
                wacc[j] = wo_tile(0, j)

            def wo_b(j):
                accs[j] = wacc[j] + wo_tile(1, j)
                finish(j)

            hrow = pl.multiple_of(s * TOK, 8)

            def finish(j):
                acc = accs[j]
                xl[j, pl.ds(srow + SEG, M), :] = acc[0:M, :].astype(BF16)
                hs[j, pl.ds(hrow, TOK), :] = (xs[j, pl.ds(hrow, TOK), :].astype(F32) + acc[M:SEG, :]).astype(BF16)

            main = ([(proj_qk, 2 * i) for i in range(NH)] + [(proj_qk, 2 * i + 1) for i in range(NH)]
                    + [(proj_v, 2 * i) for i in range(NH)] + [(proj_v, 2 * i + 1) for i in range(NH)]
                    + [(wo_a, j) for j in range(KD)] + [(wo_b, j) for j in range(KD)])
            extra = {}
            LG, PVK = CFG["LG"], CFG["PVK"]
            for i in range(NH):
                extra.setdefault(NH + i + LG, []).append((score, 2 * i))
                extra.setdefault(2 * NH + i + LG, []).append((score, 2 * i + 1))
                extra.setdefault(3 * NH + i // CFG["PVE"] + LG, []).append((pv, 2 * i))
                extra.setdefault(4 * NH + LG + i // PVK, []).append((pv, 2 * i + 1))
            for t, (fn, arg) in enumerate(main):
                fn(arg)
                for fn2, arg2 in extra.get(t, []):
                    fn2(arg2)
            return c
        lax.fori_loop(0, NSEG, step, 0)
        for cp in b_copies:
            cp.wait()
        zero_halo = jnp.zeros((HALO, LANE), BF16)
        for j in range(KD):
            h1s[j, 0:HALO, :] = zero_halo
            h1s[j, HALO + S:HALO + S + HALO, :] = zero_halo

        CH = CFG["CH"]

        def load_h(r, n):
            return _cat([hs[k, pl.ds(r, n), :] for k in range(KD)], 1).astype(F32)

        def put_cols(dst, row, val):
            for k in range(KD):
                dst[k, row:row + val.shape[0], :] = val[:, k * LANE:(k + 1) * LANE]

        def mix1_pre(r, q):
            y = _ln(load_h(r + q, CH))
            yr = pl.multiple_of(lax.rem(r, YB * TB) + q, CH)
            for k in range(KD):
                ys[k, pl.ds(yr, CH), :] = y[:, k * LANE:(k + 1) * LANE]
            put_cols(a1, q, _ln(y).astype(BF16))

        def mix1_dot(r, q):
            for j in range(KD):
                a = _cat([_rows(a1, (k,), q, CH) for k in range(KD)], 1)
                z = jnp.dot(a, _bf(w1_s[j]), preferred_element_type=F32)
                h1s[j, pl.ds(HALO + r + q, CH), :] = _gelu(z).astype(BF16)

        def mix1(r, q):
            mix1_pre(r, q)
            mix1_dot(r, q)

        shifts = (-1, 1, -2, 2)

        TE = 128
        TM = 2 * TB // (P // TE)
        assert TM % CH == 0

        def epi_body(i, c):
            r = pl.multiple_of(NSEG * SEG + i * TE, TE)
            t = pl.multiple_of(NSEG * TOK + i * TE, TE)
            r1 = pl.multiple_of(i * TM, TM)
            for q in range(0, TM, CH):
                mix1_pre(r1, q)
            for j in range(KD):
                lo_ = _cat([_rows(o2[h], (), r, TE) for h in range(H)], 1)
                acc = jnp.dot(lo_, _bf(wo_s[j]), preferred_element_type=F32)
                hs[j, pl.ds(t, TE), :] = (xs[j, pl.ds(t, TE), :].astype(F32) + acc).astype(BF16)
            for q in range(0, TM, CH):
                mix1_dot(r1, q)
            return c
        lax.fori_loop(0, P // TE, epi_body, 0)

        def out_copy(i, slot):
            return pltpu.make_async_copy(ostage.at[slot], out_hbm.at[pl.ds(i * TB, TB), :], sem_o.at[slot])

        def b2_body(i, with_mix1):
            r = pl.multiple_of(i * TB, TB)
            slot = lax.rem(i, 2)

            @pl.when(i >= 2)
            def _():
                out_copy(i - 2, slot).wait()

            def mix2(q):
                for j in range(KD):
                    d = shifts[j // (KD // 4)]
                    win = h1s[j, pl.ds(r + q, CH + 2 * HALO), :].astype(F32)
                    gs[j, q:q + CH, :] = win[HALO + d:HALO + d + CH, :].astype(BF16)
                yr = pl.multiple_of(lax.rem(r, YB * TB) + q, CH)
                for j in range(KD):
                    g = _cat([_rows(gs, (k,), q, CH) for k in range(KD)], 1)
                    x1s[j, q:q + CH, :] = (jnp.dot(g, _bf(w2_s[j]), preferred_element_type=F32)
                                           + ys[j, pl.ds(yr, CH), :])

            def up(q):
                put_cols(a3, q, _ln(_cat([x1s[k, q:q + CH, :] for k in range(KD)], 1)).astype(BF16))
                for f in range(KF):
                    a = _cat([_rows(a3, (k,), q, CH) for k in range(KD)], 1)
                    us[f, q:q + CH, :] = _gelu(jnp.dot(a, _bf(w3_s[f]), preferred_element_type=F32)).astype(BF16)

            def down(q):
                for j in range(KD):
                    u = _cat([_rows(us, (f,), q, CH) for f in range(KF)], 1)
                    y = jnp.dot(u, _bf(w4_s[j]), preferred_element_type=F32)
                    res = hs[j, pl.ds(r + q, CH), :].astype(F32) + x1s[j, q:q + CH, :]
                    ostage[slot, q:q + CH, j * LANE:(j + 1) * LANE] = (res + y).astype(BF16)

            r2 = pl.multiple_of((i + 2) * TB, TB)
            stage = {"a": lambda q: mix1(r2, q), "b": mix2, "c": up, "d": down}
            for name in CFG["ORDER" if with_mix1 else "ORDER2"].split():
                stage[name[0]](int(name[1:]) * CH)
            out_copy(i, slot).start()

        def b2_main(i, c):
            b2_body(i, True)
            return c

        def b2_tail(i, c):
            b2_body(i, False)
            return c
        lax.fori_loop(0, NB - 2, b2_main, 0)
        lax.fori_loop(NB - 2, NB, b2_tail, 0)
        for i in range(NB - 2, NB):
            out_copy(i, i % 2).wait()

    scratch = [
        pltpu.VMEM((H + 2, D // 2, LANE), U32),
        pltpu.VMEM((H, D // 2, LANE), U32),
        pltpu.VMEM((H, D // 2, LANE), U32),
        pltpu.VMEM((KD, H * DH // 2, LANE), U32),
        pltpu.VMEM((KD, D // 2, LANE), U32),
        pltpu.VMEM((KD, D // 2, LANE), U32),
        pltpu.VMEM((KF, D // 2, LANE), U32),
        pltpu.VMEM((KD, F // 2, LANE), U32),
        pltpu.VMEM((KD, S, LANE), BF16),
        pltpu.VMEM((KD, P, LANE), BF16),
        pltpu.VMEM((KD, (NSEG + 1) * SEG, LANE), BF16),
        [pltpu.VMEM((NPAIR // 2, 2, R + 16, LANE), BF16) for _ in range(2)],
        [pltpu.VMEM((NPAIR // 2, 2, R + 16, LANE), BF16) for _ in range(2)],
        [pltpu.VMEM((NPAIR // 2, 2, R + 16, LANE), BF16) for _ in range(2)],
        [pltpu.VMEM((NSEG * SEG + P, LANE), BF16) for _ in range(H)],
        [pltpu.VMEM((2 * (SEG + M), 2 * (SEG + M)), BF16) for _ in range(NPAIR)],
        pltpu.VMEM((KD, SEG, LANE), F32),
        pltpu.VMEM((KD, S, LANE), BF16),
        pltpu.VMEM((KD, S + 2 * HALO, LANE), BF16),
        pltpu.VMEM((KD, TB, LANE), BF16),
        pltpu.VMEM((KD, TB, LANE), BF16),
        pltpu.VMEM((KD, YB * TB, LANE), F32),
        pltpu.VMEM((KD, TB, LANE), F32),
        pltpu.VMEM((KD, TB, LANE), BF16),
        pltpu.VMEM((KF, TB, LANE), BF16),
        pltpu.VMEM((2, TB, D), BF16),
        pltpu.SemaphoreType.DMA((3,)),
        pltpu.SemaphoreType.DMA((3 * NPAIR + 1,)),
        pltpu.SemaphoreType.DMA((5,)),
        pltpu.SemaphoreType.DMA((2,)),
    ]
    return kernel, scratch


@functools.partial(jax.jit, static_argnames=("A_seg_len",))
def pallas_sequential_preLN__memory_aug_recurrent_mem_tr__mixer_s_mlp__prompt_kernel(
    A_x, A_mem0, A_Wq, A_Wk, A_Wv, A_Wo, A_seg_len, B_x, B_w1, B_w2, B_w3, B_w4,
):
    del B_x
    B, S, D = A_x.shape
    M = A_mem0.shape[1]
    H, DH = A_Wq.shape[1], A_Wq.shape[2]
    F = B_w3.shape[1]
    SEG = int(A_seg_len)
    assert B == 1 and DH == LANE and M == 8 and SEG == 32 and H % 8 == 0 and D == 4 * 2 * LANE
    kernel, scratch = _make_kernel(S, D, H, DH, M, SEG, F, TB=CFG["TB"])
    any_spec = pl.BlockSpec(memory_space=pl.ANY)
    out = pl.pallas_call(
        kernel,
        out_shape=jax.ShapeDtypeStruct((S, D), A_x.dtype),
        in_specs=[any_spec, pl.BlockSpec()] + [any_spec] * 8,
        out_specs=any_spec,
        scratch_shapes=scratch,
        compiler_params=pltpu.CompilerParams(vmem_limit_bytes=120 * 1024 * 1024, flags=CFG["FLAGS"]),
    )(
        A_x.reshape(S, D),
        A_mem0.reshape(M, D),
        A_Wq.reshape(D // 2, 2, H, DH),
        A_Wk.reshape(D // 2, 2, H, DH),
        A_Wv.reshape(D // 2, 2, H, DH),
        A_Wo.reshape(H * DH, D),
        B_w1, B_w2, B_w3, B_w4,
    )
    return out.reshape(B, S, D)
```

```python
import functools

import numpy as np
import jax
import jax.numpy as jnp
from jax import lax
import jax.experimental.pallas as pl
import jax.experimental.pallas.tpu as pltpu

F32 = jnp.float32
BF16 = jnp.bfloat16
U32 = jnp.uint32
LANE = 128
EPS = 1e-5
CFG = dict(TB=128, UN=2, SE=(14, 1), SO=(22, 2), PE=(24, 3), PO=(35, 2), LA=2, WOF=2, WON=4, CH=64, ORDER='b0 a0 c0 b1 a1 c1 d0 d1',
           ORDER2='b0 b1 c0 c1 d0 d1', FLAGS=None)


def _bf(w_u32):
    return pltpu.bitcast(w_u32, BF16)


def _rows(ref, idx, start, n):
    w = ref.bitcast(U32)
    if isinstance(start, int):
        words = w[(*idx, slice(start // 2, (start + n) // 2), slice(None))]
    else:
        words = w[(*idx, pl.ds(pl.multiple_of(start // 2, 8), n // 2), slice(None))]
    return pltpu.bitcast(words, BF16)


def _ln(x):
    m = jnp.mean(x, axis=-1, keepdims=True)
    d = x - m
    v = jnp.mean(d * d, axis=-1, keepdims=True)
    return d * lax.rsqrt(v + EPS)


def _gelu(x):
    c0 = np.float32(np.sqrt(2.0 / np.pi))
    c1 = np.float32(np.sqrt(2.0 / np.pi) * 0.044715)
    t = jnp.tanh(x * (c0 + c1 * (x * x)))
    hx = 0.5 * x
    return hx + hx * t


def _cat(xs, axis):
    return xs[0] if len(xs) == 1 else jnp.concatenate(xs, axis=axis)


def _make_kernel(S, D, H, DH, M, SEG, F, TB):
    NSEG = S // SEG
    TOK = SEG - M
    P = S - NSEG * TOK
    R = SEG * TOK * -(-(P + SEG) // (SEG * TOK))
    KD = D // LANE
    KF = F // LANE
    NPAIR = H // 2
    NB = S // TB
    HALO = 16
    YB = 4
    scale = np.float32(DH ** (-0.5))
    PT = P // SEG
    LNS = NSEG // NPAIR

    def kernel(x_hbm, mem0_ref, wq_hbm, wk_hbm, wv_hbm, wo_hbm, w1_hbm, w2_hbm, w3_hbm, w4_hbm,
               out_hbm,
               wq_s, wk_s, wv_s, wo_s, w1_s, w2_s, w3_s, w4_s,
               xs, xn0, xl, rq, rk, rv, o2, ps, wacc, hs, h1s, a1, gs, ys, x1s, a3, us, ostage,
               sem_x, sem_w, sem_b, sem_o):
        wqkv = ((wq_hbm, wq_s), (wk_hbm, wk_s), (wv_hbm, wv_s))

        def x_copies(lo, n, sem):
            return [pltpu.make_async_copy(x_hbm.at[pl.ds(lo, n), j * LANE:(j + 1) * LANE],
                                          xs.at[j, pl.ds(lo, n)], sem) for j in range(KD)]

        def pair_copies(j, m, src=None):
            w_hbm, w_s = wqkv[m]
            wb = w_hbm.bitcast(U32)
            src = j if src is None else src
            return [pltpu.make_async_copy(wb.at[:, p, src, :], w_s.at[2 * j + p], sem_w.at[3 * j + m])
                    for p in range(2)]

        def col_copies(w_hbm, w_s, sem):
            wb = w_hbm.bitcast(U32)
            return [pltpu.make_async_copy(wb.at[:, pl.ds(j * LANE, LANE)], w_s.at[j], sem)
                    for j in range(w_s.shape[0])]

        x_head = x_copies(0, P, sem_x.at[0])
        XC = (S - P) // (NPAIR // 2)
        XA = 2
        x_tail_a = x_copies(P, XA * XC, sem_x.at[1])
        x_tail_b = x_copies(P + XA * XC, S - P - XA * XC, sem_x.at[2])
        wo_copies = col_copies(wo_hbm, wo_s, sem_b.at[4])
        b_groups = [col_copies(wh, ws, sem_b.at[i])
                    for i, (wh, ws) in enumerate(((w1_hbm, w1_s), (w2_hbm, w2_s), (w3_hbm, w3_s), (w4_hbm, w4_s)))]
        b_copies = [c for g in b_groups for c in g]

        NI = NPAIR // 2

        def start(cps):
            for cp in cps:
                cp.start()

        def need(i):
            return [(2 * i, 1), (2 * i, 2), (2 * i + 1, 0), (2 * i + 1, 1), (2 * i + 1, 2), (2 * i + 2, 0)]

        def group_copies(j, m):
            return pair_copies(j, m, src=0) if j == NPAIR else pair_copies(j, m)

        def need_copies(i):
            return [c for j, m in need(i) for c in group_copies(j, m)]

        LA = CFG["LA"]
        wo_first, wo_n = CFG["WOF"], CFG["WON"]
        issue = [[] for _ in range(NI)]
        for k in range(1, NI):
            if k + LA < NI:
                issue[k] += need_copies(k + LA)
            if wo_first <= k < wo_first + wo_n:
                issue[k] += wo_copies[(k - wo_first) * KD // wo_n:(k - wo_first + 1) * KD // wo_n]
        start(x_head + pair_copies(0, 0) + pair_copies(0, 1))

        for k in range(KD):
            xl[k, 0:M, :] = mem0_ref[:, k * LANE:(k + 1) * LANE]
        for cp in x_head:
            cp.wait()
        start(pair_copies(0, 2) + pair_copies(1, 0) + x_tail_a)

        def ln_rows(dst, src_row, dst_row, n):
            xf = _cat([xs[k, pl.ds(src_row, n), :] for k in range(KD)], 1).astype(F32)
            xn = _ln(xf).astype(BF16)
            for k in range(KD):
                dst[k, pl.ds(dst_row, n), :] = xn[:, k * LANE:(k + 1) * LANE]

        def ln0_body(i, c):
            r = pl.multiple_of(i * 128, 128)
            ln_rows(xn0, r, r, 128)
            return c
        lax.fori_loop(0, P // 128, ln0_body, 0)

        def untangle(j, m):
            w_s = wqkv[m][1]
            a = w_s[2 * j]
            b = w_s[2 * j + 1]
            w_s[2 * j] = (a & np.uint32(0xFFFF)) | (b << 16)
            w_s[2 * j + 1] = (a >> 16) | (b & np.uint32(0xFFFF0000))

        for cp in pair_copies(0, 0):
            cp.wait()
        untangle(0, 0)

        def pro_body(i, inline_waits):
            groups = [(cls, m) for cls in range(2) for m in range(3)]
            nxt = need(i)
            if not inline_waits:
                for jn, mn in nxt:
                    for cp in pair_copies(jn, mn, src=0):
                        cp.wait()

                @pl.when(i == XA)
                def _():
                    for cp in x_tail_b:
                        cp.wait()
                for k in range(1, NI):
                    pl.when(i == k)(functools.partial(start, issue[k]))
            else:
                n1 = need_copies(1)
                rolling = [pair_copies(1, 1) + pair_copies(1, 2), pair_copies(2, 0) + n1[0:4], n1[4:8], n1[8:12],
                           x_tail_b, [c for k in range(2, LA + 1) for c in need_copies(k)]]
            for n, (cls, m) in enumerate(groups):
                j = 2 * i + cls
                jn, mn = nxt[n]
                if inline_waits:
                    if n == 1:
                        for cp in x_tail_a:
                            cp.wait()
                    start(rolling[n])
                    for cp in pair_copies(jn, mn, src=0):
                        cp.wait()
                untangle(jn, mn)
                r_s = (rq, rk, rv)[m]
                for hh in range(2):
                    lhs = _cat([_rows(xn0, (k,), 0, P) for k in range(KD)], 1)
                    w = _bf(wqkv[m][1][2 * j + hh])
                    r_s[cls][i, hh, 0:P, :] = jnp.dot(lhs, w, preferred_element_type=F32).astype(BF16)
                if 1 <= n <= LNS:
                    for t in range(2):
                        sg = i * 2 * LNS + 2 * (n - 1) + t
                        ln_rows(xl, pl.multiple_of(P + sg * TOK, 8), pl.multiple_of(sg * SEG + M, 8), TOK)

        pro_body(0, True)

        def pro_loop(i, c):
            pro_body(i, False)
            return c
        lax.fori_loop(1, NPAIR // 2, pro_loop, 0)

        for cp in wo_copies:
            cp.wait()
        start(b_copies)

        def step(s, c):
            srow = pl.multiple_of(s * SEG, SEG)
            lhs = _cat([_rows(xl, (k,), srow, SEG) for k in range(KD)], 1)
            wr = [pl.multiple_of(lax.rem(P + s * TOK + 8 * i, R), 8) for i in range(TOK // 8)]
            rr = pl.multiple_of(lax.rem(srow, R), SEG)
            orow = []
            for i in range(SEG // 8):
                p = s * (SEG // 8) + i
                a = (p // (TOK // 8)) * SEG + M + (p % (TOK // 8)) * 8
                b = (s + PT) * SEG + 8 * i
                orow.append(pl.multiple_of(jnp.where(s < NSEG - PT, a, b), 8))
            L = 2 * (SEG + M)
            ri = lax.broadcasted_iota(jnp.int32, (L, L), 0)
            ci = lax.broadcasted_iota(jnp.int32, (L, L), 1)

            def head_of(i):
                return ((i >= SEG) & (i < 2 * SEG)) | (i >= 2 * SEG + M)
            same = head_of(ri) == head_of(ci)
            allowed = same & ((ri >= 2 * SEG) | (ci >= 2 * SEG) | ((ci & (SEG - 1)) <= (ri & (SEG - 1))))
            fill = jnp.where(same, np.float32(-1e9), np.float32(-1e30))

            def proj(w_s, r_s, h):
                j, hh = h // 2, h % 2
                ring = r_s[j % 2]
                y = jnp.dot(lhs, _bf(w_s[h]), preferred_element_type=F32)
                ring[j // 2, 0, R + hh * M:R + (hh + 1) * M, :] = y[0:M, :].astype(BF16)
                for i in range(TOK // 8):
                    ring[j // 2, hh, pl.ds(wr[i], 8), :] = y[M + 8 * i:M + 8 * i + 8, :].astype(BF16)

            def stack(r_s, j):
                ring = r_s[j % 2]
                return _cat([_rows(ring, (j // 2, 0), rr, SEG), _rows(ring, (j // 2, 1), rr, SEG),
                             _rows(ring, (j // 2, 0), R, 2 * M)], 0)

            def proj_qk(j):
                for w_s, r_s in ((wq_s, rq), (wk_s, rk)):
                    proj(w_s, r_s, 2 * j)
                    proj(w_s, r_s, 2 * j + 1)

            def proj_v(j):
                proj(wv_s, rv, 2 * j)
                proj(wv_s, rv, 2 * j + 1)

            def score(j):
                q = stack(rq, j)
                k = stack(rk, j)
                sc = lax.dot_general(q, k, (((1,), (1,)), ((), ())), preferred_element_type=F32)
                sc = jnp.where(allowed, sc * scale, fill)
                mx = jnp.max(sc, axis=-1, keepdims=True)
                e = jnp.exp(sc - mx)
                l = jnp.sum(e, axis=-1, keepdims=True)
                r = pl.reciprocal(l, approx=True)
                r = r * (2.0 - l * r)
                ps[j][...] = (e * r).astype(BF16)

            def pv(j):
                o = jnp.dot(ps[j][...], stack(rv, j), preferred_element_type=F32)
                for hh in range(2):
                    dst = o2[2 * j + hh]
                    for i in range(SEG // 8):
                        dst[pl.ds(orow[i], 8), :] = o[hh * SEG + 8 * i:hh * SEG + 8 * i + 8, :].astype(BF16)
                    dst[pl.ds(srow, M), :] = o[2 * SEG + hh * M:2 * SEG + (hh + 1) * M, :].astype(BF16)

            def wo_tile(par, j):
                pairs = range(par, NPAIR, 2)
                lo_ = _cat([_rows(o2[2 * pj + hh], (), srow, SEG) for pj in pairs for hh in range(2)], 1)
                w = _cat([wo_s[j, pj * DH:(pj + 1) * DH, :] for pj in pairs], 0)
                return jnp.dot(lo_, _bf(w), preferred_element_type=F32)

            NH = NPAIR // 2
            accs = [None] * KD

            def wo_a(j):
                wacc[j] = wo_tile(0, j)

            def wo_b(j):
                accs[j] = wacc[j] + wo_tile(1, j)
                finish(j)

            hrow = pl.multiple_of(s * TOK, 8)

            def finish(j):
                acc = accs[j]
                xl[j, pl.ds(srow + SEG, M), :] = acc[0:M, :].astype(BF16)
                hs[j, pl.ds(hrow, TOK), :] = (xs[j, pl.ds(hrow, TOK), :].astype(F32) + acc[M:SEG, :]).astype(BF16)

            main = ([(proj_qk, 2 * i) for i in range(NH)] + [(proj_qk, 2 * i + 1) for i in range(NH)]
                    + [(proj_v, 2 * i) for i in range(NH)] + [(proj_v, 2 * i + 1) for i in range(NH)]
                    + [(wo_a, j) for j in range(KD)] + [(wo_b, j) for j in range(KD)])
            extra = {}
            for fn2, par, (off, rate) in ((score, 0, CFG["SE"]), (score, 1, CFG["SO"]),
                                          (pv, 0, CFG["PE"]), (pv, 1, CFG["PO"])):
                for i in range(NH):
                    extra.setdefault(off + int(i / rate), []).append((fn2, 2 * i + par))
            assert max(extra) < len(main)
            for t, (fn, arg) in enumerate(main):
                fn(arg)
                for fn2, arg2 in extra.get(t, []):
                    fn2(arg2)
            return c
        UN = CFG["UN"]

        def steps(i, c):
            for u in range(UN):
                step(i * UN + u, c)
            return c
        lax.fori_loop(0, NSEG // UN, steps, 0)
        for cp in b_copies:
            cp.wait()
        zero_halo = jnp.zeros((HALO, LANE), BF16)
        for j in range(KD):
            h1s[j, 0:HALO, :] = zero_halo
            h1s[j, HALO + S:HALO + S + HALO, :] = zero_halo

        CH = CFG["CH"]

        def load_h(r, n):
            return _cat([hs[k, pl.ds(r, n), :] for k in range(KD)], 1).astype(F32)

        def put_cols(dst, row, val):
            for k in range(KD):
                dst[k, row:row + val.shape[0], :] = val[:, k * LANE:(k + 1) * LANE]

        def mix1_pre(r, q):
            y = _ln(load_h(r + q, CH))
            yr = pl.multiple_of(lax.rem(r, YB * TB) + q, CH)
            for k in range(KD):
                ys[k, pl.ds(yr, CH), :] = y[:, k * LANE:(k + 1) * LANE]
            put_cols(a1, q, _ln(y).astype(BF16))

        def mix1_dot(r, q):
            for j in range(KD):
                a = _cat([_rows(a1, (k,), q, CH) for k in range(KD)], 1)
                z = jnp.dot(a, _bf(w1_s[j]), preferred_element_type=F32)
                h1s[j, pl.ds(HALO + r + q, CH), :] = _gelu(z).astype(BF16)

        def mix1(r, q):
            mix1_pre(r, q)
            mix1_dot(r, q)

        shifts = (-1, 1, -2, 2)

        TE = 128
        TM = 2 * TB // (P // TE)
        assert TM % CH == 0

        def epi_body(i, c):
            r = pl.multiple_of(NSEG * SEG + i * TE, TE)
            t = pl.multiple_of(NSEG * TOK + i * TE, TE)
            r1 = pl.multiple_of(i * TM, TM)
            for q in range(0, TM, CH):
                mix1_pre(r1, q)
            for j in range(KD):
                lo_ = _cat([_rows(o2[h], (), r, TE) for h in range(H)], 1)
                acc = jnp.dot(lo_, _bf(wo_s[j]), preferred_element_type=F32)
                hs[j, pl.ds(t, TE), :] = (xs[j, pl.ds(t, TE), :].astype(F32) + acc).astype(BF16)
            for q in range(0, TM, CH):
                mix1_dot(r1, q)
            return c
        lax.fori_loop(0, P // TE, epi_body, 0)

        def out_copy(i, slot):
            return pltpu.make_async_copy(ostage.at[slot], out_hbm.at[pl.ds(i * TB, TB), :], sem_o.at[slot])

        def b2_body(i, with_mix1):
            r = pl.multiple_of(i * TB, TB)
            slot = lax.rem(i, 2)

            @pl.when(i >= 2)
            def _():
                out_copy(i - 2, slot).wait()

            def mix2(q):
                for j in range(KD):
                    d = shifts[j // (KD // 4)]
                    win = h1s[j, pl.ds(r + q, CH + 2 * HALO), :].astype(F32)
                    gs[j, q:q + CH, :] = win[HALO + d:HALO + d + CH, :].astype(BF16)
                yr = pl.multiple_of(lax.rem(r, YB * TB) + q, CH)
                for j in range(KD):
                    g = _cat([_rows(gs, (k,), q, CH) for k in range(KD)], 1)
                    x1s[j, q:q + CH, :] = (jnp.dot(g, _bf(w2_s[j]), preferred_element_type=F32)
                                           + ys[j, pl.ds(yr, CH), :])

            def up(q):
                put_cols(a3, q, _ln(_cat([x1s[k, q:q + CH, :] for k in range(KD)], 1)).astype(BF16))
                for f in range(KF):
                    a = _cat([_rows(a3, (k,), q, CH) for k in range(KD)], 1)
                    us[f, q:q + CH, :] = _gelu(jnp.dot(a, _bf(w3_s[f]), preferred_element_type=F32)).astype(BF16)

            def down(q):
                for j in range(KD):
                    u = _cat([_rows(us, (f,), q, CH) for f in range(KF)], 1)
                    y = jnp.dot(u, _bf(w4_s[j]), preferred_element_type=F32)
                    res = hs[j, pl.ds(r + q, CH), :].astype(F32) + x1s[j, q:q + CH, :]
                    ostage[slot, q:q + CH, j * LANE:(j + 1) * LANE] = (res + y).astype(BF16)

            r2 = pl.multiple_of((i + 2) * TB, TB)
            stage = {"a": lambda q: mix1(r2, q), "b": mix2, "c": up, "d": down}
            for name in CFG["ORDER" if with_mix1 else "ORDER2"].split():
                stage[name[0]](int(name[1:]) * CH)
            out_copy(i, slot).start()

        def b2_main(i, c):
            b2_body(i, True)
            return c

        def b2_tail(i, c):
            b2_body(i, False)
            return c
        lax.fori_loop(0, NB - 2, b2_main, 0)
        lax.fori_loop(NB - 2, NB, b2_tail, 0)
        for i in range(NB - 2, NB):
            out_copy(i, i % 2).wait()

    scratch = [
        pltpu.VMEM((H + 2, D // 2, LANE), U32),
        pltpu.VMEM((H, D // 2, LANE), U32),
        pltpu.VMEM((H, D // 2, LANE), U32),
        pltpu.VMEM((KD, H * DH // 2, LANE), U32),
        pltpu.VMEM((KD, D // 2, LANE), U32),
        pltpu.VMEM((KD, D // 2, LANE), U32),
        pltpu.VMEM((KF, D // 2, LANE), U32),
        pltpu.VMEM((KD, F // 2, LANE), U32),
        pltpu.VMEM((KD, S, LANE), BF16),
        pltpu.VMEM((KD, P, LANE), BF16),
        pltpu.VMEM((KD, (NSEG + 1) * SEG, LANE), BF16),
        [pltpu.VMEM((NPAIR // 2, 2, R + 16, LANE), BF16) for _ in range(2)],
        [pltpu.VMEM((NPAIR // 2, 2, R + 16, LANE), BF16) for _ in range(2)],
        [pltpu.VMEM((NPAIR // 2, 2, R + 16, LANE), BF16) for _ in range(2)],
        [pltpu.VMEM((NSEG * SEG + P, LANE), BF16) for _ in range(H)],
        [pltpu.VMEM((2 * (SEG + M), 2 * (SEG + M)), BF16) for _ in range(NPAIR)],
        pltpu.VMEM((KD, SEG, LANE), F32),
        pltpu.VMEM((KD, S, LANE), BF16),
        pltpu.VMEM((KD, S + 2 * HALO, LANE), BF16),
        pltpu.VMEM((KD, TB, LANE), BF16),
        pltpu.VMEM((KD, TB, LANE), BF16),
        pltpu.VMEM((KD, YB * TB, LANE), F32),
        pltpu.VMEM((KD, TB, LANE), F32),
        pltpu.VMEM((KD, TB, LANE), BF16),
        pltpu.VMEM((KF, TB, LANE), BF16),
        pltpu.VMEM((2, TB, D), BF16),
        pltpu.SemaphoreType.DMA((3,)),
        pltpu.SemaphoreType.DMA((3 * NPAIR + 1,)),
        pltpu.SemaphoreType.DMA((5,)),
        pltpu.SemaphoreType.DMA((2,)),
    ]
    return kernel, scratch


@functools.partial(jax.jit, static_argnames=("A_seg_len",))
def pallas_sequential_preLN__memory_aug_recurrent_mem_tr__mixer_s_mlp__prompt_kernel(
    A_x, A_mem0, A_Wq, A_Wk, A_Wv, A_Wo, A_seg_len, B_x, B_w1, B_w2, B_w3, B_w4,
):
    del B_x
    B, S, D = A_x.shape
    M = A_mem0.shape[1]
    H, DH = A_Wq.shape[1], A_Wq.shape[2]
    F = B_w3.shape[1]
    SEG = int(A_seg_len)
    assert B == 1 and DH == LANE and M == 8 and SEG == 32 and H % 8 == 0 and D == 4 * 2 * LANE
    kernel, scratch = _make_kernel(S, D, H, DH, M, SEG, F, TB=CFG["TB"])
    any_spec = pl.BlockSpec(memory_space=pl.ANY)
    out = pl.pallas_call(
        kernel,
        out_shape=jax.ShapeDtypeStruct((S, D), A_x.dtype),
        in_specs=[any_spec, pl.BlockSpec()] + [any_spec] * 8,
        out_specs=any_spec,
        scratch_shapes=scratch,
        compiler_params=pltpu.CompilerParams(vmem_limit_bytes=120 * 1024 * 1024, flags=CFG["FLAGS"]),
    )(
        A_x.reshape(S, D),
        A_mem0.reshape(M, D),
        A_Wq.reshape(D // 2, 2, H, DH),
        A_Wk.reshape(D // 2, 2, H, DH),
        A_Wv.reshape(D // 2, 2, H, DH),
        A_Wo.reshape(H * DH, D),
        B_w1, B_w2, B_w3, B_w4,
    )
    return out.reshape(B, S, D)
```

```python
import functools

import numpy as np
import jax
import jax.numpy as jnp
from jax import lax
import jax.experimental.pallas as pl
import jax.experimental.pallas.tpu as pltpu

F32 = jnp.float32
BF16 = jnp.bfloat16
U32 = jnp.uint32
LANE = 128
EPS = 1e-5
CFG = dict(TB=128, TE=64, UN=2, SE=(14, 1), SO=(22, 2), PE=(24, 3), PO=(35, 2), LA=2, WOF=2, WON=4, CH=64, ORDER='b0 a0 c0 b1 a1 c1 d0 d1',
           ORDER2='b0 b1 c0 c1 d0 d1', FLAGS=None, DBC=True)


def _bf(w_u32):
    return pltpu.bitcast(w_u32, BF16)


def _rows(ref, idx, start, n):
    w = ref.bitcast(U32)
    if isinstance(start, int):
        words = w[(*idx, slice(start // 2, (start + n) // 2), slice(None))]
    else:
        words = w[(*idx, pl.ds(pl.multiple_of(start // 2, 8), n // 2), slice(None))]
    return pltpu.bitcast(words, BF16)


def _ln(x):
    m = jnp.mean(x, axis=-1, keepdims=True)
    d = x - m
    v = jnp.mean(d * d, axis=-1, keepdims=True)
    return d * lax.rsqrt(v + EPS)


def _gelu(x):
    c0 = np.float32(np.sqrt(2.0 / np.pi))
    c1 = np.float32(np.sqrt(2.0 / np.pi) * 0.044715)
    t = jnp.tanh(x * (c0 + c1 * (x * x)))
    hx = 0.5 * x
    return hx + hx * t


def _cat(xs, axis):
    return xs[0] if len(xs) == 1 else jnp.concatenate(xs, axis=axis)


def _make_kernel(S, D, H, DH, M, SEG, F, TB):
    NSEG = S // SEG
    TOK = SEG - M
    P = S - NSEG * TOK
    R = SEG * TOK * -(-(P + SEG) // (SEG * TOK))
    KD = D // LANE
    KF = F // LANE
    NPAIR = H // 2
    NB = S // TB
    HALO = 16
    YB = 4
    scale = np.float32(DH ** (-0.5))
    PT = P // SEG
    LNS = NSEG // NPAIR

    def kernel(x_hbm, mem0_ref, wq_hbm, wk_hbm, wv_hbm, wo_hbm, w1_hbm, w2_hbm, w3_hbm, w4_hbm,
               out_hbm,
               wq_s, wk_s, wv_s, wo_s, w1_s, w2_s, w3_s, w4_s,
               xs, xn0, xl, rq, rk, rv, o2, ps, wacc, hs, h1s, a1, gs, ys, x1s, a3, us, ostage,
               sem_x, sem_w, sem_b, sem_o):
        wqkv = ((wq_hbm, wq_s), (wk_hbm, wk_s), (wv_hbm, wv_s))

        def x_copies(lo, n, sem):
            return [pltpu.make_async_copy(x_hbm.at[pl.ds(lo, n), j * LANE:(j + 1) * LANE],
                                          xs.at[j, pl.ds(lo, n)], sem) for j in range(KD)]

        def pair_copies(j, m, src=None):
            w_hbm, w_s = wqkv[m]
            wb = w_hbm.bitcast(U32)
            src = j if src is None else src
            return [pltpu.make_async_copy(wb.at[:, p, src, :], w_s.at[2 * j + p], sem_w.at[3 * j + m])
                    for p in range(2)]

        def col_copies(w_hbm, w_s, sem):
            wb = w_hbm.bitcast(U32)
            return [pltpu.make_async_copy(wb.at[:, pl.ds(j * LANE, LANE)], w_s.at[j], sem)
                    for j in range(w_s.shape[0])]

        x_head = x_copies(0, P, sem_x.at[0])
        XC = (S - P) // (NPAIR // 2)
        XA = 2
        x_tail_a = x_copies(P, XA * XC, sem_x.at[1])
        x_tail_b = x_copies(P + XA * XC, S - P - XA * XC, sem_x.at[2])
        wo_copies = col_copies(wo_hbm, wo_s, sem_b.at[4])
        b_groups = [col_copies(wh, ws, sem_b.at[i])
                    for i, (wh, ws) in enumerate(((w1_hbm, w1_s), (w2_hbm, w2_s), (w3_hbm, w3_s), (w4_hbm, w4_s)))]
        b_copies = [c for g in b_groups for c in g]

        NI = NPAIR // 2

        def start(cps):
            for cp in cps:
                cp.start()

        def need(i):
            return [(2 * i, 1), (2 * i, 2), (2 * i + 1, 0), (2 * i + 1, 1), (2 * i + 1, 2), (2 * i + 2, 0)]

        def group_copies(j, m):
            return pair_copies(j, m, src=0) if j == NPAIR else pair_copies(j, m)

        def need_copies(i):
            return [c for j, m in need(i) for c in group_copies(j, m)]

        LA = CFG["LA"]
        WOF, WON = CFG["WOF"], CFG["WON"]
        assert WOF >= 1 and WOF + WON <= NI and KD % WON == 0 and 1 <= LA < NI
        start(x_head + pair_copies(0, 0) + pair_copies(0, 1))

        for k in range(KD):
            xl[k, 0:M, :] = mem0_ref[:, k * LANE:(k + 1) * LANE]
        for cp in x_head:
            cp.wait()
        start(pair_copies(0, 2) + pair_copies(1, 0) + x_tail_a)

        def ln_rows(dst, src_row, dst_row, n):
            xf = _cat([xs[k, pl.ds(src_row, n), :] for k in range(KD)], 1).astype(F32)
            xn = _ln(xf).astype(BF16)
            for k in range(KD):
                dst[k, pl.ds(dst_row, n), :] = xn[:, k * LANE:(k + 1) * LANE]
            return xn[n - 16:n, D - LANE:D]

        def ln0_body(i, c):
            r = pl.multiple_of(i * 128, 128)
            ln_rows(xn0, r, r, 128)
            return c
        lax.fori_loop(0, P // 128, ln0_body, 0)

        def untangle(j, m):
            w_s = wqkv[m][1]
            a = w_s[2 * j]
            b = w_s[2 * j + 1]
            w_s[2 * j] = (a & np.uint32(0xFFFF)) | (b << 16)
            w_s[2 * j + 1] = (a >> 16) | (b & np.uint32(0xFFFF0000))

        for cp in pair_copies(0, 0):
            cp.wait()
        untangle(0, 0)

        def pro_body(i, inline_waits):
            groups = [(cls, m) for cls in range(2) for m in range(3)]
            nxt = need(i)
            ties = []
            if not inline_waits:
                for jn, mn in nxt:
                    for cp in pair_copies(jn, mn, src=0):
                        cp.wait()

                @pl.when(i == XA)
                def _():
                    for cp in x_tail_b:
                        cp.wait()


                @pl.when(i + LA < NI)
                def _():
                    for j, m in need(i + LA):
                        start(pair_copies(j, m, src=lax.rem(j, NPAIR)))

                @pl.when((i >= WOF) & (i < WOF + WON))
                def _():
                    for t in range(KD // WON):
                        j = (i - WOF) * (KD // WON) + t
                        pltpu.make_async_copy(wo_hbm.bitcast(U32).at[:, pl.ds(pl.multiple_of(j * LANE, LANE), LANE)],
                                              wo_s.at[j], sem_b.at[4]).start()
            else:
                n1 = need_copies(1)
                rolling = [pair_copies(1, 1) + pair_copies(1, 2), pair_copies(2, 0) + n1[0:4], n1[4:8], n1[8:12],
                           x_tail_b, [c for k in range(2, LA + 1) for c in need_copies(k)]]
            for n, (cls, m) in enumerate(groups):
                j = 2 * i + cls
                jn, mn = nxt[n]
                if inline_waits:
                    if n == 1:
                        for cp in x_tail_a:
                            cp.wait()
                    start(rolling[n])
                    for cp in pair_copies(jn, mn, src=0):
                        cp.wait()
                untangle(jn, mn)
                r_s = (rq, rk, rv)[m]
                for hh in range(2):
                    tiles = [_rows(xn0, (k,), 0, P) for k in range(KD)]
                    if hh == 0 and ties and not inline_waits:
                        head = jnp.where(i > NPAIR, ties[0], jnp.where(i > NPAIR + 1, ties[1], tiles[0][0:16]))
                        tiles[0] = _cat([head, tiles[0][16:]], 0)
                    w = _bf(wqkv[m][1][2 * j + hh])
                    r_s[cls][i, hh, 0:P, :] = jnp.dot(_cat(tiles, 1), w, preferred_element_type=F32).astype(BF16)
                ties = []
                if 1 <= n <= LNS:
                    for t in range(2):
                        sg = i * 2 * LNS + 2 * (n - 1) + t
                        ties.append(ln_rows(xl, pl.multiple_of(P + sg * TOK, 8),
                                            pl.multiple_of(sg * SEG + M, 8), TOK))

        pro_body(0, True)

        def pro_loop(i, c):
            pro_body(i, False)
            return c
        lax.fori_loop(1, NPAIR // 2, pro_loop, 0)

        for cp in wo_copies:
            cp.wait()
        start(b_copies)

        def step(s, c):
            srow = pl.multiple_of(s * SEG, SEG)
            lhs = _cat([_rows(xl, (k,), srow, SEG) for k in range(KD)], 1)
            wr = [pl.multiple_of(lax.rem(P + s * TOK + 8 * i, R), 8) for i in range(TOK // 8)]
            rr = pl.multiple_of(lax.rem(srow, R), SEG)
            orow = []
            for i in range(SEG // 8):
                p = s * (SEG // 8) + i
                a = (p // (TOK // 8)) * SEG + M + (p % (TOK // 8)) * 8
                b = (s + PT) * SEG + 8 * i
                orow.append(pl.multiple_of(jnp.where(s < NSEG - PT, a, b), 8))
            L = 2 * (SEG + M)
            ri = lax.broadcasted_iota(jnp.int32, (L, L), 0)
            ci = lax.broadcasted_iota(jnp.int32, (L, L), 1)

            def head_of(i):
                return ((i >= SEG) & (i < 2 * SEG)) | (i >= 2 * SEG + M)
            same = head_of(ri) == head_of(ci)
            allowed = same & ((ri >= 2 * SEG) | (ci >= 2 * SEG) | ((ci & (SEG - 1)) <= (ri & (SEG - 1))))
            fill = jnp.where(same, np.float32(-1e9), np.float32(-1e30))

            def proj(w_s, r_s, h):
                j, hh = h // 2, h % 2
                ring = r_s[j % 2]
                y = jnp.dot(lhs, _bf(w_s[h]), preferred_element_type=F32)
                ring[j // 2, 0, R + hh * M:R + (hh + 1) * M, :] = y[0:M, :].astype(BF16)
                for i in range(TOK // 8):
                    ring[j // 2, hh, pl.ds(wr[i], 8), :] = y[M + 8 * i:M + 8 * i + 8, :].astype(BF16)

            def stack(r_s, j):
                ring = r_s[j % 2]
                return _cat([_rows(ring, (j // 2, 0), rr, SEG), _rows(ring, (j // 2, 1), rr, SEG),
                             _rows(ring, (j // 2, 0), R, 2 * M)], 0)

            def proj_qk(j):
                for w_s, r_s in ((wq_s, rq), (wk_s, rk)):
                    proj(w_s, r_s, 2 * j)
                    proj(w_s, r_s, 2 * j + 1)

            def proj_v(j):
                proj(wv_s, rv, 2 * j)
                proj(wv_s, rv, 2 * j + 1)

            def score(j):
                q = stack(rq, j)
                k = stack(rk, j)
                sc = lax.dot_general(q, k, (((1,), (1,)), ((), ())), preferred_element_type=F32)
                sc = jnp.where(allowed, sc * scale, fill)
                mx = jnp.max(sc, axis=-1, keepdims=True)
                e = jnp.exp(sc - mx)
                l = jnp.sum(e, axis=-1, keepdims=True)
                r = pl.reciprocal(l, approx=True)
                r = r * (2.0 - l * r)
                ps[j][...] = (e * r).astype(BF16)

            def pv(j):
                o = jnp.dot(ps[j][...], stack(rv, j), preferred_element_type=F32)
                for hh in range(2):
                    dst = o2[2 * j + hh]
                    for i in range(SEG // 8):
                        dst[pl.ds(orow[i], 8), :] = o[hh * SEG + 8 * i:hh * SEG + 8 * i + 8, :].astype(BF16)
                    dst[pl.ds(srow, M), :] = o[2 * SEG + hh * M:2 * SEG + (hh + 1) * M, :].astype(BF16)

            def wo_tile(par, j):
                pairs = range(par, NPAIR, 2)
                lo_ = _cat([_rows(o2[2 * pj + hh], (), srow, SEG) for pj in pairs for hh in range(2)], 1)
                w = _cat([wo_s[j, pj * DH:(pj + 1) * DH, :] for pj in pairs], 0)
                return jnp.dot(lo_, _bf(w), preferred_element_type=F32)

            NH = NPAIR // 2
            accs = [None] * KD

            def wo_a(j):
                wacc[j] = wo_tile(0, j)

            def wo_b(j):
                accs[j] = wacc[j] + wo_tile(1, j)
                finish(j)

            hrow = pl.multiple_of(s * TOK, 8)

            def finish(j):
                acc = accs[j]
                xl[j, pl.ds(srow + SEG, M), :] = acc[0:M, :].astype(BF16)
                hs[j, pl.ds(hrow, TOK), :] = (xs[j, pl.ds(hrow, TOK), :].astype(F32) + acc[M:SEG, :]).astype(BF16)

            main = ([(proj_qk, 2 * i) for i in range(NH)] + [(proj_qk, 2 * i + 1) for i in range(NH)]
                    + [(proj_v, 2 * i) for i in range(NH)] + [(proj_v, 2 * i + 1) for i in range(NH)]
                    + [(wo_a, j) for j in range(KD)] + [(wo_b, j) for j in range(KD)])
            extra = {}
            for fn2, par, (off, rate) in ((score, 0, CFG["SE"]), (score, 1, CFG["SO"]),
                                          (pv, 0, CFG["PE"]), (pv, 1, CFG["PO"])):
                for i in range(NH):
                    extra.setdefault(off + int(i / rate), []).append((fn2, 2 * i + par))
            assert max(extra) < len(main)
            for t, (fn, arg) in enumerate(main):
                fn(arg)
                for fn2, arg2 in extra.get(t, []):
                    fn2(arg2)
            return c
        UN = CFG["UN"]

        def steps(i, c):
            for u in range(UN):
                step(i * UN + u, c)
            return c
        lax.fori_loop(0, NSEG // UN, steps, 0)
        for cp in b_copies:
            cp.wait()
        zero_halo = jnp.zeros((HALO, LANE), BF16)
        for j in range(KD):
            h1s[j, 0:HALO, :] = zero_halo
            h1s[j, HALO + S:HALO + S + HALO, :] = zero_halo

        CH = CFG["CH"]

        def load_h(r, n):
            return _cat([hs[k, pl.ds(r, n), :] for k in range(KD)], 1).astype(F32)

        def put_cols(dst, row, val):
            for k in range(KD):
                dst[k, row:row + val.shape[0], :] = val[:, k * LANE:(k + 1) * LANE]

        def mix1_pre(r, q, n=CH):
            y = _ln(load_h(r + q, n))
            yr = pl.multiple_of(lax.rem(r, YB * TB) + q, n)
            for k in range(KD):
                ys[k, pl.ds(yr, n), :] = y[:, k * LANE:(k + 1) * LANE]
            put_cols(a1, q, _ln(y).astype(BF16))

        def mix1_dot(r, q, n=CH):
            for j in range(KD):
                a = _cat([_rows(a1, (k,), q, n) for k in range(KD)], 1)
                z = jnp.dot(a, _bf(w1_s[j]), preferred_element_type=F32)
                h1s[j, pl.ds(HALO + r + q, n), :] = _gelu(z).astype(BF16)

        def mix1(r, q):
            mix1_pre(r, q)
            mix1_dot(r, q)

        shifts = (-1, 1, -2, 2)

        TE = CFG["TE"]
        TM = 2 * TB // (P // TE)
        assert TM % CH == 0 or CH % TM == 0
        CM = min(CH, TM)

        def epi_body(i, c):
            r = pl.multiple_of(NSEG * SEG + i * TE, TE)
            t = pl.multiple_of(NSEG * TOK + i * TE, TE)
            r1 = pl.multiple_of(i * TM, TM)
            for q in range(0, TM, CM):
                mix1_pre(r1, q, CM)
            for j in range(KD):
                lo_ = _cat([_rows(o2[h], (), r, TE) for h in range(H)], 1)
                acc = jnp.dot(lo_, _bf(wo_s[j]), preferred_element_type=F32)
                hs[j, pl.ds(t, TE), :] = (xs[j, pl.ds(t, TE), :].astype(F32) + acc).astype(BF16)
            for q in range(0, TM, CM):
                mix1_dot(r1, q, CM)
            return c
        lax.fori_loop(0, P // TE, epi_body, 0)

        def out_copy(i, slot):
            return pltpu.make_async_copy(ostage.at[slot], out_hbm.at[pl.ds(i * TB, TB), :], sem_o.at[slot])

        def b2_body(i, with_mix1):
            r = pl.multiple_of(i * TB, TB)
            slot = lax.rem(i, 2)

            @pl.when(i >= 2)
            def _():
                out_copy(i - 2, slot).wait()

            def mix2(q):
                for j in range(KD):
                    d = shifts[j // (KD // 4)]
                    win = h1s[j, pl.ds(r + q, CH + 2 * HALO), :].astype(F32)
                    gs[j, q:q + CH, :] = win[HALO + d:HALO + d + CH, :].astype(BF16)
                yr = pl.multiple_of(lax.rem(r, YB * TB) + q, CH)
                for j in range(KD):
                    g = _cat([_rows(gs, (k,), q, CH) for k in range(KD)], 1)
                    x1s[j, q:q + CH, :] = (jnp.dot(g, _bf(w2_s[j]), preferred_element_type=F32)
                                           + ys[j, pl.ds(yr, CH), :])

            def up(q):
                put_cols(a3, q, _ln(_cat([x1s[k, q:q + CH, :] for k in range(KD)], 1)).astype(BF16))
                for f in range(KF):
                    a = _cat([_rows(a3, (k,), q, CH) for k in range(KD)], 1)
                    us[f, q:q + CH, :] = _gelu(jnp.dot(a, _bf(w3_s[f]), preferred_element_type=F32)).astype(BF16)

            def down(q):
                for j in range(KD):
                    u = _cat([_rows(us, (f,), q, CH) for f in range(KF)], 1)
                    y = jnp.dot(u, _bf(w4_s[j]), preferred_element_type=F32)
                    res = hs[j, pl.ds(r + q, CH), :].astype(F32) + x1s[j, q:q + CH, :]
                    ostage[slot, q:q + CH, j * LANE:(j + 1) * LANE] = (res + y).astype(BF16)

            r2 = pl.multiple_of((i + 2) * TB, TB)
            stage = {"a": lambda q: mix1(r2, q), "b": mix2, "c": up, "d": down}
            for name in CFG["ORDER" if with_mix1 else "ORDER2"].split():
                stage[name[0]](int(name[1:]) * CH)
            out_copy(i, slot).start()

        def b2_main(i, c):
            b2_body(i, True)
            return c

        def b2_tail(i, c):
            b2_body(i, False)
            return c
        lax.fori_loop(0, NB - 2, b2_main, 0)
        lax.fori_loop(NB - 2, NB, b2_tail, 0)
        for i in range(NB - 2, NB):
            out_copy(i, i % 2).wait()

    scratch = [
        pltpu.VMEM((H + 2, D // 2, LANE), U32),
        pltpu.VMEM((H, D // 2, LANE), U32),
        pltpu.VMEM((H, D // 2, LANE), U32),
        pltpu.VMEM((KD, H * DH // 2, LANE), U32),
        pltpu.VMEM((KD, D // 2, LANE), U32),
        pltpu.VMEM((KD, D // 2, LANE), U32),
        pltpu.VMEM((KF, D // 2, LANE), U32),
        pltpu.VMEM((KD, F // 2, LANE), U32),
        pltpu.VMEM((KD, S, LANE), BF16),
        pltpu.VMEM((KD, P, LANE), BF16),
        pltpu.VMEM((KD, (NSEG + 1) * SEG, LANE), BF16),
        [pltpu.VMEM((NPAIR // 2, 2, R + 16, LANE), BF16) for _ in range(2)],
        [pltpu.VMEM((NPAIR // 2, 2, R + 16, LANE), BF16) for _ in range(2)],
        [pltpu.VMEM((NPAIR // 2, 2, R + 16, LANE), BF16) for _ in range(2)],
        [pltpu.VMEM((NSEG * SEG + P, LANE), BF16) for _ in range(H)],
        [pltpu.VMEM((2 * (SEG + M), 2 * (SEG + M)), BF16) for _ in range(NPAIR)],
        pltpu.VMEM((KD, SEG, LANE), F32),
        pltpu.VMEM((KD, S, LANE), BF16),
        pltpu.VMEM((KD, S + 2 * HALO, LANE), BF16),
        pltpu.VMEM((KD, TB, LANE), BF16),
        pltpu.VMEM((KD, TB, LANE), BF16),
        pltpu.VMEM((KD, YB * TB, LANE), F32),
        pltpu.VMEM((KD, TB, LANE), F32),
        pltpu.VMEM((KD, TB, LANE), BF16),
        pltpu.VMEM((KF, TB, LANE), BF16),
        pltpu.VMEM((2, TB, D), BF16),
        pltpu.SemaphoreType.DMA((3,)),
        pltpu.SemaphoreType.DMA((3 * NPAIR + 1,)),
        pltpu.SemaphoreType.DMA((5,)),
        pltpu.SemaphoreType.DMA((2,)),
    ]
    return kernel, scratch


@functools.partial(jax.jit, static_argnames=("A_seg_len",))
def pallas_sequential_preLN__memory_aug_recurrent_mem_tr__mixer_s_mlp__prompt_kernel(
    A_x, A_mem0, A_Wq, A_Wk, A_Wv, A_Wo, A_seg_len, B_x, B_w1, B_w2, B_w3, B_w4,
):
    del B_x
    B, S, D = A_x.shape
    M = A_mem0.shape[1]
    H, DH = A_Wq.shape[1], A_Wq.shape[2]
    F = B_w3.shape[1]
    SEG = int(A_seg_len)
    assert B == 1 and DH == LANE and M == 8 and SEG == 32 and H % 8 == 0 and D == 4 * 2 * LANE
    kernel, scratch = _make_kernel(S, D, H, DH, M, SEG, F, TB=CFG["TB"])
    any_spec = pl.BlockSpec(memory_space=pl.ANY)
    out = pl.pallas_call(
        kernel,
        out_shape=jax.ShapeDtypeStruct((S, D), A_x.dtype),
        in_specs=[any_spec, pl.BlockSpec()] + [any_spec] * 8,
        out_specs=any_spec,
        scratch_shapes=scratch,
        compiler_params=pltpu.CompilerParams(vmem_limit_bytes=120 * 1024 * 1024, flags=CFG["FLAGS"],
                                             disable_bounds_checks=CFG["DBC"]),
    )(
        A_x.reshape(S, D),
        A_mem0.reshape(M, D),
        A_Wq.reshape(D // 2, 2, H, DH),
        A_Wk.reshape(D // 2, 2, H, DH),
        A_Wv.reshape(D // 2, 2, H, DH),
        A_Wo.reshape(H * DH, D),
        B_w1, B_w2, B_w3, B_w4,
    )
    return out.reshape(B, S, D)
```

```python
import functools

import numpy as np
import jax
import jax.numpy as jnp
from jax import lax
import jax.experimental.pallas as pl
import jax.experimental.pallas.tpu as pltpu

F32 = jnp.float32
BF16 = jnp.bfloat16
U32 = jnp.uint32
LANE = 128
EPS = 1e-5
CFG = dict(TB=128, TE=64, UN=2, SE=(13, 4), SO=(19, 4), PE=(25, 4), PO=(35, 4), LA=2, WOF=2, WON=4, CH=64, ORDER='b0 a0 c0 b1 a1 c1 d0 d1',
           ORDER2='b0 b1 c0 c1 d0 d1', FLAGS=None, DBC=True)


def _bf(w_u32):
    return pltpu.bitcast(w_u32, BF16)


def _rows(ref, idx, start, n, align=16):
    w = ref.bitcast(U32)
    if isinstance(start, int):
        words = w[(*idx, slice(start // 2, (start + n) // 2), slice(None))]
    else:
        words = w[(*idx, pl.ds(pl.multiple_of(start // 2, align // 2), n // 2), slice(None))]
    return pltpu.bitcast(words, BF16)


def _ln(x):
    m = jnp.mean(x, axis=-1, keepdims=True)
    d = x - m
    v = jnp.mean(d * d, axis=-1, keepdims=True)
    return d * lax.rsqrt(v + EPS)


def _gelu(x):
    c0 = np.float32(np.sqrt(2.0 / np.pi))
    c1 = np.float32(np.sqrt(2.0 / np.pi) * 0.044715)
    t = jnp.tanh(x * (c0 + c1 * (x * x)))
    hx = 0.5 * x
    return hx + hx * t


def _cat(xs, axis):
    return xs[0] if len(xs) == 1 else jnp.concatenate(xs, axis=axis)


def _make_kernel(S, D, H, DH, M, SEG, F, TB):
    NSEG = S // SEG
    TOK = SEG - M
    P = S - NSEG * TOK
    R = SEG * TOK * -(-(P + SEG) // (SEG * TOK))
    KD = D // LANE
    KF = F // LANE
    NPAIR = H // 2
    NB = S // TB
    HALO = 16
    YB = 4
    scale = np.float32(DH ** (-0.5))
    PT = P // SEG
    LNS = NSEG // NPAIR

    def kernel(x_hbm, mem0_ref, wq_hbm, wk_hbm, wv_hbm, wo_hbm, w1_hbm, w2_hbm, w3_hbm, w4_hbm,
               out_hbm,
               wq_s, wk_s, wv_s, wo_s, w1_s, w2_s, w3_s, w4_s,
               xs, xn0, xl, rq, rk, rv, o2, ps, wacc, hs, h1s, a1, gs, ys, x1s, a3, us, ostage,
               sem_x, sem_w, sem_b, sem_o):
        wqkv = ((wq_hbm, wq_s), (wk_hbm, wk_s), (wv_hbm, wv_s))

        def x_copies(lo, n, sem):
            return [pltpu.make_async_copy(x_hbm.at[pl.ds(lo, n), j * LANE:(j + 1) * LANE],
                                          xs.at[j, pl.ds(lo, n)], sem) for j in range(KD)]

        def pair_copies(j, m, src=None):
            w_hbm, w_s = wqkv[m]
            wb = w_hbm.bitcast(U32)
            src = j if src is None else src
            return [pltpu.make_async_copy(wb.at[:, p, src, :], w_s.at[2 * j + p], sem_w.at[3 * j + m])
                    for p in range(2)]

        def col_copies(w_hbm, w_s, sem):
            wb = w_hbm.bitcast(U32)
            return [pltpu.make_async_copy(wb.at[:, pl.ds(j * LANE, LANE)], w_s.at[j], sem)
                    for j in range(w_s.shape[0])]

        x_head = x_copies(0, P, sem_x.at[0])
        XC = (S - P) // (NPAIR // 2)
        XA = 2
        x_tail_a = x_copies(P, XA * XC, sem_x.at[1])
        x_tail_b = x_copies(P + XA * XC, S - P - XA * XC, sem_x.at[2])
        wo_copies = col_copies(wo_hbm, wo_s, sem_b.at[4])
        b_groups = [col_copies(wh, ws, sem_b.at[i])
                    for i, (wh, ws) in enumerate(((w1_hbm, w1_s), (w2_hbm, w2_s), (w3_hbm, w3_s), (w4_hbm, w4_s)))]
        b_copies = [c for g in b_groups for c in g]

        NI = NPAIR // 2

        def start(cps):
            for cp in cps:
                cp.start()

        def need(i):
            return [(2 * i, 1), (2 * i, 2), (2 * i + 1, 0), (2 * i + 1, 1), (2 * i + 1, 2), (2 * i + 2, 0)]

        def group_copies(j, m):
            return pair_copies(j, m, src=0) if j == NPAIR else pair_copies(j, m)

        def need_copies(i):
            return [c for j, m in need(i) for c in group_copies(j, m)]

        LA = CFG["LA"]
        WOF, WON = CFG["WOF"], CFG["WON"]
        assert WOF >= 1 and WOF + WON <= NI and KD % WON == 0 and 1 <= LA < NI
        start(x_head + pair_copies(0, 0) + pair_copies(0, 1))

        for k in range(KD):
            xl[0, k, 0:M, :] = mem0_ref[:, k * LANE:(k + 1) * LANE]
        for cp in x_head:
            cp.wait()
        start(pair_copies(0, 2) + pair_copies(1, 0) + x_tail_a)

        def ln_rows(store, src_row, n):
            xf = _cat([xs[k, pl.ds(src_row, n), :] for k in range(KD)], 1).astype(F32)
            xn = _ln(xf).astype(BF16)
            for k in range(KD):
                store(k, xn[:, k * LANE:(k + 1) * LANE])
            return xn[n - 16:n, D - LANE:D]

        def ln0_body(i, c):
            r = pl.multiple_of(i * 128, 128)

            def store(k, v):
                xn0[k, pl.ds(r, 128), :] = v
            ln_rows(store, r, 128)
            return c
        lax.fori_loop(0, P // 128, ln0_body, 0)

        def untangle(j, m):
            w_s = wqkv[m][1]
            a = w_s[2 * j]
            b = w_s[2 * j + 1]
            w_s[2 * j] = (a & np.uint32(0xFFFF)) | (b << 16)
            w_s[2 * j + 1] = (a >> 16) | (b & np.uint32(0xFFFF0000))

        for cp in pair_copies(0, 0):
            cp.wait()
        untangle(0, 0)

        def pro_body(i, inline_waits):
            groups = [(cls, m) for cls in range(2) for m in range(3)]
            nxt = need(i)
            ties = []
            if not inline_waits:
                for jn, mn in nxt:
                    for cp in pair_copies(jn, mn, src=0):
                        cp.wait()

                @pl.when(i == XA)
                def _():
                    for cp in x_tail_b:
                        cp.wait()


                @pl.when(i + LA < NI)
                def _():
                    for j, m in need(i + LA):
                        start(pair_copies(j, m, src=lax.rem(j, NPAIR)))

                @pl.when((i >= WOF) & (i < WOF + WON))
                def _():
                    for t in range(KD // WON):
                        j = (i - WOF) * (KD // WON) + t
                        pltpu.make_async_copy(wo_hbm.bitcast(U32).at[:, pl.ds(pl.multiple_of(j * LANE, LANE), LANE)],
                                              wo_s.at[j], sem_b.at[4]).start()
            else:
                n1 = need_copies(1)
                rolling = [pair_copies(1, 1) + pair_copies(1, 2), pair_copies(2, 0) + n1[0:4], n1[4:8], n1[8:12],
                           x_tail_b, [c for k in range(2, LA + 1) for c in need_copies(k)]]
            for n, (cls, m) in enumerate(groups):
                j = 2 * i + cls
                jn, mn = nxt[n]
                if inline_waits:
                    if n == 1:
                        for cp in x_tail_a:
                            cp.wait()
                    start(rolling[n])
                    for cp in pair_copies(jn, mn, src=0):
                        cp.wait()
                untangle(jn, mn)
                r_s = (rq, rk, rv)[m]
                for hh in range(2):
                    tiles = [_rows(xn0, (k,), 0, P) for k in range(KD)]
                    if hh == 0 and ties and not inline_waits:
                        head = jnp.where(i > NPAIR, ties[0], jnp.where(i > NPAIR + 1, ties[1], tiles[0][0:16]))
                        tiles[0] = _cat([head, tiles[0][16:]], 0)
                    w = _bf(wqkv[m][1][2 * j + hh])
                    r_s[cls][i, hh, 0:P, :] = jnp.dot(_cat(tiles, 1), w, preferred_element_type=F32).astype(BF16)
                ties = []
                if 1 <= n <= LNS:
                    for t in range(2):
                        sg = i * 2 * LNS + 2 * (n - 1) + t

                        def store(k, v, sg=sg):
                            xl[sg, k, M:SEG, :] = v
                        ties.append(ln_rows(store, pl.multiple_of(P + sg * TOK, 8), TOK))

        pro_body(0, True)

        def pro_loop(i, c):
            pro_body(i, False)
            return c
        lax.fori_loop(1, NPAIR // 2, pro_loop, 0)

        for cp in wo_copies:
            cp.wait()
        start(b_copies)

        def step(s, c):
            srow = pl.multiple_of(s * SEG, SEG)
            lhs = _cat([_rows(xl, (s, k), 0, SEG) for k in range(KD)], 1)
            wr = [pl.multiple_of(lax.rem(P + s * TOK + 8 * i, R), 8) for i in range(TOK // 8)]
            rr = pl.multiple_of(lax.rem(srow, R), SEG)
            oblk, orow = [], []
            for i in range(SEG // 8):
                p = s * (SEG // 8) + i
                oblk.append(jnp.where(s < NSEG - PT, p // (TOK // 8), s + PT))
                orow.append(pl.multiple_of(jnp.where(s < NSEG - PT, M + (p % (TOK // 8)) * 8, 8 * i), 8))
            L = 2 * (SEG + M)
            ri = lax.broadcasted_iota(jnp.int32, (L, L), 0)
            ci = lax.broadcasted_iota(jnp.int32, (L, L), 1)

            def head_of(i):
                return ((i >= SEG) & (i < 2 * SEG)) | (i >= 2 * SEG + M)
            same = head_of(ri) == head_of(ci)
            allowed = same & ((ri >= 2 * SEG) | (ci >= 2 * SEG) | ((ci & (SEG - 1)) <= (ri & (SEG - 1))))
            fill = jnp.where(same, np.float32(-1e9), np.float32(-1e30))

            def proj(w_s, r_s, h):
                j, hh = h // 2, h % 2
                ring = r_s[j % 2]
                y = jnp.dot(lhs, _bf(w_s[h]), preferred_element_type=F32)
                ring[j // 2, 0, R + hh * M:R + (hh + 1) * M, :] = y[0:M, :].astype(BF16)
                for i in range(TOK // 8):
                    ring[j // 2, hh, pl.ds(wr[i], 8), :] = y[M + 8 * i:M + 8 * i + 8, :].astype(BF16)

            def stack(r_s, j):
                ring = r_s[j % 2]
                return _cat([_rows(ring, (j // 2, 0), rr, SEG, SEG), _rows(ring, (j // 2, 1), rr, SEG, SEG),
                             _rows(ring, (j // 2, 0), R, 2 * M)], 0)

            def proj_qk(j):
                for w_s, r_s in ((wq_s, rq), (wk_s, rk)):
                    proj(w_s, r_s, 2 * j)
                    proj(w_s, r_s, 2 * j + 1)

            def proj_v(j):
                proj(wv_s, rv, 2 * j)
                proj(wv_s, rv, 2 * j + 1)

            def score(j):
                q = stack(rq, j)
                k = stack(rk, j)
                sc = lax.dot_general(q, k, (((1,), (1,)), ((), ())), preferred_element_type=F32)
                sc = jnp.where(allowed, sc * scale, fill)
                mx = jnp.max(sc, axis=-1, keepdims=True)
                e = jnp.exp(sc - mx)
                l = jnp.sum(e, axis=-1, keepdims=True)
                r = pl.reciprocal(l, approx=True)
                r = r * (2.0 - l * r)
                ps[j][...] = (e * r).astype(BF16)

            def pv(j):
                o = jnp.dot(ps[j][...], stack(rv, j), preferred_element_type=F32)
                for hh in range(2):
                    dst, slot = o2[j % 2], (j // 2) * 2 + hh
                    for i in range(SEG // 8):
                        dst[oblk[i], slot, pl.ds(orow[i], 8), :] = (
                            o[hh * SEG + 8 * i:hh * SEG + 8 * i + 8, :].astype(BF16))
                    dst[s, slot, 0:M, :] = o[2 * SEG + hh * M:2 * SEG + (hh + 1) * M, :].astype(BF16)

            def wo_tile(par, j):
                pairs = range(par, NPAIR, 2)
                lo_ = _cat([_rows(o2[par], (s, slot), 0, SEG) for slot in range(NPAIR)], 1)
                w = _cat([wo_s[j, pj * DH:(pj + 1) * DH, :] for pj in pairs], 0)
                return jnp.dot(lo_, _bf(w), preferred_element_type=F32)

            NH = NPAIR // 2
            accs = [None] * KD

            def wo_a(j):
                wacc[j] = wo_tile(0, j)

            def wo_b(j):
                accs[j] = wacc[j] + wo_tile(1, j)
                finish(j)

            hrow = pl.multiple_of(s * TOK, 8)
            snext = jnp.minimum(s + 1, NSEG)

            def finish(j):
                acc = accs[j]
                xl[snext, j, 0:M, :] = acc[0:M, :].astype(BF16)
                hs[j, pl.ds(hrow, TOK), :] = (xs[j, pl.ds(hrow, TOK), :].astype(F32) + acc[M:SEG, :]).astype(BF16)

            main = ([(proj_qk, 2 * i) for i in range(NH)] + [(proj_qk, 2 * i + 1) for i in range(NH)]
                    + [(proj_v, 2 * i) for i in range(NH)] + [(proj_v, 2 * i + 1) for i in range(NH)]
                    + [(wo_a, j) for j in range(KD)] + [(wo_b, j) for j in range(KD)])
            extra = {}
            for fn2, par, (off, rate) in ((score, 0, CFG["SE"]), (score, 1, CFG["SO"]),
                                          (pv, 0, CFG["PE"]), (pv, 1, CFG["PO"])):
                for i in range(NH):
                    extra.setdefault(off + int(i / rate), []).append((fn2, 2 * i + par))
            assert max(extra) < len(main)
            for t, (fn, arg) in enumerate(main):
                fn(arg)
                for fn2, arg2 in extra.get(t, []):
                    fn2(arg2)
            return c
        UN = CFG["UN"]

        def steps(i, c):
            for u in range(UN):
                step(i * UN + u, c)
            return c
        lax.fori_loop(0, NSEG // UN, steps, 0)
        for cp in b_copies:
            cp.wait()
        zero_halo = jnp.zeros((HALO, LANE), BF16)
        for j in range(KD):
            h1s[j, 0:HALO, :] = zero_halo
            h1s[j, HALO + S:HALO + S + HALO, :] = zero_halo

        CH = CFG["CH"]

        def load_h(r, n):
            return _cat([hs[k, pl.ds(r, n), :] for k in range(KD)], 1).astype(F32)

        def put_cols(dst, row, val):
            for k in range(KD):
                dst[k, row:row + val.shape[0], :] = val[:, k * LANE:(k + 1) * LANE]

        def mix1_pre(r, q, n=CH):
            y = _ln(load_h(r + q, n))
            yr = pl.multiple_of(lax.rem(r, YB * TB) + q, n)
            for k in range(KD):
                ys[k, pl.ds(yr, n), :] = y[:, k * LANE:(k + 1) * LANE]
            put_cols(a1, q, _ln(y).astype(BF16))

        def mix1_dot(r, q, n=CH):
            for j in range(KD):
                a = _cat([_rows(a1, (k,), q, n) for k in range(KD)], 1)
                z = jnp.dot(a, _bf(w1_s[j]), preferred_element_type=F32)
                h1s[j, pl.ds(HALO + r + q, n), :] = _gelu(z).astype(BF16)

        def mix1(r, q):
            mix1_pre(r, q)
            mix1_dot(r, q)

        shifts = (-1, 1, -2, 2)

        TE = CFG["TE"]
        TM = 2 * TB // (P // TE)
        assert TM % CH == 0 or CH % TM == 0
        CM = min(CH, TM)

        def epi_body(i, c):
            blk = NSEG + i * (TE // SEG)
            t = pl.multiple_of(NSEG * TOK + i * TE, TE)
            r1 = pl.multiple_of(i * TM, TM)
            for q in range(0, TM, CM):
                mix1_pre(r1, q, CM)
            for j in range(KD):
                lo_ = _cat([_cat([_rows(o2[(h // 2) % 2], (blk + b, (h // 4) * 2 + h % 2), 0, SEG)
                                  for b in range(TE // SEG)], 0) for h in range(H)], 1)
                acc = jnp.dot(lo_, _bf(wo_s[j]), preferred_element_type=F32)
                hs[j, pl.ds(t, TE), :] = (xs[j, pl.ds(t, TE), :].astype(F32) + acc).astype(BF16)
            for q in range(0, TM, CM):
                mix1_dot(r1, q, CM)
            return c
        lax.fori_loop(0, P // TE, epi_body, 0)

        def out_copy(i, slot):
            return pltpu.make_async_copy(ostage.at[slot], out_hbm.at[pl.ds(i * TB, TB), :], sem_o.at[slot])

        def b2_body(i, with_mix1):
            r = pl.multiple_of(i * TB, TB)
            slot = lax.rem(i, 2)

            @pl.when(i >= 2)
            def _():
                out_copy(i - 2, slot).wait()

            def mix2(q):
                for j in range(KD):
                    d = shifts[j // (KD // 4)]
                    win = h1s[j, pl.ds(r + q, CH + 2 * HALO), :].astype(F32)
                    gs[j, q:q + CH, :] = win[HALO + d:HALO + d + CH, :].astype(BF16)
                yr = pl.multiple_of(lax.rem(r, YB * TB) + q, CH)
                for j in range(KD):
                    g = _cat([_rows(gs, (k,), q, CH) for k in range(KD)], 1)
                    x1s[j, q:q + CH, :] = (jnp.dot(g, _bf(w2_s[j]), preferred_element_type=F32)
                                           + ys[j, pl.ds(yr, CH), :])

            def up(q):
                put_cols(a3, q, _ln(_cat([x1s[k, q:q + CH, :] for k in range(KD)], 1)).astype(BF16))
                for f in range(KF):
                    a = _cat([_rows(a3, (k,), q, CH) for k in range(KD)], 1)
                    us[f, q:q + CH, :] = _gelu(jnp.dot(a, _bf(w3_s[f]), preferred_element_type=F32)).astype(BF16)

            def down(q):
                for j in range(KD):
                    u = _cat([_rows(us, (f,), q, CH) for f in range(KF)], 1)
                    y = jnp.dot(u, _bf(w4_s[j]), preferred_element_type=F32)
                    res = hs[j, pl.ds(r + q, CH), :].astype(F32) + x1s[j, q:q + CH, :]
                    ostage[slot, q:q + CH, j * LANE:(j + 1) * LANE] = (res + y).astype(BF16)

            r2 = pl.multiple_of((i + 2) * TB, TB)
            stage = {"a": lambda q: mix1(r2, q), "b": mix2, "c": up, "d": down}
            for name in CFG["ORDER" if with_mix1 else "ORDER2"].split():
                stage[name[0]](int(name[1:]) * CH)
            out_copy(i, slot).start()

        def b2_main(i, c):
            b2_body(i, True)
            return c

        def b2_tail(i, c):
            b2_body(i, False)
            return c
        lax.fori_loop(0, NB - 2, b2_main, 0)
        lax.fori_loop(NB - 2, NB, b2_tail, 0)
        for i in range(NB - 2, NB):
            out_copy(i, i % 2).wait()

    scratch = [
        pltpu.VMEM((H + 2, D // 2, LANE), U32),
        pltpu.VMEM((H, D // 2, LANE), U32),
        pltpu.VMEM((H, D // 2, LANE), U32),
        pltpu.VMEM((KD, H * DH // 2, LANE), U32),
        pltpu.VMEM((KD, D // 2, LANE), U32),
        pltpu.VMEM((KD, D // 2, LANE), U32),
        pltpu.VMEM((KF, D // 2, LANE), U32),
        pltpu.VMEM((KD, F // 2, LANE), U32),
        pltpu.VMEM((KD, S, LANE), BF16),
        pltpu.VMEM((KD, P, LANE), BF16),
        pltpu.VMEM((NSEG + 1, KD, SEG, LANE), BF16),
        [pltpu.VMEM((NPAIR // 2, 2, R + 16, LANE), BF16) for _ in range(2)],
        [pltpu.VMEM((NPAIR // 2, 2, R + 16, LANE), BF16) for _ in range(2)],
        [pltpu.VMEM((NPAIR // 2, 2, R + 16, LANE), BF16) for _ in range(2)],
        [pltpu.VMEM((NSEG + PT, NPAIR, SEG, LANE), BF16) for _ in range(2)],
        [pltpu.VMEM((2 * (SEG + M), 2 * (SEG + M)), BF16) for _ in range(NPAIR)],
        pltpu.VMEM((KD, SEG, LANE), F32),
        pltpu.VMEM((KD, S, LANE), BF16),
        pltpu.VMEM((KD, S + 2 * HALO, LANE), BF16),
        pltpu.VMEM((KD, TB, LANE), BF16),
        pltpu.VMEM((KD, TB, LANE), BF16),
        pltpu.VMEM((KD, YB * TB, LANE), F32),
        pltpu.VMEM((KD, TB, LANE), F32),
        pltpu.VMEM((KD, TB, LANE), BF16),
        pltpu.VMEM((KF, TB, LANE), BF16),
        pltpu.VMEM((2, TB, D), BF16),
        pltpu.SemaphoreType.DMA((3,)),
        pltpu.SemaphoreType.DMA((3 * NPAIR + 1,)),
        pltpu.SemaphoreType.DMA((5,)),
        pltpu.SemaphoreType.DMA((2,)),
    ]
    return kernel, scratch


@functools.partial(jax.jit, static_argnames=("A_seg_len",))
def pallas_sequential_preLN__memory_aug_recurrent_mem_tr__mixer_s_mlp__prompt_kernel(
    A_x, A_mem0, A_Wq, A_Wk, A_Wv, A_Wo, A_seg_len, B_x, B_w1, B_w2, B_w3, B_w4,
):
    del B_x
    B, S, D = A_x.shape
    M = A_mem0.shape[1]
    H, DH = A_Wq.shape[1], A_Wq.shape[2]
    F = B_w3.shape[1]
    SEG = int(A_seg_len)
    assert B == 1 and DH == LANE and M == 8 and SEG == 32 and H % 8 == 0 and D == 4 * 2 * LANE
    kernel, scratch = _make_kernel(S, D, H, DH, M, SEG, F, TB=CFG["TB"])
    any_spec = pl.BlockSpec(memory_space=pl.ANY)
    out = pl.pallas_call(
        kernel,
        out_shape=jax.ShapeDtypeStruct((S, D), A_x.dtype),
        in_specs=[any_spec, pl.BlockSpec()] + [any_spec] * 8,
        out_specs=any_spec,
        scratch_shapes=scratch,
        compiler_params=pltpu.CompilerParams(vmem_limit_bytes=120 * 1024 * 1024, flags=CFG["FLAGS"],
                                             disable_bounds_checks=CFG["DBC"]),
    )(
        A_x.reshape(S, D),
        A_mem0.reshape(M, D),
        A_Wq.reshape(D // 2, 2, H, DH),
        A_Wk.reshape(D // 2, 2, H, DH),
        A_Wv.reshape(D // 2, 2, H, DH),
        A_Wo.reshape(H * DH, D),
        B_w1, B_w2, B_w3, B_w4,
    )
    return out.reshape(B, S, D)
```

```python
import functools

import numpy as np
import jax
import jax.numpy as jnp
from jax import lax
import jax.experimental.pallas as pl
import jax.experimental.pallas.tpu as pltpu

F32 = jnp.float32
BF16 = jnp.bfloat16
U32 = jnp.uint32
LANE = 128
EPS = 1e-5
CFG = dict(TB=256, TT=128, TE=64, UN=2, SE=(13, 4), SO=(19, 4), PE=(25, 4), PO=(35, 4), LA=2, WOF=2, WON=4, CH=64, ORDER='b0 a0 c0 b1 a1 c1 d0 b2 a2 c2 d1 b3 a3 c3 d2 d3',
           ORDER2='b0 b1 c0 c1 d0 d1', FLAGS=None, DBC=True)


def _bf(w_u32):
    return pltpu.bitcast(w_u32, BF16)


def _rows(ref, idx, start, n, align=16):
    w = ref.bitcast(U32)
    if isinstance(start, int):
        words = w[(*idx, slice(start // 2, (start + n) // 2), slice(None))]
    else:
        words = w[(*idx, pl.ds(pl.multiple_of(start // 2, align // 2), n // 2), slice(None))]
    return pltpu.bitcast(words, BF16)


def _ln(x):
    m = jnp.mean(x, axis=-1, keepdims=True)
    d = x - m
    v = jnp.mean(d * d, axis=-1, keepdims=True)
    return d * lax.rsqrt(v + EPS)


def _gelu(x):
    c0 = np.float32(np.sqrt(2.0 / np.pi))
    c1 = np.float32(np.sqrt(2.0 / np.pi) * 0.044715)
    t = jnp.tanh(x * (c0 + c1 * (x * x)))
    hx = 0.5 * x
    return hx + hx * t


def _cat(xs, axis):
    return xs[0] if len(xs) == 1 else jnp.concatenate(xs, axis=axis)


def _make_kernel(S, D, H, DH, M, SEG, F, TB):
    NSEG = S // SEG
    TOK = SEG - M
    P = S - NSEG * TOK
    R = P + SEG
    KD = D // LANE
    KF = F // LANE
    NPAIR = H // 2
    NB = S // TB
    HALO = 16
    YB = 4
    scale = np.float32(DH ** (-0.5))
    PT = P // SEG
    LNS = NSEG // NPAIR

    def kernel(x_hbm, mem0_ref, wq_hbm, wk_hbm, wv_hbm, wo_hbm, w1_hbm, w2_hbm, w3_hbm, w4_hbm,
               out_hbm,
               wq_s, wk_s, wv_s, wo_s, w1_s, w2_s, w3_s, w4_s,
               xs, xn0, xl, rq, rk, rv, o2, ps, wacc, hs, h1s, a1, gs, ys, x1s, a3, us, ostage,
               sem_x, sem_w, sem_b, sem_o):
        wqkv = ((wq_hbm, wq_s), (wk_hbm, wk_s), (wv_hbm, wv_s))

        def x_copies(lo, n, sem):
            return [pltpu.make_async_copy(x_hbm.at[pl.ds(lo, n), j * LANE:(j + 1) * LANE],
                                          xs.at[j, pl.ds(lo, n)], sem) for j in range(KD)]

        def pair_copies(j, m, src=None):
            w_hbm, w_s = wqkv[m]
            wb = w_hbm.bitcast(U32)
            src = j if src is None else src
            return [pltpu.make_async_copy(wb.at[:, p, src, :], w_s.at[2 * j + p], sem_w.at[3 * j + m])
                    for p in range(2)]

        def col_copies(w_hbm, w_s, sem):
            wb = w_hbm.bitcast(U32)
            return [pltpu.make_async_copy(wb.at[:, pl.ds(j * LANE, LANE)], w_s.at[j], sem)
                    for j in range(w_s.shape[0])]

        x_head = x_copies(0, P, sem_x.at[0])
        XC = (S - P) // (NPAIR // 2)
        XA = 2
        x_tail_a = x_copies(P, XA * XC, sem_x.at[1])
        x_tail_b = x_copies(P + XA * XC, S - P - XA * XC, sem_x.at[2])
        wo_copies = col_copies(wo_hbm, wo_s, sem_b.at[4])
        b_groups = [col_copies(wh, ws, sem_b.at[i])
                    for i, (wh, ws) in enumerate(((w1_hbm, w1_s), (w2_hbm, w2_s), (w3_hbm, w3_s), (w4_hbm, w4_s)))]
        b_copies = [c for g in b_groups for c in g]

        NI = NPAIR // 2

        def start(cps):
            for cp in cps:
                cp.start()

        def need(i):
            return [(2 * i, 1), (2 * i, 2), (2 * i + 1, 0), (2 * i + 1, 1), (2 * i + 1, 2), (2 * i + 2, 0)]

        def group_copies(j, m):
            return pair_copies(j, m, src=0) if j == NPAIR else pair_copies(j, m)

        def need_copies(i):
            return [c for j, m in need(i) for c in group_copies(j, m)]

        LA = CFG["LA"]
        WOF, WON = CFG["WOF"], CFG["WON"]
        assert WOF >= 1 and WOF + WON <= NI and KD % WON == 0 and 1 <= LA < NI
        start(x_head + pair_copies(0, 0) + pair_copies(0, 1))

        for k in range(KD):
            xl[0, k, 0:M, :] = mem0_ref[:, k * LANE:(k + 1) * LANE]
        for cp in x_head:
            cp.wait()
        start(pair_copies(0, 2) + pair_copies(1, 0) + x_tail_a)

        def ln_rows(store, src_row, n):
            xf = _cat([xs[k, pl.ds(src_row, n), :] for k in range(KD)], 1).astype(F32)
            xn = _ln(xf).astype(BF16)
            for k in range(KD):
                store(k, xn[:, k * LANE:(k + 1) * LANE])
            return xn[n - 16:n, D - LANE:D]

        def ln0_body(i, c):
            r = pl.multiple_of(i * 128, 128)

            def store(k, v):
                xn0[k, pl.ds(r, 128), :] = v
            ln_rows(store, r, 128)
            return c
        lax.fori_loop(0, P // 128, ln0_body, 0)

        def untangle(j, m):
            w_s = wqkv[m][1]
            a = w_s[2 * j]
            b = w_s[2 * j + 1]
            w_s[2 * j] = (a & np.uint32(0xFFFF)) | (b << 16)
            w_s[2 * j + 1] = (a >> 16) | (b & np.uint32(0xFFFF0000))

        for cp in pair_copies(0, 0):
            cp.wait()
        untangle(0, 0)

        def pro_body(i, inline_waits):
            groups = [(cls, m) for cls in range(2) for m in range(3)]
            nxt = need(i)
            ties = []
            if not inline_waits:
                for jn, mn in nxt:
                    for cp in pair_copies(jn, mn, src=0):
                        cp.wait()

                @pl.when(i == XA)
                def _():
                    for cp in x_tail_b:
                        cp.wait()


                @pl.when(i + LA < NI)
                def _():
                    for j, m in need(i + LA):
                        start(pair_copies(j, m, src=lax.rem(j, NPAIR)))

                @pl.when((i >= WOF) & (i < WOF + WON))
                def _():
                    for t in range(KD // WON):
                        j = (i - WOF) * (KD // WON) + t
                        pltpu.make_async_copy(wo_hbm.bitcast(U32).at[:, pl.ds(pl.multiple_of(j * LANE, LANE), LANE)],
                                              wo_s.at[j], sem_b.at[4]).start()
            else:
                n1 = need_copies(1)
                rolling = [pair_copies(1, 1) + pair_copies(1, 2), pair_copies(2, 0) + n1[0:4], n1[4:8], n1[8:12],
                           x_tail_b, [c for k in range(2, LA + 1) for c in need_copies(k)]]
            for n, (cls, m) in enumerate(groups):
                j = 2 * i + cls
                jn, mn = nxt[n]
                if inline_waits:
                    if n == 1:
                        for cp in x_tail_a:
                            cp.wait()
                    start(rolling[n])
                    for cp in pair_copies(jn, mn, src=0):
                        cp.wait()
                untangle(jn, mn)
                r_s = (rq, rk, rv)[m]
                for hh in range(2):
                    tiles = [_rows(xn0, (k,), 0, P) for k in range(KD)]
                    if hh == 0 and ties and not inline_waits:
                        head = jnp.where(i > NPAIR, ties[0], jnp.where(i > NPAIR + 1, ties[1], tiles[0][0:16]))
                        tiles[0] = _cat([head, tiles[0][16:]], 0)
                    w = _bf(wqkv[m][1][2 * j + hh])
                    r_s[cls][i, hh, 0:P, :] = jnp.dot(_cat(tiles, 1), w, preferred_element_type=F32).astype(BF16)
                ties = []
                if 1 <= n <= LNS:
                    for t in range(2):
                        sg = i * 2 * LNS + 2 * (n - 1) + t

                        def store(k, v, sg=sg):
                            xl[sg, k, M:SEG, :] = v
                        ties.append(ln_rows(store, pl.multiple_of(P + sg * TOK, 8), TOK))

        pro_body(0, True)

        def pro_loop(i, c):
            pro_body(i, False)
            return c
        lax.fori_loop(1, NPAIR // 2, pro_loop, 0)

        for cp in wo_copies:
            cp.wait()
        start(b_copies)

        def step(s, c):
            srow = pl.multiple_of(s * SEG, SEG)
            lhs = _cat([_rows(xl, (s, k), 0, SEG) for k in range(KD)], 1)
            wr = [pl.multiple_of(lax.rem(P + s * TOK + 8 * i, R), 8) for i in range(TOK // 8)]
            rr = pl.multiple_of(lax.rem(srow, R), SEG)
            oblk, orow = [], []
            for i in range(SEG // 8):
                p = s * (SEG // 8) + i
                oblk.append(jnp.where(s < NSEG - PT, p // (TOK // 8), s + PT))
                orow.append(pl.multiple_of(jnp.where(s < NSEG - PT, M + (p % (TOK // 8)) * 8, 8 * i), 8))
            L = 2 * (SEG + M)
            ri = lax.broadcasted_iota(jnp.int32, (L, L), 0)
            ci = lax.broadcasted_iota(jnp.int32, (L, L), 1)

            def head_of(i):
                return ((i >= SEG) & (i < 2 * SEG)) | (i >= 2 * SEG + M)
            same = head_of(ri) == head_of(ci)
            allowed = same & ((ri >= 2 * SEG) | (ci >= 2 * SEG) | ((ci & (SEG - 1)) <= (ri & (SEG - 1))))
            fill = jnp.where(same, np.float32(-1e9), np.float32(-1e30))

            def proj(w_s, r_s, h):
                j, hh = h // 2, h % 2
                ring = r_s[j % 2]
                y = jnp.dot(lhs, _bf(w_s[h]), preferred_element_type=F32)
                ring[j // 2, 0, R + hh * M:R + (hh + 1) * M, :] = y[0:M, :].astype(BF16)
                for i in range(TOK // 8):
                    ring[j // 2, hh, pl.ds(wr[i], 8), :] = y[M + 8 * i:M + 8 * i + 8, :].astype(BF16)

            def stack(r_s, j):
                ring = r_s[j % 2]
                return _cat([_rows(ring, (j // 2, 0), rr, SEG, SEG), _rows(ring, (j // 2, 1), rr, SEG, SEG),
                             _rows(ring, (j // 2, 0), R, 2 * M)], 0)

            def proj_qk(j):
                for w_s, r_s in ((wq_s, rq), (wk_s, rk)):
                    proj(w_s, r_s, 2 * j)
                    proj(w_s, r_s, 2 * j + 1)

            def proj_v(j):
                proj(wv_s, rv, 2 * j)
                proj(wv_s, rv, 2 * j + 1)

            def score(j):
                q = stack(rq, j)
                k = stack(rk, j)
                sc = lax.dot_general(q, k, (((1,), (1,)), ((), ())), preferred_element_type=F32)
                sc = jnp.where(allowed, sc * scale, fill)
                mx = jnp.max(sc, axis=-1, keepdims=True)
                e = jnp.exp(sc - mx)
                l = jnp.sum(e, axis=-1, keepdims=True)
                r = pl.reciprocal(l, approx=True)
                r = r * (2.0 - l * r)
                ps[j][...] = (e * r).astype(BF16)

            def pv(j):
                o = jnp.dot(ps[j][...], stack(rv, j), preferred_element_type=F32)
                for hh in range(2):
                    dst, slot = o2[j % 2], (j // 2) * 2 + hh
                    for i in range(SEG // 8):
                        dst[oblk[i], slot, pl.ds(orow[i], 8), :] = (
                            o[hh * SEG + 8 * i:hh * SEG + 8 * i + 8, :].astype(BF16))
                    dst[s, slot, 0:M, :] = o[2 * SEG + hh * M:2 * SEG + (hh + 1) * M, :].astype(BF16)

            def wo_tile(par, j):
                pairs = range(par, NPAIR, 2)
                lo_ = _cat([_rows(o2[par], (s, slot), 0, SEG) for slot in range(NPAIR)], 1)
                w = _cat([wo_s[j, pj * DH:(pj + 1) * DH, :] for pj in pairs], 0)
                return jnp.dot(lo_, _bf(w), preferred_element_type=F32)

            NH = NPAIR // 2
            accs = [None] * KD

            def wo_a(j):
                wacc[j] = wo_tile(0, j)

            def wo_b(j):
                accs[j] = wacc[j] + wo_tile(1, j)
                finish(j)

            hrow = pl.multiple_of(s * TOK, 8)
            snext = jnp.minimum(s + 1, NSEG)

            def finish(j):
                acc = accs[j]
                xl[snext, j, 0:M, :] = acc[0:M, :].astype(BF16)
                hs[j, pl.ds(hrow, TOK), :] = (xs[j, pl.ds(hrow, TOK), :].astype(F32) + acc[M:SEG, :]).astype(BF16)

            main = ([(proj_qk, 2 * i) for i in range(NH)] + [(proj_qk, 2 * i + 1) for i in range(NH)]
                    + [(proj_v, 2 * i) for i in range(NH)] + [(proj_v, 2 * i + 1) for i in range(NH)]
                    + [(wo_a, j) for j in range(KD)] + [(wo_b, j) for j in range(KD)])
            extra = {}
            for fn2, par, (off, rate) in ((score, 0, CFG["SE"]), (score, 1, CFG["SO"]),
                                          (pv, 0, CFG["PE"]), (pv, 1, CFG["PO"])):
                for i in range(NH):
                    extra.setdefault(off + int(i / rate), []).append((fn2, 2 * i + par))
            assert max(extra) < len(main)
            for t, (fn, arg) in enumerate(main):
                fn(arg)
                for fn2, arg2 in extra.get(t, []):
                    fn2(arg2)
            return c
        UN = CFG["UN"]

        def steps(i, c):
            for u in range(UN):
                step(i * UN + u, c)
            return c
        lax.fori_loop(0, NSEG // UN, steps, 0)
        for cp in b_copies:
            cp.wait()
        zero_halo = jnp.zeros((HALO, LANE), BF16)
        for j in range(KD):
            h1s[j, 0:HALO, :] = zero_halo
            h1s[j, HALO + S:HALO + S + HALO, :] = zero_halo

        CH = CFG["CH"]

        def load_h(r, n):
            return _cat([hs[k, pl.ds(r, n), :] for k in range(KD)], 1).astype(F32)

        def put_cols(dst, row, val):
            for k in range(KD):
                dst[k, row:row + val.shape[0], :] = val[:, k * LANE:(k + 1) * LANE]

        def mix1_pre(r, q, n=CH):
            y = _ln(load_h(r + q, n))
            yr = pl.multiple_of(lax.rem(r, YB * TB) + q, n)
            for k in range(KD):
                ys[k, pl.ds(yr, n), :] = y[:, k * LANE:(k + 1) * LANE]
            put_cols(a1, q, _ln(y).astype(BF16))

        def mix1_dot(r, q, n=CH):
            for j in range(KD):
                a = _cat([_rows(a1, (k,), q, n) for k in range(KD)], 1)
                z = jnp.dot(a, _bf(w1_s[j]), preferred_element_type=F32)
                h1s[j, pl.ds(HALO + r + q, n), :] = _gelu(z).astype(BF16)

        def mix1(r, q):
            mix1_pre(r, q)
            mix1_dot(r, q)

        shifts = (-1, 1, -2, 2)

        TE = CFG["TE"]
        TM = 2 * TB // (P // TE)
        assert TM % CH == 0 or CH % TM == 0
        CM = min(CH, TM)

        def epi_body(i, c):
            blk = NSEG + i * (TE // SEG)
            t = pl.multiple_of(NSEG * TOK + i * TE, TE)
            r1 = pl.multiple_of(i * TM, TM)
            for q in range(0, TM, CM):
                mix1_pre(r1, q, CM)
            for j in range(KD):
                lo_ = _cat([_cat([_rows(o2[(h // 2) % 2], (blk + b, (h // 4) * 2 + h % 2), 0, SEG)
                                  for b in range(TE // SEG)], 0) for h in range(H)], 1)
                acc = jnp.dot(lo_, _bf(wo_s[j]), preferred_element_type=F32)
                hs[j, pl.ds(t, TE), :] = (xs[j, pl.ds(t, TE), :].astype(F32) + acc).astype(BF16)
            for q in range(0, TM, CM):
                mix1_dot(r1, q, CM)
            return c
        lax.fori_loop(0, P // TE, epi_body, 0)

        TT = CFG["TT"]
        NT, TBASE = 2 * TB // TT, (NB - 2) * TB

        def out_copy(r, n, slot):
            return pltpu.make_async_copy(ostage.at[slot, pl.ds(0, n)], out_hbm.at[pl.ds(r, n), :], sem_o.at[slot])

        def b2_body(i, with_mix1):
            n = TB if with_mix1 else TT
            r = pl.multiple_of(i * TB if with_mix1 else TBASE + i * TT, n)
            slot = lax.rem(i, 2)

            @pl.when(i >= 2)
            def _():
                out_copy(0, n, slot).wait()
            if not with_mix1:
                @pl.when(i < 2)
                def _():
                    out_copy(0, TB, slot).wait()

            def mix2(q):
                for j in range(KD):
                    d = shifts[j // (KD // 4)]
                    win = h1s[j, pl.ds(r + q, CH + 2 * HALO), :].astype(F32)
                    gs[j, q:q + CH, :] = win[HALO + d:HALO + d + CH, :].astype(BF16)
                yr = pl.multiple_of(lax.rem(r, YB * TB) + q, CH)
                for j in range(KD):
                    g = _cat([_rows(gs, (k,), q, CH) for k in range(KD)], 1)
                    x1s[j, q:q + CH, :] = (jnp.dot(g, _bf(w2_s[j]), preferred_element_type=F32)
                                           + ys[j, pl.ds(yr, CH), :])

            def up(q):
                put_cols(a3, q, _ln(_cat([x1s[k, q:q + CH, :] for k in range(KD)], 1)).astype(BF16))
                for f in range(KF):
                    a = _cat([_rows(a3, (k,), q, CH) for k in range(KD)], 1)
                    us[f, q:q + CH, :] = _gelu(jnp.dot(a, _bf(w3_s[f]), preferred_element_type=F32)).astype(BF16)

            def down(q):
                for j in range(KD):
                    u = _cat([_rows(us, (f,), q, CH) for f in range(KF)], 1)
                    y = jnp.dot(u, _bf(w4_s[j]), preferred_element_type=F32)
                    res = hs[j, pl.ds(r + q, CH), :].astype(F32) + x1s[j, q:q + CH, :]
                    ostage[slot, q:q + CH, j * LANE:(j + 1) * LANE] = (res + y).astype(BF16)

            r2 = pl.multiple_of((i + 2) * TB, TB)
            stage = {"a": lambda q: mix1(r2, q), "b": mix2, "c": up, "d": down}
            for name in CFG["ORDER" if with_mix1 else "ORDER2"].split():
                stage[name[0]](int(name[1:]) * CH)
            out_copy(r, n, slot).start()

        def b2_main(i, c):
            b2_body(i, True)
            return c

        def b2_tail(i, c):
            b2_body(i, False)
            return c
        lax.fori_loop(0, NB - 2, b2_main, 0)
        lax.fori_loop(0, NT, b2_tail, 0)
        for slot in range(2):
            out_copy(0, TT, slot).wait()

    scratch = [
        pltpu.VMEM((H + 2, D // 2, LANE), U32),
        pltpu.VMEM((H, D // 2, LANE), U32),
        pltpu.VMEM((H, D // 2, LANE), U32),
        pltpu.VMEM((KD, H * DH // 2, LANE), U32),
        pltpu.VMEM((KD, D // 2, LANE), U32),
        pltpu.VMEM((KD, D // 2, LANE), U32),
        pltpu.VMEM((KF, D // 2, LANE), U32),
        pltpu.VMEM((KD, F // 2, LANE), U32),
        pltpu.VMEM((KD, S, LANE), BF16),
        pltpu.VMEM((KD, P, LANE), BF16),
        pltpu.VMEM((NSEG + 1, KD, SEG, LANE), BF16),
        [pltpu.VMEM((NPAIR // 2, 2, R + 16, LANE), BF16) for _ in range(2)],
        [pltpu.VMEM((NPAIR // 2, 2, R + 16, LANE), BF16) for _ in range(2)],
        [pltpu.VMEM((NPAIR // 2, 2, R + 16, LANE), BF16) for _ in range(2)],
        [pltpu.VMEM((NSEG + PT, NPAIR, SEG, LANE), BF16) for _ in range(2)],
        [pltpu.VMEM((2 * (SEG + M), 2 * (SEG + M)), BF16) for _ in range(NPAIR)],
        pltpu.VMEM((KD, SEG, LANE), F32),
        pltpu.VMEM((KD, S, LANE), BF16),
        pltpu.VMEM((KD, S + 2 * HALO, LANE), BF16),
        pltpu.VMEM((KD, TB, LANE), BF16),
        pltpu.VMEM((KD, TB, LANE), BF16),
        pltpu.VMEM((KD, YB * TB, LANE), F32),
        pltpu.VMEM((KD, TB, LANE), F32),
        pltpu.VMEM((KD, TB, LANE), BF16),
        pltpu.VMEM((KF, TB, LANE), BF16),
        pltpu.VMEM((2, TB, D), BF16),
        pltpu.SemaphoreType.DMA((3,)),
        pltpu.SemaphoreType.DMA((3 * NPAIR + 1,)),
        pltpu.SemaphoreType.DMA((5,)),
        pltpu.SemaphoreType.DMA((2,)),
    ]
    return kernel, scratch


@functools.partial(jax.jit, static_argnames=("A_seg_len",))
def pallas_sequential_preLN__memory_aug_recurrent_mem_tr__mixer_s_mlp__prompt_kernel(
    A_x, A_mem0, A_Wq, A_Wk, A_Wv, A_Wo, A_seg_len, B_x, B_w1, B_w2, B_w3, B_w4,
):
    del B_x
    B, S, D = A_x.shape
    M = A_mem0.shape[1]
    H, DH = A_Wq.shape[1], A_Wq.shape[2]
    F = B_w3.shape[1]
    SEG = int(A_seg_len)
    assert B == 1 and DH == LANE and M == 8 and SEG == 32 and H % 8 == 0 and D == 4 * 2 * LANE
    kernel, scratch = _make_kernel(S, D, H, DH, M, SEG, F, TB=CFG["TB"])
    any_spec = pl.BlockSpec(memory_space=pl.ANY)
    out = pl.pallas_call(
        kernel,
        out_shape=jax.ShapeDtypeStruct((S, D), A_x.dtype),
        in_specs=[any_spec, pl.BlockSpec()] + [any_spec] * 8,
        out_specs=any_spec,
        scratch_shapes=scratch,
        compiler_params=pltpu.CompilerParams(vmem_limit_bytes=120 * 1024 * 1024, flags=CFG["FLAGS"],
                                             disable_bounds_checks=CFG["DBC"]),
    )(
        A_x.reshape(S, D),
        A_mem0.reshape(M, D),
        A_Wq.reshape(D // 2, 2, H, DH),
        A_Wk.reshape(D // 2, 2, H, DH),
        A_Wv.reshape(D // 2, 2, H, DH),
        A_Wo.reshape(H * DH, D),
        B_w1, B_w2, B_w3, B_w4,
    )
    return out.reshape(B, S, D)
```

```python
import functools

import numpy as np
import jax
import jax.numpy as jnp
from jax import lax
import jax.experimental.pallas as pl
import jax.experimental.pallas.tpu as pltpu

F32 = jnp.float32
BF16 = jnp.bfloat16
U32 = jnp.uint32
LANE = 128
EPS = 1e-5
CFG = dict(LN0=2, B0=2, E1=1, E2=1, E3=12, TB=256, TT=128, TE=64, UN=2, SE=(13, 4), SO=(19, 4), PE=(25, 4), PO=(35, 4), LA=2, WOF=2, WON=4, CH=64, ORDER='b0 a0 c0 b1 a1 c1 d0 b2 a2 c2 d1 b3 a3 c3 d2 d3',
           ORDER2='b0 b1 c0 c1 d0 d1', FLAGS=None, DBC=True)


def _bf(w_u32):
    return pltpu.bitcast(w_u32, BF16)


def _rows(ref, idx, start, n, align=16):
    w = ref.bitcast(U32)
    if isinstance(start, int):
        words = w[(*idx, slice(start // 2, (start + n) // 2), slice(None))]
    else:
        words = w[(*idx, pl.ds(pl.multiple_of(start // 2, align // 2), n // 2), slice(None))]
    return pltpu.bitcast(words, BF16)


def _ln(x):
    m = jnp.mean(x, axis=-1, keepdims=True)
    d = x - m
    v = jnp.mean(d * d, axis=-1, keepdims=True)
    return d * lax.rsqrt(v + EPS)


def _gelu(x):
    c0 = np.float32(np.sqrt(2.0 / np.pi))
    c1 = np.float32(np.sqrt(2.0 / np.pi) * 0.044715)
    t = jnp.tanh(x * (c0 + c1 * (x * x)))
    hx = 0.5 * x
    return hx + hx * t


def _cat(xs, axis):
    return xs[0] if len(xs) == 1 else jnp.concatenate(xs, axis=axis)


def _make_kernel(S, D, H, DH, M, SEG, F, TB):
    NSEG = S // SEG
    TOK = SEG - M
    P = S - NSEG * TOK
    R = P + SEG
    KD = D // LANE
    KF = F // LANE
    NPAIR = H // 2
    NB = S // TB
    HALO = 16
    YB = 4
    scale = np.float32(DH ** (-0.5))
    PT = P // SEG
    LNS = NSEG // NPAIR

    def kernel(zero_ref, x_hbm, mem0_ref, wq_hbm, wk_hbm, wv_hbm, wo_hbm, w1_hbm, w2_hbm, w3_hbm, w4_hbm,
               out_hbm,
               wq_s, wk_s, wv_s, wo_s, w1_s, w2_s, w3_s, w4_s,
               xs, xn0, xl, rq, rk, rv, o2, ps, wacc, hs, h1s, a1, gs, ys, x1s, a3, us, ostage,
               sem_x, sem_w, sem_b, sem_o):
        wqkv = ((wq_hbm, wq_s), (wk_hbm, wk_s), (wv_hbm, wv_s))

        def x_copies(lo, n, sem):
            return [pltpu.make_async_copy(x_hbm.at[pl.ds(lo, n), j * LANE:(j + 1) * LANE],
                                          xs.at[j, pl.ds(lo, n)], sem) for j in range(KD)]

        def pair_copies(j, m, src=None):
            w_hbm, w_s = wqkv[m]
            wb = w_hbm.bitcast(U32)
            src = j if src is None else src
            return [pltpu.make_async_copy(wb.at[:, p, src, :], w_s.at[2 * j + p], sem_w.at[3 * j + m])
                    for p in range(2)]

        def col_copies(w_hbm, w_s, sem):
            wb = w_hbm.bitcast(U32)
            return [pltpu.make_async_copy(wb.at[:, pl.ds(j * LANE, LANE)], w_s.at[j], sem)
                    for j in range(w_s.shape[0])]

        x_head = x_copies(0, P, sem_x.at[0])
        XC = (S - P) // (NPAIR // 2)
        XA = 2
        x_tail_a = x_copies(P, XA * XC, sem_x.at[1])
        x_tail_b = x_copies(P + XA * XC, S - P - XA * XC, sem_x.at[2])
        wo_copies = col_copies(wo_hbm, wo_s, sem_b.at[4])
        b_groups = [col_copies(wh, ws, sem_b.at[i])
                    for i, (wh, ws) in enumerate(((w1_hbm, w1_s), (w2_hbm, w2_s), (w3_hbm, w3_s), (w4_hbm, w4_s)))]
        b_copies = [c for g in b_groups for c in g]

        NI = NPAIR // 2

        def start(cps):
            for cp in cps:
                cp.start()

        def need(i):
            return [(2 * i, 1), (2 * i, 2), (2 * i + 1, 0), (2 * i + 1, 1), (2 * i + 1, 2), (2 * i + 2, 0)]

        def group_copies(j, m):
            return pair_copies(j, m, src=0) if j == NPAIR else pair_copies(j, m)

        def need_copies(i):
            return [c for j, m in need(i) for c in group_copies(j, m)]

        LA = CFG["LA"]
        WOF, WON = CFG["WOF"], CFG["WON"]
        assert WOF >= 1 and WOF + WON <= NI and KD % WON == 0 and 1 <= LA < NI
        B0 = CFG["B0"]
        start(x_head + [c for m in range(B0) for c in pair_copies(0, m)])

        for k in range(KD):
            xl[0, k, 0:M, :] = mem0_ref[:, k * LANE:(k + 1) * LANE]

        def wait(cps):
            for cp in cps:
                cp.wait()

        wait(x_head + pair_copies(0, 0))
        start([c for m in range(B0, 3) for c in pair_copies(0, m)] + CFG["E1"] * (pair_copies(1, 0) + x_tail_a))

        def ln_rows(store, src_row, n):
            xf = _cat([xs[k, pl.ds(src_row, n), :] for k in range(KD)], 1).astype(F32)
            xn = _ln(xf).astype(BF16)
            for k in range(KD):
                store(k, xn[:, k * LANE:(k + 1) * LANE])
            return xn[n - 16:n, D - LANE:D]

        def untangle(j, m):
            w_s = wqkv[m][1]
            a = w_s[2 * j]
            b = w_s[2 * j + 1]
            w_s[2 * j] = (a & np.uint32(0xFFFF)) | (b << 16)
            w_s[2 * j + 1] = (a >> 16) | (b & np.uint32(0xFFFF0000))

        untangle(0, 0)
        for r in range(0, P, 128):
            def store(k, v, r=r):
                xn0[k, r:r + 128, :] = v
            ln_rows(store, r, 128)
            for hh in range(2):
                lhs0 = _cat([_rows(xn0, (k,), r, 128) for k in range(KD)], 1)
                rq[0][0, hh, r:r + 128, :] = jnp.dot(lhs0, _bf(wq_s[hh]), preferred_element_type=F32).astype(BF16)

        def pro_body(i, first):
            groups = [(cls, m) for cls in range(2) for m in range(3)]
            nxt = need(i)
            ties = []
            if not first:
                for jn, mn in nxt:
                    wait(pair_copies(jn, mn, src=0))
                pl.when(i == XA)(functools.partial(wait, x_tail_b))

                @pl.when(i + LA < NI)
                def _():
                    for j, m in need(i + LA):
                        start(pair_copies(j, m, src=lax.rem(j, NPAIR)))

                @pl.when((i >= WOF) & (i < WOF + WON))
                def _():
                    for t in range(KD // WON):
                        j = (i - WOF) * (KD // WON) + t
                        pltpu.make_async_copy(wo_hbm.bitcast(U32).at[:, pl.ds(pl.multiple_of(j * LANE, LANE), LANE)],
                                              wo_s.at[j], sem_b.at[4]).start()
            ln_at = CFG["LN0"] if first else 1
            for n, (cls, m) in enumerate(groups):
                j = 2 * i + cls
                jn, mn = nxt[n]
                if first:
                    n1 = need_copies(1)
                    if n == 0:
                        wait(pair_copies(0, 1) + pair_copies(0, 2))
                        start((1 - CFG["E1"]) * (pair_copies(1, 0) + x_tail_a) + pair_copies(1, 1))
                        start(CFG["E2"] * (pair_copies(1, 2) + pair_copies(2, 0)))
                        untangle(jn, mn)
                        continue
                    if n == 2:
                        wait(pair_copies(1, 0) + pair_copies(1, 1) + x_tail_a)
                        start((1 - CFG["E2"]) * (pair_copies(1, 2) + pair_copies(2, 0)) + n1[0:CFG["E3"]])
                    if n == 4:
                        wait(pair_copies(1, 2) + pair_copies(2, 0))
                        start(n1[CFG["E3"]:] + x_tail_b + [c for k in range(2, LA + 1) for c in need_copies(k)])
                untangle(jn, mn)
                r_s = (rq, rk, rv)[m]
                for hh in range(2):
                    tiles = [_rows(xn0, (k,), 0, P) for k in range(KD)]
                    if hh == 0 and ties:
                        head = tiles[0][0:16]
                        for t, tie in enumerate(ties):
                            head = jnp.where(never > t, tie, head)
                        tiles[0] = _cat([head, tiles[0][16:]], 0)
                    w = _bf(wqkv[m][1][2 * j + hh])
                    r_s[cls][i, hh, 0:P, :] = jnp.dot(_cat(tiles, 1), w, preferred_element_type=F32).astype(BF16)
                ties = []
                if ln_at <= n < ln_at + LNS:
                    for t in range(2):
                        sg = i * 2 * LNS + 2 * (n - ln_at) + t

                        def store(k, v, sg=sg):
                            xl[sg, k, M:SEG, :] = v
                        ties.append(ln_rows(store, pl.multiple_of(P + sg * TOK, 8), TOK))

        never = zero_ref[0]
        pro_body(0, True)

        def pro_loop(i, c):
            pro_body(i, False)
            return c
        lax.fori_loop(1, NPAIR // 2, pro_loop, 0)

        for cp in wo_copies:
            cp.wait()
        start(b_copies)

        def step(s, c):
            srow = pl.multiple_of(s * SEG, SEG)
            lhs = _cat([_rows(xl, (s, k), 0, SEG) for k in range(KD)], 1)
            wr = [pl.multiple_of(lax.rem(P + s * TOK + 8 * i, R), 8) for i in range(TOK // 8)]
            rr = pl.multiple_of(lax.rem(srow, R), SEG)
            oblk, orow = [], []
            for i in range(SEG // 8):
                p = s * (SEG // 8) + i
                oblk.append(jnp.where(s < NSEG - PT, p // (TOK // 8), s + PT))
                orow.append(pl.multiple_of(jnp.where(s < NSEG - PT, M + (p % (TOK // 8)) * 8, 8 * i), 8))
            L = 2 * (SEG + M)
            ri = lax.broadcasted_iota(jnp.int32, (L, L), 0)
            ci = lax.broadcasted_iota(jnp.int32, (L, L), 1)

            def head_of(i):
                return ((i >= SEG) & (i < 2 * SEG)) | (i >= 2 * SEG + M)
            same = head_of(ri) == head_of(ci)
            allowed = same & ((ri >= 2 * SEG) | (ci >= 2 * SEG) | ((ci & (SEG - 1)) <= (ri & (SEG - 1))))
            fill = jnp.where(same, np.float32(-1e9), np.float32(-1e30))

            def proj(w_s, r_s, h):
                j, hh = h // 2, h % 2
                ring = r_s[j % 2]
                y = jnp.dot(lhs, _bf(w_s[h]), preferred_element_type=F32)
                ring[j // 2, 0, R + hh * M:R + (hh + 1) * M, :] = y[0:M, :].astype(BF16)
                for i in range(TOK // 8):
                    ring[j // 2, hh, pl.ds(wr[i], 8), :] = y[M + 8 * i:M + 8 * i + 8, :].astype(BF16)

            def stack(r_s, j):
                ring = r_s[j % 2]
                return _cat([_rows(ring, (j // 2, 0), rr, SEG, SEG), _rows(ring, (j // 2, 1), rr, SEG, SEG),
                             _rows(ring, (j // 2, 0), R, 2 * M)], 0)

            def proj_qk(j):
                for w_s, r_s in ((wq_s, rq), (wk_s, rk)):
                    proj(w_s, r_s, 2 * j)
                    proj(w_s, r_s, 2 * j + 1)

            def proj_v(j):
                proj(wv_s, rv, 2 * j)
                proj(wv_s, rv, 2 * j + 1)

            def score(j):
                q = stack(rq, j)
                k = stack(rk, j)
                sc = lax.dot_general(q, k, (((1,), (1,)), ((), ())), preferred_element_type=F32)
                sc = jnp.where(allowed, sc * scale, fill)
                mx = jnp.max(sc, axis=-1, keepdims=True)
                e = jnp.exp(sc - mx)
                l = jnp.sum(e, axis=-1, keepdims=True)
                r = pl.reciprocal(l, approx=True)
                r = r * (2.0 - l * r)
                ps[j][...] = (e * r).astype(BF16)

            def pv(j):
                o = jnp.dot(ps[j][...], stack(rv, j), preferred_element_type=F32)
                for hh in range(2):
                    dst, slot = o2[j % 2], (j // 2) * 2 + hh
                    for i in range(SEG // 8):
                        dst[oblk[i], slot, pl.ds(orow[i], 8), :] = (
                            o[hh * SEG + 8 * i:hh * SEG + 8 * i + 8, :].astype(BF16))
                    dst[s, slot, 0:M, :] = o[2 * SEG + hh * M:2 * SEG + (hh + 1) * M, :].astype(BF16)

            def wo_tile(par, j):
                pairs = range(par, NPAIR, 2)
                lo_ = _cat([_rows(o2[par], (s, slot), 0, SEG) for slot in range(NPAIR)], 1)
                w = _cat([wo_s[j, pj * DH:(pj + 1) * DH, :] for pj in pairs], 0)
                return jnp.dot(lo_, _bf(w), preferred_element_type=F32)

            NH = NPAIR // 2
            accs = [None] * KD

            def wo_a(j):
                wacc[j] = wo_tile(0, j)

            def wo_b(j):
                accs[j] = wacc[j] + wo_tile(1, j)
                finish(j)

            hrow = pl.multiple_of(s * TOK, 8)
            snext = jnp.minimum(s + 1, NSEG)

            def finish(j):
                acc = accs[j]
                xl[snext, j, 0:M, :] = acc[0:M, :].astype(BF16)
                hs[j, pl.ds(hrow, TOK), :] = (xs[j, pl.ds(hrow, TOK), :].astype(F32) + acc[M:SEG, :]).astype(BF16)

            main = ([(proj_qk, 2 * i) for i in range(NH)] + [(proj_qk, 2 * i + 1) for i in range(NH)]
                    + [(proj_v, 2 * i) for i in range(NH)] + [(proj_v, 2 * i + 1) for i in range(NH)]
                    + [(wo_a, j) for j in range(KD)] + [(wo_b, j) for j in range(KD)])
            extra = {}
            for fn2, par, (off, rate) in ((score, 0, CFG["SE"]), (score, 1, CFG["SO"]),
                                          (pv, 0, CFG["PE"]), (pv, 1, CFG["PO"])):
                for i in range(NH):
                    extra.setdefault(off + int(i / rate), []).append((fn2, 2 * i + par))
            assert max(extra) < len(main)
            for t, (fn, arg) in enumerate(main):
                fn(arg)
                for fn2, arg2 in extra.get(t, []):
                    fn2(arg2)
            return c
        UN = CFG["UN"]

        def steps(i, c):
            for u in range(UN):
                step(i * UN + u, c)
            return c
        lax.fori_loop(0, NSEG // UN, steps, 0)
        for cp in b_copies:
            cp.wait()
        zero_halo = jnp.zeros((HALO, LANE), BF16)
        for j in range(KD):
            h1s[j, 0:HALO, :] = zero_halo
            h1s[j, HALO + S:HALO + S + HALO, :] = zero_halo

        CH = CFG["CH"]

        def load_h(r, n):
            return _cat([hs[k, pl.ds(r, n), :] for k in range(KD)], 1).astype(F32)

        def put_cols(dst, row, val):
            for k in range(KD):
                dst[k, row:row + val.shape[0], :] = val[:, k * LANE:(k + 1) * LANE]

        def mix1_pre(r, q, n=CH):
            y = _ln(load_h(r + q, n))
            yr = pl.multiple_of(lax.rem(r, YB * TB) + q, n)
            for k in range(KD):
                ys[k, pl.ds(yr, n), :] = y[:, k * LANE:(k + 1) * LANE]
            put_cols(a1, q, _ln(y).astype(BF16))

        def mix1_dot(r, q, n=CH):
            for j in range(KD):
                a = _cat([_rows(a1, (k,), q, n) for k in range(KD)], 1)
                z = jnp.dot(a, _bf(w1_s[j]), preferred_element_type=F32)
                h1s[j, pl.ds(HALO + r + q, n), :] = _gelu(z).astype(BF16)

        def mix1(r, q):
            mix1_pre(r, q)
            mix1_dot(r, q)

        shifts = (-1, 1, -2, 2)

        TE = CFG["TE"]
        TM = 2 * TB // (P // TE)
        assert TM % CH == 0 or CH % TM == 0
        CM = min(CH, TM)

        def epi_body(i, c):
            blk = NSEG + i * (TE // SEG)
            t = pl.multiple_of(NSEG * TOK + i * TE, TE)
            r1 = pl.multiple_of(i * TM, TM)
            for q in range(0, TM, CM):
                mix1_pre(r1, q, CM)
            for j in range(KD):
                lo_ = _cat([_cat([_rows(o2[(h // 2) % 2], (blk + b, (h // 4) * 2 + h % 2), 0, SEG)
                                  for b in range(TE // SEG)], 0) for h in range(H)], 1)
                acc = jnp.dot(lo_, _bf(wo_s[j]), preferred_element_type=F32)
                hs[j, pl.ds(t, TE), :] = (xs[j, pl.ds(t, TE), :].astype(F32) + acc).astype(BF16)
            for q in range(0, TM, CM):
                mix1_dot(r1, q, CM)
            return c
        lax.fori_loop(0, P // TE, epi_body, 0)

        TT = CFG["TT"]
        NT, TBASE = 2 * TB // TT, (NB - 2) * TB

        def out_copy(r, n, slot):
            return pltpu.make_async_copy(ostage.at[slot, pl.ds(0, n)], out_hbm.at[pl.ds(r, n), :], sem_o.at[slot])

        def b2_body(i, with_mix1):
            n = TB if with_mix1 else TT
            r = pl.multiple_of(i * TB if with_mix1 else TBASE + i * TT, n)
            slot = lax.rem(i, 2)

            @pl.when(i >= 2)
            def _():
                out_copy(0, n, slot).wait()
            if not with_mix1:
                @pl.when(i < 2)
                def _():
                    out_copy(0, TB, slot).wait()

            def mix2(q):
                for j in range(KD):
                    d = shifts[j // (KD // 4)]
                    win = h1s[j, pl.ds(r + q, CH + 2 * HALO), :].astype(F32)
                    gs[j, q:q + CH, :] = win[HALO + d:HALO + d + CH, :].astype(BF16)
                yr = pl.multiple_of(lax.rem(r, YB * TB) + q, CH)
                for j in range(KD):
                    g = _cat([_rows(gs, (k,), q, CH) for k in range(KD)], 1)
                    x1s[j, q:q + CH, :] = (jnp.dot(g, _bf(w2_s[j]), preferred_element_type=F32)
                                           + ys[j, pl.ds(yr, CH), :])

            def up(q):
                put_cols(a3, q, _ln(_cat([x1s[k, q:q + CH, :] for k in range(KD)], 1)).astype(BF16))
                for f in range(KF):
                    a = _cat([_rows(a3, (k,), q, CH) for k in range(KD)], 1)
                    us[f, q:q + CH, :] = _gelu(jnp.dot(a, _bf(w3_s[f]), preferred_element_type=F32)).astype(BF16)

            def down(q):
                for j in range(KD):
                    u = _cat([_rows(us, (f,), q, CH) for f in range(KF)], 1)
                    y = jnp.dot(u, _bf(w4_s[j]), preferred_element_type=F32)
                    res = hs[j, pl.ds(r + q, CH), :].astype(F32) + x1s[j, q:q + CH, :]
                    ostage[slot, q:q + CH, j * LANE:(j + 1) * LANE] = (res + y).astype(BF16)

            r2 = pl.multiple_of((i + 2) * TB, TB)
            stage = {"a": lambda q: mix1(r2, q), "b": mix2, "c": up, "d": down}
            for name in CFG["ORDER" if with_mix1 else "ORDER2"].split():
                stage[name[0]](int(name[1:]) * CH)
            out_copy(r, n, slot).start()

        def b2_main(i, c):
            b2_body(i, True)
            return c

        def b2_tail(i, c):
            b2_body(i, False)
            return c
        lax.fori_loop(0, NB - 2, b2_main, 0)
        lax.fori_loop(0, NT, b2_tail, 0)
        for slot in range(2):
            out_copy(0, TT, slot).wait()

    scratch = [
        pltpu.VMEM((H + 2, D // 2, LANE), U32),
        pltpu.VMEM((H, D // 2, LANE), U32),
        pltpu.VMEM((H, D // 2, LANE), U32),
        pltpu.VMEM((KD, H * DH // 2, LANE), U32),
        pltpu.VMEM((KD, D // 2, LANE), U32),
        pltpu.VMEM((KD, D // 2, LANE), U32),
        pltpu.VMEM((KF, D // 2, LANE), U32),
        pltpu.VMEM((KD, F // 2, LANE), U32),
        pltpu.VMEM((KD, S, LANE), BF16),
        pltpu.VMEM((KD, P, LANE), BF16),
        pltpu.VMEM((NSEG + 1, KD, SEG, LANE), BF16),
        [pltpu.VMEM((NPAIR // 2, 2, R + 16, LANE), BF16) for _ in range(2)],
        [pltpu.VMEM((NPAIR // 2, 2, R + 16, LANE), BF16) for _ in range(2)],
        [pltpu.VMEM((NPAIR // 2, 2, R + 16, LANE), BF16) for _ in range(2)],
        [pltpu.VMEM((NSEG + PT, NPAIR, SEG, LANE), BF16) for _ in range(2)],
        [pltpu.VMEM((2 * (SEG + M), 2 * (SEG + M)), BF16) for _ in range(NPAIR)],
        pltpu.VMEM((KD, SEG, LANE), F32),
        pltpu.VMEM((KD, S, LANE), BF16),
        pltpu.VMEM((KD, S + 2 * HALO, LANE), BF16),
        pltpu.VMEM((KD, TB, LANE), BF16),
        pltpu.VMEM((KD, TB, LANE), BF16),
        pltpu.VMEM((KD, YB * TB, LANE), F32),
        pltpu.VMEM((KD, TB, LANE), F32),
        pltpu.VMEM((KD, TB, LANE), BF16),
        pltpu.VMEM((KF, TB, LANE), BF16),
        pltpu.VMEM((2, TB, D), BF16),
        pltpu.SemaphoreType.DMA((3,)),
        pltpu.SemaphoreType.DMA((3 * NPAIR + 1,)),
        pltpu.SemaphoreType.DMA((5,)),
        pltpu.SemaphoreType.DMA((2,)),
    ]
    return kernel, scratch


@functools.partial(jax.jit, static_argnames=("A_seg_len",))
def pallas_sequential_preLN__memory_aug_recurrent_mem_tr__mixer_s_mlp__prompt_kernel(
    A_x, A_mem0, A_Wq, A_Wk, A_Wv, A_Wo, A_seg_len, B_x, B_w1, B_w2, B_w3, B_w4,
):
    del B_x
    B, S, D = A_x.shape
    M = A_mem0.shape[1]
    H, DH = A_Wq.shape[1], A_Wq.shape[2]
    F = B_w3.shape[1]
    SEG = int(A_seg_len)
    assert B == 1 and DH == LANE and M == 8 and SEG == 32 and H % 8 == 0 and D == 4 * 2 * LANE
    kernel, scratch = _make_kernel(S, D, H, DH, M, SEG, F, TB=CFG["TB"])
    any_spec = pl.BlockSpec(memory_space=pl.ANY)
    out = pl.pallas_call(
        kernel,
        out_shape=jax.ShapeDtypeStruct((S, D), A_x.dtype),
        in_specs=[pl.BlockSpec(memory_space=pltpu.SMEM), any_spec, pl.BlockSpec()] + [any_spec] * 8,
        out_specs=any_spec,
        scratch_shapes=scratch,
        compiler_params=pltpu.CompilerParams(vmem_limit_bytes=120 * 1024 * 1024, flags=CFG["FLAGS"],
                                             disable_bounds_checks=CFG["DBC"]),
    )(
        jnp.zeros((1,), jnp.int32),
        A_x.reshape(S, D),
        A_mem0.reshape(M, D),
        A_Wq.reshape(D // 2, 2, H, DH),
        A_Wk.reshape(D // 2, 2, H, DH),
        A_Wv.reshape(D // 2, 2, H, DH),
        A_Wo.reshape(H * DH, D),
        B_w1, B_w2, B_w3, B_w4,
    )
    return out.reshape(B, S, D)
```

```python
import functools

import numpy as np
import jax
import jax.numpy as jnp
from jax import lax
import jax.experimental.pallas as pl
import jax.experimental.pallas.tpu as pltpu

F32 = jnp.float32
BF16 = jnp.bfloat16
U32 = jnp.uint32
LANE = 128
EPS = 1e-5
CFG = dict(LN0=2, B0=2, E1=1, E2=1, E3=12, TB=256, TT=128, TE=128, UN=2, SE=(13, 4), SO=(19, 4), PE=(25, 4), PO=(35, 4), LA=2, WOF=2, WON=4, CH=64, ORDER='b0 a0 c0 b1 a1 c1 d0 b2 a2 c2 d1 b3 a3 c3 d2 d3',
           ORDER2='b0 b1 c0 c1 d0 d1', FLAGS=None)


def _bf(w_u32):
    return pltpu.bitcast(w_u32, BF16)


def _rows(ref, idx, start, n, align=16):
    w = ref.bitcast(U32)
    if isinstance(start, int):
        words = w[(*idx, slice(start // 2, (start + n) // 2), slice(None))]
    else:
        words = w[(*idx, pl.ds(pl.multiple_of(start // 2, align // 2), n // 2), slice(None))]
    return pltpu.bitcast(words, BF16)


def _ln(x):
    m = jnp.mean(x, axis=-1, keepdims=True)
    d = x - m
    v = jnp.mean(d * d, axis=-1, keepdims=True)
    return d * lax.rsqrt(v + EPS)


def _gelu(x):
    c0 = np.float32(np.sqrt(2.0 / np.pi))
    c1 = np.float32(np.sqrt(2.0 / np.pi) * 0.044715)
    t = jnp.tanh(x * (c0 + c1 * (x * x)))
    hx = 0.5 * x
    return hx + hx * t


def _cat(xs, axis):
    return xs[0] if len(xs) == 1 else jnp.concatenate(xs, axis=axis)


def _make_kernel(S, D, H, DH, M, SEG, F, TB):
    NSEG = S // SEG
    TOK = SEG - M
    P = S - NSEG * TOK
    R = P + SEG
    KD = D // LANE
    KF = F // LANE
    NPAIR = H // 2
    NB = S // TB
    HALO = 16
    YB = 4
    scale = np.float32(DH ** (-0.5))
    PT = P // SEG
    LNS = NSEG // NPAIR

    def kernel(zero_ref, x_hbm, mem0_ref, wq_hbm, wk_hbm, wv_hbm, wo_hbm, w1_hbm, w2_hbm, w3_hbm, w4_hbm,
               out_hbm,
               wq_s, wk_s, wv_s, wo_s, w1_s, w2_s, w3_s, w4_s,
               xs, xn0, xl, rq, rk, rv, o2, ps, wacc, hs, h1s, a1, gs, ys, x1s, a3, us, ostage,
               sem_x, sem_w, sem_b, sem_o):
        wqkv = ((wq_hbm, wq_s), (wk_hbm, wk_s), (wv_hbm, wv_s))

        def x_copies(lo, n, sem):
            return [pltpu.make_async_copy(x_hbm.at[pl.ds(lo, n), j * LANE:(j + 1) * LANE],
                                          xs.at[j, pl.ds(lo, n)], sem) for j in range(KD)]

        def pair_copies(j, m, src=None):
            w_hbm, w_s = wqkv[m]
            wb = w_hbm.bitcast(U32)
            src = j if src is None else src
            return [pltpu.make_async_copy(wb.at[:, p, src, :], w_s.at[2 * j + p], sem_w.at[3 * j + m])
                    for p in range(2)]

        def col_copies(w_hbm, w_s, sem):
            wb = w_hbm.bitcast(U32)
            return [pltpu.make_async_copy(wb.at[:, pl.ds(j * LANE, LANE)], w_s.at[j], sem)
                    for j in range(w_s.shape[0])]

        x_head = x_copies(0, P, sem_x.at[0])
        XC = (S - P) // (NPAIR // 2)
        XA = 2
        x_tail_a = x_copies(P, XA * XC, sem_x.at[1])
        x_tail_b = x_copies(P + XA * XC, S - P - XA * XC, sem_x.at[2])
        wo_copies = functools.partial(col_copies, wo_hbm, wo_s, sem_b.at[4])
        b_groups = [col_copies(wh, ws, sem_b.at[i])
                    for i, (wh, ws) in enumerate(((w1_hbm, w1_s), (w2_hbm, w2_s), (w3_hbm, w3_s), (w4_hbm, w4_s)))]
        b_copies = [c for g in b_groups for c in g]

        NI = NPAIR // 2

        def start(cps):
            for cp in cps:
                cp.start()

        def need(i):
            return [(2 * i, 1), (2 * i, 2), (2 * i + 1, 0), (2 * i + 1, 1), (2 * i + 1, 2), (2 * i + 2, 0)]

        def group_copies(j, m):
            return pair_copies(j, m, src=0) if j == NPAIR else pair_copies(j, m)

        def need_copies(i):
            return [c for j, m in need(i) for c in group_copies(j, m)]

        LA = CFG["LA"]
        WOF, WON = CFG["WOF"], CFG["WON"]
        assert WOF >= 1 and WOF + WON <= NI and KD % WON == 0 and 1 <= LA < NI
        B0 = CFG["B0"]
        start(x_head + [c for m in range(B0) for c in pair_copies(0, m)])

        for k in range(KD):
            xl[0, k, 0:M, :] = mem0_ref[:, k * LANE:(k + 1) * LANE]

        def wait(cps):
            for cp in cps:
                cp.wait()

        wait(x_head + pair_copies(0, 0))
        start([c for m in range(B0, 3) for c in pair_copies(0, m)] + CFG["E1"] * (pair_copies(1, 0) + x_tail_a))

        def ln_rows(store, src_row, n):
            xf = _cat([xs[k, pl.ds(src_row, n), :] for k in range(KD)], 1).astype(F32)
            xn = _ln(xf).astype(BF16)
            for k in range(KD):
                store(k, xn[:, k * LANE:(k + 1) * LANE])
            return xn[n - 16:n, D - LANE:D]

        def untangle(j, m):
            w_s = wqkv[m][1]
            a = w_s[2 * j]
            b = w_s[2 * j + 1]
            w_s[2 * j] = (a & np.uint32(0xFFFF)) | (b << 16)
            w_s[2 * j + 1] = (a >> 16) | (b & np.uint32(0xFFFF0000))

        untangle(0, 0)
        for r in range(0, P, 128):
            def store(k, v, r=r):
                xn0[k, r:r + 128, :] = v
            ln_rows(store, r, 128)
            for hh in range(2):
                lhs0 = _cat([_rows(xn0, (k,), r, 128) for k in range(KD)], 1)
                rq[0][0, hh, r:r + 128, :] = jnp.dot(lhs0, _bf(wq_s[hh]), preferred_element_type=F32).astype(BF16)

        def pro_body(i, first):
            groups = [(cls, m) for cls in range(2) for m in range(3)]
            nxt = need(i)
            ties = []
            if not first:
                for jn, mn in nxt:
                    wait(pair_copies(jn, mn, src=0))
                pl.when(i == XA)(functools.partial(wait, x_tail_b))

                for k in range(1, NI):
                    late = (need_copies(k + LA) if k + LA < NI else []) + (
                        wo_copies()[(k - WOF) * KD // WON:(k - WOF + 1) * KD // WON] if WOF <= k < WOF + WON else [])
                    if late:
                        pl.when(i == k)(functools.partial(start, late))
            ln_at = CFG["LN0"] if first else 1
            for n, (cls, m) in enumerate(groups):
                j = 2 * i + cls
                jn, mn = nxt[n]
                if first:
                    n1 = need_copies(1)
                    if n == 0:
                        wait(pair_copies(0, 1) + pair_copies(0, 2))
                        start((1 - CFG["E1"]) * (pair_copies(1, 0) + x_tail_a) + pair_copies(1, 1))
                        start(CFG["E2"] * (pair_copies(1, 2) + pair_copies(2, 0)))
                        untangle(jn, mn)
                        continue
                    if n == 2:
                        wait(pair_copies(1, 0) + pair_copies(1, 1) + x_tail_a)
                        start((1 - CFG["E2"]) * (pair_copies(1, 2) + pair_copies(2, 0)) + n1[0:CFG["E3"]])
                    if n == 4:
                        wait(pair_copies(1, 2) + pair_copies(2, 0))
                        start(n1[CFG["E3"]:] + x_tail_b + [c for k in range(2, LA + 1) for c in need_copies(k)])
                untangle(jn, mn)
                r_s = (rq, rk, rv)[m]
                for hh in range(2):
                    tiles = [_rows(xn0, (k,), 0, P) for k in range(KD)]
                    if hh == 0 and ties:
                        head = tiles[0][0:16]
                        for t, tie in enumerate(ties):
                            head = jnp.where(never > t, tie, head)
                        tiles[0] = _cat([head, tiles[0][16:]], 0)
                    w = _bf(wqkv[m][1][2 * j + hh])
                    r_s[cls][i, hh, 0:P, :] = jnp.dot(_cat(tiles, 1), w, preferred_element_type=F32).astype(BF16)
                ties = []
                if ln_at <= n < ln_at + LNS:
                    for t in range(2):
                        sg = i * 2 * LNS + 2 * (n - ln_at) + t

                        def store(k, v, sg=sg):
                            xl[sg, k, M:SEG, :] = v
                        ties.append(ln_rows(store, pl.multiple_of(P + sg * TOK, 8), TOK))

        never = zero_ref[0]
        pro_body(0, True)

        def pro_loop(i, c):
            pro_body(i, False)
            return c
        lax.fori_loop(1, NPAIR // 2, pro_loop, 0)

        wait(wo_copies())
        start(b_copies)

        def step(s, c):
            srow = pl.multiple_of(s * SEG, SEG)
            lhs = _cat([_rows(xl, (s, k), 0, SEG) for k in range(KD)], 1)
            wr = [pl.multiple_of(lax.rem(P + s * TOK + 8 * i, R), 8) for i in range(TOK // 8)]
            rr = pl.multiple_of(lax.rem(srow, R), SEG)
            oblk, orow = [], []
            for i in range(SEG // 8):
                p = s * (SEG // 8) + i
                oblk.append(jnp.where(s < NSEG - PT, p // (TOK // 8), s + PT))
                orow.append(pl.multiple_of(jnp.where(s < NSEG - PT, M + (p % (TOK // 8)) * 8, 8 * i), 8))
            L = 2 * (SEG + M)
            ri = lax.broadcasted_iota(jnp.int32, (L, L), 0)
            ci = lax.broadcasted_iota(jnp.int32, (L, L), 1)

            def head_of(i):
                return ((i >= SEG) & (i < 2 * SEG)) | (i >= 2 * SEG + M)
            same = head_of(ri) == head_of(ci)
            allowed = same & ((ri >= 2 * SEG) | (ci >= 2 * SEG) | ((ci & (SEG - 1)) <= (ri & (SEG - 1))))
            fill = jnp.where(same, np.float32(-1e9), np.float32(-1e30))

            def proj(w_s, r_s, h):
                j, hh = h // 2, h % 2
                ring = r_s[j % 2]
                y = jnp.dot(lhs, _bf(w_s[h]), preferred_element_type=F32)
                ring[j // 2, 0, R + hh * M:R + (hh + 1) * M, :] = y[0:M, :].astype(BF16)
                for i in range(TOK // 8):
                    ring[j // 2, hh, pl.ds(wr[i], 8), :] = y[M + 8 * i:M + 8 * i + 8, :].astype(BF16)

            def stack(r_s, j):
                ring = r_s[j % 2]
                return _cat([_rows(ring, (j // 2, 0), rr, SEG, SEG), _rows(ring, (j // 2, 1), rr, SEG, SEG),
                             _rows(ring, (j // 2, 0), R, 2 * M)], 0)

            def proj_qk(j):
                for w_s, r_s in ((wq_s, rq), (wk_s, rk)):
                    proj(w_s, r_s, 2 * j)
                    proj(w_s, r_s, 2 * j + 1)

            def proj_v(j):
                proj(wv_s, rv, 2 * j)
                proj(wv_s, rv, 2 * j + 1)

            def score(j):
                q = stack(rq, j)
                k = stack(rk, j)
                sc = lax.dot_general(q, k, (((1,), (1,)), ((), ())), preferred_element_type=F32)
                sc = jnp.where(allowed, sc * scale, fill)
                mx = jnp.max(sc, axis=-1, keepdims=True)
                e = jnp.exp(sc - mx)
                l = jnp.sum(e, axis=-1, keepdims=True)
                r = pl.reciprocal(l, approx=True)
                r = r * (2.0 - l * r)
                ps[j][...] = (e * r).astype(BF16)

            def pv(j):
                o = jnp.dot(ps[j][...], stack(rv, j), preferred_element_type=F32)
                for hh in range(2):
                    dst, slot = o2[j % 2], (j // 2) * 2 + hh
                    for i in range(SEG // 8):
                        dst[oblk[i], slot, pl.ds(orow[i], 8), :] = (
                            o[hh * SEG + 8 * i:hh * SEG + 8 * i + 8, :].astype(BF16))
                    dst[s, slot, 0:M, :] = o[2 * SEG + hh * M:2 * SEG + (hh + 1) * M, :].astype(BF16)

            def wo_tile(par, j):
                pairs = range(par, NPAIR, 2)
                lo_ = _cat([_rows(o2[par], (s, slot), 0, SEG) for slot in range(NPAIR)], 1)
                w = _cat([wo_s[j, pj * DH:(pj + 1) * DH, :] for pj in pairs], 0)
                return jnp.dot(lo_, _bf(w), preferred_element_type=F32)

            NH = NPAIR // 2
            accs = [None] * KD

            def wo_a(j):
                wacc[j] = wo_tile(0, j)

            def wo_b(j):
                accs[j] = wacc[j] + wo_tile(1, j)
                finish(j)

            hrow = pl.multiple_of(s * TOK, 8)
            snext = jnp.minimum(s + 1, NSEG)

            def finish(j):
                acc = accs[j]
                xl[snext, j, 0:M, :] = acc[0:M, :].astype(BF16)
                hs[j, pl.ds(hrow, TOK), :] = (xs[j, pl.ds(hrow, TOK), :].astype(F32) + acc[M:SEG, :]).astype(BF16)

            main = ([(proj_qk, 2 * i) for i in range(NH)] + [(proj_qk, 2 * i + 1) for i in range(NH)]
                    + [(proj_v, 2 * i) for i in range(NH)] + [(proj_v, 2 * i + 1) for i in range(NH)]
                    + [(wo_a, j) for j in range(KD)] + [(wo_b, j) for j in range(KD)])
            extra = {}
            for fn2, par, (off, rate) in ((score, 0, CFG["SE"]), (score, 1, CFG["SO"]),
                                          (pv, 0, CFG["PE"]), (pv, 1, CFG["PO"])):
                for i in range(NH):
                    extra.setdefault(off + int(i / rate), []).append((fn2, 2 * i + par))
            assert max(extra) < len(main)
            for t, (fn, arg) in enumerate(main):
                fn(arg)
                for fn2, arg2 in extra.get(t, []):
                    fn2(arg2)
            return c
        UN = CFG["UN"]

        def steps(i, c):
            for u in range(UN):
                step(i * UN + u, c)
            return c
        lax.fori_loop(0, NSEG // UN, steps, 0)
        for cp in b_copies:
            cp.wait()
        zero_halo = jnp.zeros((HALO, LANE), BF16)
        for j in range(KD):
            h1s[j, 0:HALO, :] = zero_halo
            h1s[j, HALO + S:HALO + S + HALO, :] = zero_halo

        CH = CFG["CH"]

        def load_h(r, n):
            return _cat([hs[k, pl.ds(r, n), :] for k in range(KD)], 1).astype(F32)

        def put_cols(dst, row, val):
            for k in range(KD):
                dst[k, row:row + val.shape[0], :] = val[:, k * LANE:(k + 1) * LANE]

        def mix1_pre(r, q, n=CH):
            y = _ln(load_h(r + q, n))
            yr = pl.multiple_of(lax.rem(r, YB * TB) + q, n)
            for k in range(KD):
                ys[k, pl.ds(yr, n), :] = y[:, k * LANE:(k + 1) * LANE]
            put_cols(a1, q, _ln(y).astype(BF16))

        def mix1_dot(r, q, n=CH):
            for j in range(KD):
                a = _cat([_rows(a1, (k,), q, n) for k in range(KD)], 1)
                z = jnp.dot(a, _bf(w1_s[j]), preferred_element_type=F32)
                h1s[j, pl.ds(HALO + r + q, n), :] = _gelu(z).astype(BF16)

        def mix1(r, q):
            mix1_pre(r, q)
            mix1_dot(r, q)

        shifts = (-1, 1, -2, 2)

        TE = CFG["TE"]
        TM = 2 * TB // (P // TE)
        assert TM % CH == 0 or CH % TM == 0
        CM = min(CH, TM)

        def epi_body(i, c):
            blk = NSEG + i * (TE // SEG)
            t = pl.multiple_of(NSEG * TOK + i * TE, TE)
            r1 = pl.multiple_of(i * TM, TM)
            for q in range(0, TM, CM):
                mix1_pre(r1, q, CM)
            for j in range(KD):
                lo_ = _cat([_cat([_rows(o2[(h // 2) % 2], (blk + b, (h // 4) * 2 + h % 2), 0, SEG)
                                  for b in range(TE // SEG)], 0) for h in range(H)], 1)
                acc = jnp.dot(lo_, _bf(wo_s[j]), preferred_element_type=F32)
                hs[j, pl.ds(t, TE), :] = (xs[j, pl.ds(t, TE), :].astype(F32) + acc).astype(BF16)
            for q in range(0, TM, CM):
                mix1_dot(r1, q, CM)
            return c
        lax.fori_loop(0, P // TE, epi_body, 0)

        TT = CFG["TT"]
        NT, TBASE = 2 * TB // TT, (NB - 2) * TB

        def out_copy(r, n, slot):
            return pltpu.make_async_copy(ostage.at[slot, pl.ds(0, n)], out_hbm.at[pl.ds(r, n), :], sem_o.at[slot])

        def b2_body(i, with_mix1):
            n = TB if with_mix1 else TT
            r = pl.multiple_of(i * TB if with_mix1 else TBASE + i * TT, n)
            slot = lax.rem(i, 2)

            @pl.when(i >= 2)
            def _():
                out_copy(0, n, slot).wait()
            if not with_mix1:
                @pl.when(i < 2)
                def _():
                    out_copy(0, TB, slot).wait()

            def mix2(q):
                for j in range(KD):
                    d = shifts[j // (KD // 4)]
                    win = h1s[j, pl.ds(r + q, CH + 2 * HALO), :].astype(F32)
                    gs[j, q:q + CH, :] = win[HALO + d:HALO + d + CH, :].astype(BF16)
                yr = pl.multiple_of(lax.rem(r, YB * TB) + q, CH)
                for j in range(KD):
                    g = _cat([_rows(gs, (k,), q, CH) for k in range(KD)], 1)
                    x1s[j, q:q + CH, :] = (jnp.dot(g, _bf(w2_s[j]), preferred_element_type=F32)
                                           + ys[j, pl.ds(yr, CH), :])

            def up(q):
                put_cols(a3, q, _ln(_cat([x1s[k, q:q + CH, :] for k in range(KD)], 1)).astype(BF16))
                for f in range(KF):
                    a = _cat([_rows(a3, (k,), q, CH) for k in range(KD)], 1)
                    us[f, q:q + CH, :] = _gelu(jnp.dot(a, _bf(w3_s[f]), preferred_element_type=F32)).astype(BF16)

            def down(q):
                for j in range(KD):
                    u = _cat([_rows(us, (f,), q, CH) for f in range(KF)], 1)
                    y = jnp.dot(u, _bf(w4_s[j]), preferred_element_type=F32)
                    res = hs[j, pl.ds(r + q, CH), :].astype(F32) + x1s[j, q:q + CH, :]
                    ostage[slot, q:q + CH, j * LANE:(j + 1) * LANE] = (res + y).astype(BF16)

            r2 = pl.multiple_of((i + 2) * TB, TB)
            stage = {"a": lambda q: mix1(r2, q), "b": mix2, "c": up, "d": down}
            for name in CFG["ORDER" if with_mix1 else "ORDER2"].split():
                stage[name[0]](int(name[1:]) * CH)
            out_copy(r, n, slot).start()

        def b2_main(i, c):
            b2_body(i, True)
            return c

        def b2_tail(i, c):
            b2_body(i, False)
            return c
        lax.fori_loop(0, NB - 2, b2_main, 0)
        lax.fori_loop(0, NT, b2_tail, 0)
        for slot in range(2):
            out_copy(0, TT, slot).wait()

    scratch = [
        pltpu.VMEM((H + 2, D // 2, LANE), U32),
        pltpu.VMEM((H, D // 2, LANE), U32),
        pltpu.VMEM((H, D // 2, LANE), U32),
        pltpu.VMEM((KD, H * DH // 2, LANE), U32),
        pltpu.VMEM((KD, D // 2, LANE), U32),
        pltpu.VMEM((KD, D // 2, LANE), U32),
        pltpu.VMEM((KF, D // 2, LANE), U32),
        pltpu.VMEM((KD, F // 2, LANE), U32),
        pltpu.VMEM((KD, S, LANE), BF16),
        pltpu.VMEM((KD, P, LANE), BF16),
        pltpu.VMEM((NSEG + 1, KD, SEG, LANE), BF16),
        [pltpu.VMEM((NPAIR // 2, 2, R + 16, LANE), BF16) for _ in range(2)],
        [pltpu.VMEM((NPAIR // 2, 2, R + 16, LANE), BF16) for _ in range(2)],
        [pltpu.VMEM((NPAIR // 2, 2, R + 16, LANE), BF16) for _ in range(2)],
        [pltpu.VMEM((NSEG + PT, NPAIR, SEG, LANE), BF16) for _ in range(2)],
        [pltpu.VMEM((2 * (SEG + M), 2 * (SEG + M)), BF16) for _ in range(NPAIR)],
        pltpu.VMEM((KD, SEG, LANE), F32),
        pltpu.VMEM((KD, S, LANE), BF16),
        pltpu.VMEM((KD, S + 2 * HALO, LANE), BF16),
        pltpu.VMEM((KD, TB, LANE), BF16),
        pltpu.VMEM((KD, TB, LANE), BF16),
        pltpu.VMEM((KD, YB * TB, LANE), F32),
        pltpu.VMEM((KD, TB, LANE), F32),
        pltpu.VMEM((KD, TB, LANE), BF16),
        pltpu.VMEM((KF, TB, LANE), BF16),
        pltpu.VMEM((2, TB, D), BF16),
        pltpu.SemaphoreType.DMA((3,)),
        pltpu.SemaphoreType.DMA((3 * NPAIR + 1,)),
        pltpu.SemaphoreType.DMA((5,)),
        pltpu.SemaphoreType.DMA((2,)),
    ]
    return kernel, scratch


@functools.partial(jax.jit, static_argnames=("A_seg_len",))
def pallas_sequential_preLN__memory_aug_recurrent_mem_tr__mixer_s_mlp__prompt_kernel(
    A_x, A_mem0, A_Wq, A_Wk, A_Wv, A_Wo, A_seg_len, B_x, B_w1, B_w2, B_w3, B_w4,
):
    del B_x
    B, S, D = A_x.shape
    M = A_mem0.shape[1]
    H, DH = A_Wq.shape[1], A_Wq.shape[2]
    F = B_w3.shape[1]
    SEG = int(A_seg_len)
    assert B == 1 and DH == LANE and M == 8 and SEG == 32 and H % 8 == 0 and D == 4 * 2 * LANE
    kernel, scratch = _make_kernel(S, D, H, DH, M, SEG, F, TB=CFG["TB"])
    any_spec = pl.BlockSpec(memory_space=pl.ANY)
    out = pl.pallas_call(
        kernel,
        out_shape=jax.ShapeDtypeStruct((S, D), A_x.dtype),
        in_specs=[pl.BlockSpec(memory_space=pltpu.SMEM), any_spec, pl.BlockSpec()] + [any_spec] * 8,
        out_specs=any_spec,
        scratch_shapes=scratch,
        compiler_params=pltpu.CompilerParams(vmem_limit_bytes=120 * 1024 * 1024, flags=CFG["FLAGS"]),
    )(
        jnp.zeros((1,), jnp.int32),
        A_x.reshape(S, D),
        A_mem0.reshape(M, D),
        A_Wq.reshape(D // 2, 2, H, DH),
        A_Wk.reshape(D // 2, 2, H, DH),
        A_Wv.reshape(D // 2, 2, H, DH),
        A_Wo.reshape(H * DH, D),
        B_w1, B_w2, B_w3, B_w4,
    )
    return out.reshape(B, S, D)
```

```python
import functools

import numpy as np
import jax
import jax.numpy as jnp
from jax import lax
import jax.experimental.pallas as pl
import jax.experimental.pallas.tpu as pltpu

F32 = jnp.float32
BF16 = jnp.bfloat16
U32 = jnp.uint32
LANE = 128
EPS = 1e-5
CFG = dict(
    TB=256, TT=128, TE=128, CH=64,
    UN=2,
    SE=(13, 4), SO=(19, 4), PE=(25, 4), PO=(35, 4),
    LA=2, WOF=2, WON=4,
    ORDER="b0 a0 c0 b1 a1 c1 d0 b2 a2 c2 d1 b3 a3 c3 d2 d3", ORDER2="b0 b1 c0 c1 d0 d1",
    FLAGS=None,
)


def _bf(w_u32):
    return pltpu.bitcast(w_u32, BF16)


def _rows(ref, idx, start, n, align=16):
    w = ref.bitcast(U32)
    if isinstance(start, int):
        words = w[(*idx, slice(start // 2, (start + n) // 2), slice(None))]
    else:
        words = w[(*idx, pl.ds(pl.multiple_of(start // 2, align // 2), n // 2), slice(None))]
    return pltpu.bitcast(words, BF16)


def _ln(x):
    m = jnp.mean(x, axis=-1, keepdims=True)
    d = x - m
    v = jnp.mean(d * d, axis=-1, keepdims=True)
    return d * lax.rsqrt(v + EPS)


def _gelu(x):
    c0 = np.float32(np.sqrt(2.0 / np.pi))
    c1 = np.float32(np.sqrt(2.0 / np.pi) * 0.044715)
    t = jnp.tanh(x * (c0 + c1 * (x * x)))
    hx = 0.5 * x
    return hx + hx * t


def _cat(xs, axis):
    return xs[0] if len(xs) == 1 else jnp.concatenate(xs, axis=axis)


def _make_kernel(S, D, H, DH, M, SEG, F, TB):
    NSEG = S // SEG
    TOK = SEG - M
    P = S - NSEG * TOK
    R = P + SEG
    KD = D // LANE
    KF = F // LANE
    NPAIR = H // 2
    NB = S // TB
    HALO = 16
    YB = 4
    scale = np.float32(DH ** (-0.5))
    PT = P // SEG
    LNS = NSEG // NPAIR

    def kernel(zero_ref, x_hbm, mem0_ref, wq_hbm, wk_hbm, wv_hbm, wo_hbm, w1_hbm, w2_hbm, w3_hbm, w4_hbm,
               out_hbm,
               wq_s, wk_s, wv_s, wo_s, w1_s, w2_s, w3_s, w4_s,
               xs, xn0, xl, rq, rk, rv, o2, ps, wacc, hs, h1s, a1, gs, ys, x1s, a3, us, ostage,
               sem_x, sem_w, sem_b, sem_o):
        wqkv = ((wq_hbm, wq_s), (wk_hbm, wk_s), (wv_hbm, wv_s))

        def x_copies(lo, n, sem):
            return [pltpu.make_async_copy(x_hbm.at[pl.ds(lo, n), j * LANE:(j + 1) * LANE],
                                          xs.at[j, pl.ds(lo, n)], sem) for j in range(KD)]

        def pair_copies(j, m, src=None):
            w_hbm, w_s = wqkv[m]
            wb = w_hbm.bitcast(U32)
            src = j if src is None else src
            return [pltpu.make_async_copy(wb.at[:, p, src, :], w_s.at[2 * j + p], sem_w.at[3 * j + m])
                    for p in range(2)]

        def col_copies(w_hbm, w_s, sem):
            wb = w_hbm.bitcast(U32)
            return [pltpu.make_async_copy(wb.at[:, pl.ds(j * LANE, LANE)], w_s.at[j], sem)
                    for j in range(w_s.shape[0])]

        x_head = x_copies(0, P, sem_x.at[0])
        XC = (S - P) // (NPAIR // 2)
        XA = 2
        x_tail_a = x_copies(P, XA * XC, sem_x.at[1])
        x_tail_b = x_copies(P + XA * XC, S - P - XA * XC, sem_x.at[2])
        wo_copies = functools.partial(col_copies, wo_hbm, wo_s, sem_b.at[4])
        b_groups = [col_copies(wh, ws, sem_b.at[i])
                    for i, (wh, ws) in enumerate(((w1_hbm, w1_s), (w2_hbm, w2_s), (w3_hbm, w3_s), (w4_hbm, w4_s)))]
        b_copies = [c for g in b_groups for c in g]

        NI = NPAIR // 2

        def start(cps):
            for cp in cps:
                cp.start()

        def need(i):
            return [(2 * i, 1), (2 * i, 2), (2 * i + 1, 0), (2 * i + 1, 1), (2 * i + 1, 2), (2 * i + 2, 0)]

        def group_copies(j, m):
            return pair_copies(j, m, src=0) if j == NPAIR else pair_copies(j, m)

        def need_copies(i):
            return [c for j, m in need(i) for c in group_copies(j, m)]

        LA = CFG["LA"]
        WOF, WON = CFG["WOF"], CFG["WON"]
        assert WOF >= 1 and WOF + WON <= NI and KD % WON == 0 and 1 <= LA < NI
        start(x_head + pair_copies(0, 0) + pair_copies(0, 1))

        for k in range(KD):
            xl[0, k, 0:M, :] = mem0_ref[:, k * LANE:(k + 1) * LANE]

        def wait(cps):
            for cp in cps:
                cp.wait()

        wait(x_head + pair_copies(0, 0))
        start(pair_copies(0, 2) + pair_copies(1, 0) + x_tail_a)

        def ln_rows(store, src_row, n):
            xf = _cat([xs[k, pl.ds(src_row, n), :] for k in range(KD)], 1).astype(F32)
            xn = _ln(xf).astype(BF16)
            for k in range(KD):
                store(k, xn[:, k * LANE:(k + 1) * LANE])
            return xn[n - 16:n, D - LANE:D]

        def untangle(j, m):
            w_s = wqkv[m][1]
            a = w_s[2 * j]
            b = w_s[2 * j + 1]
            w_s[2 * j] = (a & np.uint32(0xFFFF)) | (b << 16)
            w_s[2 * j + 1] = (a >> 16) | (b & np.uint32(0xFFFF0000))

        untangle(0, 0)
        for r in range(0, P, 128):
            def store(k, v, r=r):
                xn0[k, r:r + 128, :] = v
            ln_rows(store, r, 128)
            for hh in range(2):
                lhs0 = _cat([_rows(xn0, (k,), r, 128) for k in range(KD)], 1)
                rq[0][0, hh, r:r + 128, :] = jnp.dot(lhs0, _bf(wq_s[hh]), preferred_element_type=F32).astype(BF16)

        def pro_body(i, first):
            groups = [(cls, m) for cls in range(2) for m in range(3)]
            nxt = need(i)
            ties = []
            if not first:
                for jn, mn in nxt:
                    wait(pair_copies(jn, mn, src=0))
                pl.when(i == XA)(functools.partial(wait, x_tail_b))

                for k in range(1, NI):
                    late = (need_copies(k + LA) if k + LA < NI else []) + (
                        wo_copies()[(k - WOF) * KD // WON:(k - WOF + 1) * KD // WON] if WOF <= k < WOF + WON else [])
                    if late:
                        pl.when(i == k)(functools.partial(start, late))
            ln_at = 2 if first else 1
            for n, (cls, m) in enumerate(groups):
                j = 2 * i + cls
                jn, mn = nxt[n]
                if first:
                    if n == 0:
                        wait(pair_copies(0, 1) + pair_copies(0, 2))
                        start(pair_copies(1, 1) + pair_copies(1, 2) + pair_copies(2, 0))
                        untangle(jn, mn)
                        continue
                    if n == 2:
                        wait(pair_copies(1, 0) + pair_copies(1, 1) + x_tail_a)
                        start(need_copies(1))
                    if n == 4:
                        wait(pair_copies(1, 2) + pair_copies(2, 0))
                        start(x_tail_b + [c for k in range(2, LA + 1) for c in need_copies(k)])
                untangle(jn, mn)
                r_s = (rq, rk, rv)[m]
                for hh in range(2):
                    tiles = [_rows(xn0, (k,), 0, P) for k in range(KD)]
                    if hh == 0 and ties:
                        head = tiles[0][0:16]
                        for t, tie in enumerate(ties):
                            head = jnp.where(never > t, tie, head)
                        tiles[0] = _cat([head, tiles[0][16:]], 0)
                    w = _bf(wqkv[m][1][2 * j + hh])
                    r_s[cls][i, hh, 0:P, :] = jnp.dot(_cat(tiles, 1), w, preferred_element_type=F32).astype(BF16)
                ties = []
                if ln_at <= n < ln_at + LNS:
                    for t in range(2):
                        sg = i * 2 * LNS + 2 * (n - ln_at) + t

                        def store(k, v, sg=sg):
                            xl[sg, k, M:SEG, :] = v
                        ties.append(ln_rows(store, pl.multiple_of(P + sg * TOK, 8), TOK))

        never = zero_ref[0]
        pro_body(0, True)

        def pro_loop(i, c):
            pro_body(i, False)
            return c
        lax.fori_loop(1, NPAIR // 2, pro_loop, 0)

        wait(wo_copies())
        start(b_copies)

        def step(s, c):
            srow = pl.multiple_of(s * SEG, SEG)
            lhs = _cat([_rows(xl, (s, k), 0, SEG) for k in range(KD)], 1)
            wr = [pl.multiple_of(lax.rem(P + s * TOK + 8 * i, R), 8) for i in range(TOK // 8)]
            rr = pl.multiple_of(lax.rem(srow, R), SEG)
            oblk, orow = [], []
            for i in range(SEG // 8):
                p = s * (SEG // 8) + i
                oblk.append(jnp.where(s < NSEG - PT, p // (TOK // 8), s + PT))
                orow.append(pl.multiple_of(jnp.where(s < NSEG - PT, M + (p % (TOK // 8)) * 8, 8 * i), 8))
            L = 2 * (SEG + M)
            ri = lax.broadcasted_iota(jnp.int32, (L, L), 0)
            ci = lax.broadcasted_iota(jnp.int32, (L, L), 1)

            def head_of(i):
                return ((i >= SEG) & (i < 2 * SEG)) | (i >= 2 * SEG + M)
            same = head_of(ri) == head_of(ci)
            allowed = same & ((ri >= 2 * SEG) | (ci >= 2 * SEG) | ((ci & (SEG - 1)) <= (ri & (SEG - 1))))
            fill = jnp.where(same, np.float32(-1e9), np.float32(-1e30))

            def proj(w_s, r_s, h):
                j, hh = h // 2, h % 2
                ring = r_s[j % 2]
                y = jnp.dot(lhs, _bf(w_s[h]), preferred_element_type=F32)
                ring[j // 2, 0, R + hh * M:R + (hh + 1) * M, :] = y[0:M, :].astype(BF16)
                for i in range(TOK // 8):
                    ring[j // 2, hh, pl.ds(wr[i], 8), :] = y[M + 8 * i:M + 8 * i + 8, :].astype(BF16)

            def stack(r_s, j):
                ring = r_s[j % 2]
                return _cat([_rows(ring, (j // 2, 0), rr, SEG, SEG), _rows(ring, (j // 2, 1), rr, SEG, SEG),
                             _rows(ring, (j // 2, 0), R, 2 * M)], 0)

            def proj_qk(j):
                for w_s, r_s in ((wq_s, rq), (wk_s, rk)):
                    proj(w_s, r_s, 2 * j)
                    proj(w_s, r_s, 2 * j + 1)

            def proj_v(j):
                proj(wv_s, rv, 2 * j)
                proj(wv_s, rv, 2 * j + 1)

            def score(j):
                q = stack(rq, j)
                k = stack(rk, j)
                sc = lax.dot_general(q, k, (((1,), (1,)), ((), ())), preferred_element_type=F32)
                sc = jnp.where(allowed, sc * scale, fill)
                mx = jnp.max(sc, axis=-1, keepdims=True)
                e = jnp.exp(sc - mx)
                l = jnp.sum(e, axis=-1, keepdims=True)
                r = pl.reciprocal(l, approx=True)
                r = r * (2.0 - l * r)
                ps[j][...] = (e * r).astype(BF16)

            def pv(j):
                o = jnp.dot(ps[j][...], stack(rv, j), preferred_element_type=F32)
                for hh in range(2):
                    dst, slot = o2[j % 2], (j // 2) * 2 + hh
                    for i in range(SEG // 8):
                        dst[oblk[i], slot, pl.ds(orow[i], 8), :] = (
                            o[hh * SEG + 8 * i:hh * SEG + 8 * i + 8, :].astype(BF16))
                    dst[s, slot, 0:M, :] = o[2 * SEG + hh * M:2 * SEG + (hh + 1) * M, :].astype(BF16)

            def wo_tile(par, j):
                pairs = range(par, NPAIR, 2)
                lo_ = _cat([_rows(o2[par], (s, slot), 0, SEG) for slot in range(NPAIR)], 1)
                w = _cat([wo_s[j, pj * DH:(pj + 1) * DH, :] for pj in pairs], 0)
                return jnp.dot(lo_, _bf(w), preferred_element_type=F32)

            NH = NPAIR // 2
            accs = [None] * KD

            def wo_a(j):
                wacc[j] = wo_tile(0, j)

            def wo_b(j):
                accs[j] = wacc[j] + wo_tile(1, j)
                finish(j)

            hrow = pl.multiple_of(s * TOK, 8)
            snext = jnp.minimum(s + 1, NSEG)

            def finish(j):
                acc = accs[j]
                xl[snext, j, 0:M, :] = acc[0:M, :].astype(BF16)
                hs[j, pl.ds(hrow, TOK), :] = (xs[j, pl.ds(hrow, TOK), :].astype(F32) + acc[M:SEG, :]).astype(BF16)

            main = ([(proj_qk, 2 * i) for i in range(NH)] + [(proj_qk, 2 * i + 1) for i in range(NH)]
                    + [(proj_v, 2 * i) for i in range(NH)] + [(proj_v, 2 * i + 1) for i in range(NH)]
                    + [(wo_a, j) for j in range(KD)] + [(wo_b, j) for j in range(KD)])
            extra = {}
            for fn2, par, (off, rate) in ((score, 0, CFG["SE"]), (score, 1, CFG["SO"]),
                                          (pv, 0, CFG["PE"]), (pv, 1, CFG["PO"])):
                for i in range(NH):
                    extra.setdefault(off + int(i / rate), []).append((fn2, 2 * i + par))
            assert max(extra) < len(main)
            for t, (fn, arg) in enumerate(main):
                fn(arg)
                for fn2, arg2 in extra.get(t, []):
                    fn2(arg2)
            return c
        UN = CFG["UN"]

        def steps(i, c):
            for u in range(UN):
                step(i * UN + u, c)
            return c
        lax.fori_loop(0, NSEG // UN, steps, 0)
        for cp in b_copies:
            cp.wait()
        zero_halo = jnp.zeros((HALO, LANE), BF16)
        for j in range(KD):
            h1s[j, 0:HALO, :] = zero_halo
            h1s[j, HALO + S:HALO + S + HALO, :] = zero_halo

        CH = CFG["CH"]

        def load_h(r, n):
            return _cat([hs[k, pl.ds(r, n), :] for k in range(KD)], 1).astype(F32)

        def put_cols(dst, row, val):
            for k in range(KD):
                dst[k, row:row + val.shape[0], :] = val[:, k * LANE:(k + 1) * LANE]

        def mix1_pre(r, q, n=CH):
            y = _ln(load_h(r + q, n))
            yr = pl.multiple_of(lax.rem(r, YB * TB) + q, n)
            for k in range(KD):
                ys[k, pl.ds(yr, n), :] = y[:, k * LANE:(k + 1) * LANE]
            put_cols(a1, q, _ln(y).astype(BF16))

        def mix1_dot(r, q, n=CH):
            for j in range(KD):
                a = _cat([_rows(a1, (k,), q, n) for k in range(KD)], 1)
                z = jnp.dot(a, _bf(w1_s[j]), preferred_element_type=F32)
                h1s[j, pl.ds(HALO + r + q, n), :] = _gelu(z).astype(BF16)

        def mix1(r, q):
            mix1_pre(r, q)
            mix1_dot(r, q)

        shifts = (-1, 1, -2, 2)

        TE = CFG["TE"]
        TM = 2 * TB // (P // TE)
        assert TM % CH == 0 or CH % TM == 0
        CM = min(CH, TM)

        def epi_body(i, c):
            blk = NSEG + i * (TE // SEG)
            t = pl.multiple_of(NSEG * TOK + i * TE, TE)
            r1 = pl.multiple_of(i * TM, TM)
            for q in range(0, TM, CM):
                mix1_pre(r1, q, CM)
            for j in range(KD):
                lo_ = _cat([_cat([_rows(o2[(h // 2) % 2], (blk + b, (h // 4) * 2 + h % 2), 0, SEG)
                                  for b in range(TE // SEG)], 0) for h in range(H)], 1)
                acc = jnp.dot(lo_, _bf(wo_s[j]), preferred_element_type=F32)
                hs[j, pl.ds(t, TE), :] = (xs[j, pl.ds(t, TE), :].astype(F32) + acc).astype(BF16)
            for q in range(0, TM, CM):
                mix1_dot(r1, q, CM)
            return c
        lax.fori_loop(0, P // TE, epi_body, 0)

        TT = CFG["TT"]
        NT, TBASE = 2 * TB // TT, (NB - 2) * TB

        def out_copy(r, n, slot):
            return pltpu.make_async_copy(ostage.at[slot, pl.ds(0, n)], out_hbm.at[pl.ds(r, n), :], sem_o.at[slot])

        def b2_body(i, with_mix1):
            n = TB if with_mix1 else TT
            r = pl.multiple_of(i * TB if with_mix1 else TBASE + i * TT, n)
            slot = lax.rem(i, 2)

            @pl.when(i >= 2)
            def _():
                out_copy(0, n, slot).wait()
            if not with_mix1:
                @pl.when(i < 2)
                def _():
                    out_copy(0, TB, slot).wait()

            def mix2(q):
                for j in range(KD):
                    d = shifts[j // (KD // 4)]
                    win = h1s[j, pl.ds(r + q, CH + 2 * HALO), :].astype(F32)
                    gs[j, q:q + CH, :] = win[HALO + d:HALO + d + CH, :].astype(BF16)
                yr = pl.multiple_of(lax.rem(r, YB * TB) + q, CH)
                for j in range(KD):
                    g = _cat([_rows(gs, (k,), q, CH) for k in range(KD)], 1)
                    x1s[j, q:q + CH, :] = (jnp.dot(g, _bf(w2_s[j]), preferred_element_type=F32)
                                           + ys[j, pl.ds(yr, CH), :])

            def up(q):
                put_cols(a3, q, _ln(_cat([x1s[k, q:q + CH, :] for k in range(KD)], 1)).astype(BF16))
                for f in range(KF):
                    a = _cat([_rows(a3, (k,), q, CH) for k in range(KD)], 1)
                    us[f, q:q + CH, :] = _gelu(jnp.dot(a, _bf(w3_s[f]), preferred_element_type=F32)).astype(BF16)

            def down(q):
                for j in range(KD):
                    u = _cat([_rows(us, (f,), q, CH) for f in range(KF)], 1)
                    y = jnp.dot(u, _bf(w4_s[j]), preferred_element_type=F32)
                    res = hs[j, pl.ds(r + q, CH), :].astype(F32) + x1s[j, q:q + CH, :]
                    ostage[slot, q:q + CH, j * LANE:(j + 1) * LANE] = (res + y).astype(BF16)

            r2 = pl.multiple_of((i + 2) * TB, TB)
            stage = {"a": lambda q: mix1(r2, q), "b": mix2, "c": up, "d": down}
            for name in CFG["ORDER" if with_mix1 else "ORDER2"].split():
                stage[name[0]](int(name[1:]) * CH)
            out_copy(r, n, slot).start()

        def b2_main(i, c):
            b2_body(i, True)
            return c

        def b2_tail(i, c):
            b2_body(i, False)
            return c
        lax.fori_loop(0, NB - 2, b2_main, 0)
        lax.fori_loop(0, NT, b2_tail, 0)
        for slot in range(2):
            out_copy(0, TT, slot).wait()

    scratch = [
        pltpu.VMEM((H + 2, D // 2, LANE), U32),
        pltpu.VMEM((H, D // 2, LANE), U32),
        pltpu.VMEM((H, D // 2, LANE), U32),
        pltpu.VMEM((KD, H * DH // 2, LANE), U32),
        pltpu.VMEM((KD, D // 2, LANE), U32),
        pltpu.VMEM((KD, D // 2, LANE), U32),
        pltpu.VMEM((KF, D // 2, LANE), U32),
        pltpu.VMEM((KD, F // 2, LANE), U32),
        pltpu.VMEM((KD, S, LANE), BF16),
        pltpu.VMEM((KD, P, LANE), BF16),
        pltpu.VMEM((NSEG + 1, KD, SEG, LANE), BF16),
        [pltpu.VMEM((NPAIR // 2, 2, R + 16, LANE), BF16) for _ in range(2)],
        [pltpu.VMEM((NPAIR // 2, 2, R + 16, LANE), BF16) for _ in range(2)],
        [pltpu.VMEM((NPAIR // 2, 2, R + 16, LANE), BF16) for _ in range(2)],
        [pltpu.VMEM((NSEG + PT, NPAIR, SEG, LANE), BF16) for _ in range(2)],
        [pltpu.VMEM((2 * (SEG + M), 2 * (SEG + M)), BF16) for _ in range(NPAIR)],
        pltpu.VMEM((KD, SEG, LANE), F32),
        pltpu.VMEM((KD, S, LANE), BF16),
        pltpu.VMEM((KD, S + 2 * HALO, LANE), BF16),
        pltpu.VMEM((KD, TB, LANE), BF16),
        pltpu.VMEM((KD, TB, LANE), BF16),
        pltpu.VMEM((KD, YB * TB, LANE), F32),
        pltpu.VMEM((KD, TB, LANE), F32),
        pltpu.VMEM((KD, TB, LANE), BF16),
        pltpu.VMEM((KF, TB, LANE), BF16),
        pltpu.VMEM((2, TB, D), BF16),
        pltpu.SemaphoreType.DMA((3,)),
        pltpu.SemaphoreType.DMA((3 * NPAIR + 1,)),
        pltpu.SemaphoreType.DMA((5,)),
        pltpu.SemaphoreType.DMA((2,)),
    ]
    return kernel, scratch


@functools.partial(jax.jit, static_argnames=("A_seg_len",))
def pallas_sequential_preLN__memory_aug_recurrent_mem_tr__mixer_s_mlp__prompt_kernel(
    A_x, A_mem0, A_Wq, A_Wk, A_Wv, A_Wo, A_seg_len, B_x, B_w1, B_w2, B_w3, B_w4,
):
    del B_x
    B, S, D = A_x.shape
    M = A_mem0.shape[1]
    H, DH = A_Wq.shape[1], A_Wq.shape[2]
    F = B_w3.shape[1]
    SEG = int(A_seg_len)
    assert B == 1 and DH == LANE and M == 8 and SEG == 32 and H % 8 == 0 and D == 4 * 2 * LANE
    kernel, scratch = _make_kernel(S, D, H, DH, M, SEG, F, TB=CFG["TB"])
    any_spec = pl.BlockSpec(memory_space=pl.ANY)
    out = pl.pallas_call(
        kernel,
        out_shape=jax.ShapeDtypeStruct((S, D), A_x.dtype),
        in_specs=[pl.BlockSpec(memory_space=pltpu.SMEM), any_spec, pl.BlockSpec()] + [any_spec] * 8,
        out_specs=any_spec,
        scratch_shapes=scratch,
        compiler_params=pltpu.CompilerParams(vmem_limit_bytes=120 * 1024 * 1024, flags=CFG["FLAGS"]),
    )(
        jnp.zeros((1,), jnp.int32),
        A_x.reshape(S, D),
        A_mem0.reshape(M, D),
        A_Wq.reshape(D // 2, 2, H, DH),
        A_Wk.reshape(D // 2, 2, H, DH),
        A_Wv.reshape(D // 2, 2, H, DH),
        A_Wo.reshape(H * DH, D),
        B_w1, B_w2, B_w3, B_w4,
    )
    return out.reshape(B, S, D)
```

```python
import functools

import numpy as np
import jax
import jax.numpy as jnp
from jax import lax
import jax.experimental.pallas as pl
import jax.experimental.pallas.tpu as pltpu

F32 = jnp.float32
BF16 = jnp.bfloat16
U32 = jnp.uint32
LANE = 128
EPS = 1e-5
CFG = dict(
    TB=256, TT=128, TE=128, CH=64,
    LAG=2,
    UN=2,
    SE=(13, 4), SO=(19, 4), PE=(25, 4), PO=(35, 4),
    LA=2, WOF=2, WON=4,
    ORDER="b0 a0 c0 b1 a1 c1 d0 b2 a2 c2 d1 b3 a3 c3 d2 d3", ORDER2="b0 b1 c0 c1 d0 d1",
    FLAGS=None,
)


def _bf(w_u32):
    return pltpu.bitcast(w_u32, BF16)


def _rows(ref, idx, start, n, align=16):
    w = ref.bitcast(U32)
    if isinstance(start, int):
        words = w[(*idx, slice(start // 2, (start + n) // 2), slice(None))]
    else:
        words = w[(*idx, pl.ds(pl.multiple_of(start // 2, align // 2), n // 2), slice(None))]
    return pltpu.bitcast(words, BF16)


def _ln(x):
    m = jnp.mean(x, axis=-1, keepdims=True)
    d = x - m
    v = jnp.mean(d * d, axis=-1, keepdims=True)
    return d * lax.rsqrt(v + EPS)


def _gelu(x):
    c0 = np.float32(np.sqrt(2.0 / np.pi))
    c1 = np.float32(np.sqrt(2.0 / np.pi) * 0.044715)
    t = jnp.tanh(x * (c0 + c1 * (x * x)))
    hx = 0.5 * x
    return hx + hx * t


def _cat(xs, axis):
    return xs[0] if len(xs) == 1 else jnp.concatenate(xs, axis=axis)


def _make_kernel(S, D, H, DH, M, SEG, F, TB):
    NSEG = S // SEG
    TOK = SEG - M
    P = S - NSEG * TOK
    R = P + SEG
    KD = D // LANE
    KF = F // LANE
    NPAIR = H // 2
    NB = S // TB
    HALO = 16
    YB = 4
    scale = np.float32(DH ** (-0.5))
    PT = P // SEG
    LNS = NSEG // NPAIR

    def kernel(zero_ref, x_hbm, mem0_ref, wq_hbm, wk_hbm, wv_hbm, wo_hbm, w1_hbm, w2_hbm, w3_hbm, w4_hbm,
               out_hbm,
               wq_s, wk_s, wv_s, wo_s, w1_s, w2_s, w3_s, w4_s,
               xs, xn0, xl, rq, rk, rv, o2, ps, wacc, hs, h1s, a1, gs, ys, x1s, a3, us, ostage,
               sem_x, sem_w, sem_b, sem_o):
        wqkv = ((wq_hbm, wq_s), (wk_hbm, wk_s), (wv_hbm, wv_s))

        def x_copies(lo, n, sem):
            return [pltpu.make_async_copy(x_hbm.at[pl.ds(lo, n), j * LANE:(j + 1) * LANE],
                                          xs.at[j, pl.ds(lo, n)], sem) for j in range(KD)]

        def pair_copies(j, m, src=None):
            w_hbm, w_s = wqkv[m]
            wb = w_hbm.bitcast(U32)
            src = j if src is None else src
            return [pltpu.make_async_copy(wb.at[:, p, src, :], w_s.at[2 * j + p], sem_w.at[3 * j + m])
                    for p in range(2)]

        def col_copies(w_hbm, w_s, sem, lo=0, hi=None):
            wb = w_hbm.bitcast(U32)
            return [pltpu.make_async_copy(wb.at[:, pl.ds(j * LANE, LANE)], w_s.at[j], sem)
                    for j in range(lo, w_s.shape[0] if hi is None else hi)]

        x_head = x_copies(0, P, sem_x.at[0])
        XC = (S - P) // (NPAIR // 2)
        XA = 2
        x_tail_a = x_copies(P, XA * XC, sem_x.at[1])
        x_tail_b = x_copies(P + XA * XC, S - P - XA * XC, sem_x.at[2])
        wo_copies = functools.partial(col_copies, wo_hbm, wo_s, sem_b.at[4])
        b_groups = [col_copies(wh, ws, sem_b.at[i])
                    for i, (wh, ws) in enumerate(((w1_hbm, w1_s), (w2_hbm, w2_s), (w3_hbm, w3_s), (w4_hbm, w4_s)))]
        b_copies = [c for g in b_groups for c in g]

        NI = NPAIR // 2

        def start(cps):
            for cp in cps:
                cp.start()

        def need(i):
            return [(2 * i, 1), (2 * i, 2), (2 * i + 1, 0), (2 * i + 1, 1), (2 * i + 1, 2), (2 * i + 2, 0)]

        def group_copies(j, m):
            return pair_copies(j, m, src=0) if j == NPAIR else pair_copies(j, m)

        def need_copies(i):
            return [c for j, m in need(i) for c in group_copies(j, m)]

        LA = CFG["LA"]
        WOF, WON = CFG["WOF"], CFG["WON"]
        assert WOF >= 1 and WOF + WON <= NI and KD % WON == 0 and 1 <= LA < NI
        start(x_head + pair_copies(0, 0) + pair_copies(0, 1))

        for k in range(KD):
            xl[0, k, 0:M, :] = mem0_ref[:, k * LANE:(k + 1) * LANE]

        def wait(cps):
            for cp in cps:
                cp.wait()

        wait(x_head + pair_copies(0, 0))
        start(pair_copies(0, 2) + pair_copies(1, 0) + x_tail_a)

        def ln_rows(store, src_row, n):
            xf = _cat([xs[k, pl.ds(src_row, n), :] for k in range(KD)], 1).astype(F32)
            xn = _ln(xf).astype(BF16)
            for k in range(KD):
                store(k, xn[:, k * LANE:(k + 1) * LANE])
            return xn[n - 16:n, D - LANE:D]

        def untangle(j, m):
            w_s = wqkv[m][1]
            a = w_s[2 * j]
            b = w_s[2 * j + 1]
            w_s[2 * j] = (a & np.uint32(0xFFFF)) | (b << 16)
            w_s[2 * j + 1] = (a >> 16) | (b & np.uint32(0xFFFF0000))

        untangle(0, 0)
        for r in range(0, P, 128):
            def store(k, v, r=r):
                xn0[k, r:r + 128, :] = v
            ln_rows(store, r, 128)
            for hh in range(2):
                lhs0 = _cat([_rows(xn0, (k,), r, 128) for k in range(KD)], 1)
                rq[0][0, hh, r:r + 128, :] = jnp.dot(lhs0, _bf(wq_s[hh]), preferred_element_type=F32).astype(BF16)

        def pro_body(i, first):
            groups = [(cls, m) for cls in range(2) for m in range(3)]
            nxt = need(i)
            ties = []
            if not first:
                for jn, mn in nxt:
                    wait(pair_copies(jn, mn, src=0))
                pl.when(i == XA)(functools.partial(wait, x_tail_b))

                for k in range(1, NI):
                    late = (need_copies(k + LA) if k + LA < NI else []) + (
                        wo_copies((k - WOF) * KD // WON, (k - WOF + 1) * KD // WON) if WOF <= k < WOF + WON else [])
                    if late:
                        pl.when(i == k)(functools.partial(start, late))
            ln_at = 2 if first else 1
            for n, (cls, m) in enumerate(groups):
                j = 2 * i + cls
                jn, mn = nxt[n]
                if first:
                    if n == 0:
                        wait(pair_copies(0, 1) + pair_copies(0, 2))
                        start(pair_copies(1, 1) + pair_copies(1, 2) + pair_copies(2, 0))
                        untangle(jn, mn)
                        continue
                    if n == 2:
                        wait(pair_copies(1, 0) + pair_copies(1, 1) + x_tail_a)
                        start(need_copies(1))
                    if n == 4:
                        wait(pair_copies(1, 2) + pair_copies(2, 0))
                        start(x_tail_b + [c for k in range(2, LA + 1) for c in need_copies(k)])
                untangle(jn, mn)
                r_s = (rq, rk, rv)[m]
                for hh in range(2):
                    tiles = [_rows(xn0, (k,), 0, P) for k in range(KD)]
                    if hh == 0 and ties:
                        head = tiles[0][0:16]
                        for t, tie in enumerate(ties):
                            head = jnp.where(never > t, tie, head)
                        tiles[0] = _cat([head, tiles[0][16:]], 0)
                    w = _bf(wqkv[m][1][2 * j + hh])
                    r_s[cls][i, hh, 0:P, :] = jnp.dot(_cat(tiles, 1), w, preferred_element_type=F32).astype(BF16)
                ties = []
                if ln_at <= n < ln_at + LNS:
                    for t in range(2):
                        sg = i * 2 * LNS + 2 * (n - ln_at) + t

                        def store(k, v, sg=sg):
                            xl[sg, k, M:SEG, :] = v
                        ties.append(ln_rows(store, pl.multiple_of(P + sg * TOK, 8), TOK))

        never = zero_ref[0]
        pro_body(0, True)

        def pro_loop(i, c):
            pro_body(i, False)
            return c
        lax.fori_loop(1, NPAIR // 2, pro_loop, 0)

        wait(wo_copies())
        start(b_copies)

        def step(s, c):
            srow = pl.multiple_of(s * SEG, SEG)
            lhs = _cat([_rows(xl, (s, k), 0, SEG) for k in range(KD)], 1)
            wr = [pl.multiple_of(lax.rem(P + s * TOK + 8 * i, R), 8) for i in range(TOK // 8)]
            rr = pl.multiple_of(lax.rem(srow, R), SEG)
            oblk, orow = [], []
            for i in range(SEG // 8):
                p = s * (SEG // 8) + i
                oblk.append(jnp.where(s < NSEG - PT, p // (TOK // 8), s + PT))
                orow.append(pl.multiple_of(jnp.where(s < NSEG - PT, M + (p % (TOK // 8)) * 8, 8 * i), 8))
            L = 2 * (SEG + M)
            ri = lax.broadcasted_iota(jnp.int32, (L, L), 0)
            ci = lax.broadcasted_iota(jnp.int32, (L, L), 1)

            def head_of(i):
                return ((i >= SEG) & (i < 2 * SEG)) | (i >= 2 * SEG + M)
            same = head_of(ri) == head_of(ci)
            allowed = same & ((ri >= 2 * SEG) | (ci >= 2 * SEG) | ((ci & (SEG - 1)) <= (ri & (SEG - 1))))
            fill = jnp.where(same, np.float32(-1e9), np.float32(-1e30))

            def proj(w_s, r_s, h):
                j, hh = h // 2, h % 2
                ring = r_s[j % 2]
                y = jnp.dot(lhs, _bf(w_s[h]), preferred_element_type=F32)
                ring[j // 2, 0, R + hh * M:R + (hh + 1) * M, :] = y[0:M, :].astype(BF16)
                for i in range(TOK // 8):
                    ring[j // 2, hh, pl.ds(wr[i], 8), :] = y[M + 8 * i:M + 8 * i + 8, :].astype(BF16)

            def stack(r_s, j):
                ring = r_s[j % 2]
                return _cat([_rows(ring, (j // 2, 0), rr, SEG, SEG), _rows(ring, (j // 2, 1), rr, SEG, SEG),
                             _rows(ring, (j // 2, 0), R, 2 * M)], 0)

            def proj_qk(j):
                for w_s, r_s in ((wq_s, rq), (wk_s, rk)):
                    proj(w_s, r_s, 2 * j)
                    proj(w_s, r_s, 2 * j + 1)

            def proj_v(j):
                proj(wv_s, rv, 2 * j)
                proj(wv_s, rv, 2 * j + 1)

            def score(j):
                q = stack(rq, j)
                k = stack(rk, j)
                sc = lax.dot_general(q, k, (((1,), (1,)), ((), ())), preferred_element_type=F32)
                sc = jnp.where(allowed, sc * scale, fill)
                mx = jnp.max(sc, axis=-1, keepdims=True)
                e = jnp.exp(sc - mx)
                l = jnp.sum(e, axis=-1, keepdims=True)
                r = pl.reciprocal(l, approx=True)
                r = r * (2.0 - l * r)
                ps[j][...] = (e * r).astype(BF16)

            def pv(j):
                o = jnp.dot(ps[j][...], stack(rv, j), preferred_element_type=F32)
                for hh in range(2):
                    dst, slot = o2[j % 2], (j // 2) * 2 + hh
                    for i in range(SEG // 8):
                        dst[oblk[i], slot, pl.ds(orow[i], 8), :] = (
                            o[hh * SEG + 8 * i:hh * SEG + 8 * i + 8, :].astype(BF16))
                    dst[s, slot, 0:M, :] = o[2 * SEG + hh * M:2 * SEG + (hh + 1) * M, :].astype(BF16)

            def wo_tile(par, j):
                pairs = range(par, NPAIR, 2)
                lo_ = _cat([_rows(o2[par], (s, slot), 0, SEG) for slot in range(NPAIR)], 1)
                w = _cat([wo_s[j, pj * DH:(pj + 1) * DH, :] for pj in pairs], 0)
                return jnp.dot(lo_, _bf(w), preferred_element_type=F32)

            NH = NPAIR // 2
            accs = [None] * KD

            def wo_a(j):
                wacc[j] = wo_tile(0, j)

            def wo_b(j):
                accs[j] = wacc[j] + wo_tile(1, j)
                finish(j)

            hrow = pl.multiple_of(s * TOK, 8)
            snext = jnp.minimum(s + 1, NSEG)

            def finish(j):
                acc = accs[j]
                xl[snext, j, 0:M, :] = acc[0:M, :].astype(BF16)
                hs[j, pl.ds(hrow, TOK), :] = (xs[j, pl.ds(hrow, TOK), :].astype(F32) + acc[M:SEG, :]).astype(BF16)

            main = ([(proj_qk, 2 * i) for i in range(NH)] + [(proj_qk, 2 * i + 1) for i in range(NH)]
                    + [(proj_v, 2 * i) for i in range(NH)] + [(proj_v, 2 * i + 1) for i in range(NH)]
                    + [(wo_a, j) for j in range(KD)] + [(wo_b, j) for j in range(KD)])
            extra = {}
            for fn2, par, (off, rate) in ((score, 0, CFG["SE"]), (score, 1, CFG["SO"]),
                                          (pv, 0, CFG["PE"]), (pv, 1, CFG["PO"])):
                for i in range(NH):
                    extra.setdefault(off + int(i / rate), []).append((fn2, 2 * i + par))
            assert max(extra) < len(main)
            for t, (fn, arg) in enumerate(main):
                fn(arg)
                for fn2, arg2 in extra.get(t, []):
                    fn2(arg2)
            return c
        UN = CFG["UN"]

        def steps(i, c):
            for u in range(UN):
                step(i * UN + u, c)
            return c
        lax.fori_loop(0, NSEG // UN, steps, 0)
        for cp in b_copies:
            cp.wait()
        zero_halo = jnp.zeros((HALO, LANE), BF16)
        for j in range(KD):
            h1s[j, 0:HALO, :] = zero_halo
            h1s[j, HALO + S:HALO + S + HALO, :] = zero_halo

        CH = CFG["CH"]

        def load_h(r, n):
            return _cat([hs[k, pl.ds(r, n), :] for k in range(KD)], 1).astype(F32)

        def put_cols(dst, row, val):
            for k in range(KD):
                dst[k, row:row + val.shape[0], :] = val[:, k * LANE:(k + 1) * LANE]

        def mix1_pre(r, q, n=CH):
            y = _ln(load_h(r + q, n))
            yr = pl.multiple_of(lax.rem(r, YB * TB) + q, n)
            for k in range(KD):
                ys[k, pl.ds(yr, n), :] = y[:, k * LANE:(k + 1) * LANE]
            put_cols(a1, q, _ln(y).astype(BF16))

        def mix1_dot(r, q, n=CH):
            for j in range(KD):
                a = _cat([_rows(a1, (k,), q, n) for k in range(KD)], 1)
                z = jnp.dot(a, _bf(w1_s[j]), preferred_element_type=F32)
                h1s[j, pl.ds(HALO + r + q, n), :] = _gelu(z).astype(BF16)

        def mix1(r, q):
            mix1_pre(r, q)
            mix1_dot(r, q)

        shifts = (-1, 1, -2, 2)

        TE = CFG["TE"]
        LAG = CFG["LAG"]
        TM = LAG * TB // (P // TE)
        assert TM % CH == 0 or CH % TM == 0
        CM = min(CH, TM)

        def epi_body(i, c):
            blk = NSEG + i * (TE // SEG)
            t = pl.multiple_of(NSEG * TOK + i * TE, TE)
            r1 = pl.multiple_of(i * TM, TM)
            for q in range(0, TM, CM):
                mix1_pre(r1, q, CM)
            for j in range(KD):
                lo_ = _cat([_cat([_rows(o2[(h // 2) % 2], (blk + b, (h // 4) * 2 + h % 2), 0, SEG)
                                  for b in range(TE // SEG)], 0) for h in range(H)], 1)
                acc = jnp.dot(lo_, _bf(wo_s[j]), preferred_element_type=F32)
                hs[j, pl.ds(t, TE), :] = (xs[j, pl.ds(t, TE), :].astype(F32) + acc).astype(BF16)
            for q in range(0, TM, CM):
                mix1_dot(r1, q, CM)
            return c
        lax.fori_loop(0, P // TE, epi_body, 0)

        TT = CFG["TT"]
        NT, TBASE = LAG * TB // TT, (NB - LAG) * TB

        def out_copy(r, n, slot):
            return pltpu.make_async_copy(ostage.at[slot, pl.ds(0, n)], out_hbm.at[pl.ds(r, n), :], sem_o.at[slot])

        def b2_body(i, with_mix1):
            n = TB if with_mix1 else TT
            r = pl.multiple_of(i * TB if with_mix1 else TBASE + i * TT, n)
            slot = lax.rem(i if with_mix1 else i + NB - LAG, 2)

            @pl.when(i >= 2)
            def _():
                out_copy(0, n, slot).wait()
            if not with_mix1:
                @pl.when(i < 2)
                def _():
                    out_copy(0, TB, slot).wait()

            def mix2(q):
                for j in range(KD):
                    d = shifts[j // (KD // 4)]
                    win = h1s[j, pl.ds(r + q, CH + 2 * HALO), :].astype(F32)
                    gs[j, q:q + CH, :] = win[HALO + d:HALO + d + CH, :].astype(BF16)
                yr = pl.multiple_of(lax.rem(r, YB * TB) + q, CH)
                for j in range(KD):
                    g = _cat([_rows(gs, (k,), q, CH) for k in range(KD)], 1)
                    x1s[j, q:q + CH, :] = (jnp.dot(g, _bf(w2_s[j]), preferred_element_type=F32)
                                           + ys[j, pl.ds(yr, CH), :])

            def up(q):
                put_cols(a3, q, _ln(_cat([x1s[k, q:q + CH, :] for k in range(KD)], 1)).astype(BF16))
                for f in range(KF):
                    a = _cat([_rows(a3, (k,), q, CH) for k in range(KD)], 1)
                    us[f, q:q + CH, :] = _gelu(jnp.dot(a, _bf(w3_s[f]), preferred_element_type=F32)).astype(BF16)

            def down(q):
                for j in range(KD):
                    u = _cat([_rows(us, (f,), q, CH) for f in range(KF)], 1)
                    y = jnp.dot(u, _bf(w4_s[j]), preferred_element_type=F32)
                    res = hs[j, pl.ds(r + q, CH), :].astype(F32) + x1s[j, q:q + CH, :]
                    ostage[slot, q:q + CH, j * LANE:(j + 1) * LANE] = (res + y).astype(BF16)

            r2 = pl.multiple_of((i + LAG) * TB, TB)
            stage = {"a": lambda q: mix1(r2, q), "b": mix2, "c": up, "d": down}
            for name in CFG["ORDER" if with_mix1 else "ORDER2"].split():
                stage[name[0]](int(name[1:]) * CH)
            out_copy(r, n, slot).start()

        def b2_main(i, c):
            b2_body(i, True)
            return c

        def b2_tail(i, c):
            b2_body(i, False)
            return c
        lax.fori_loop(0, NB - LAG, b2_main, 0)
        lax.fori_loop(0, NT, b2_tail, 0)
        for slot in range(2):
            out_copy(0, TT, slot).wait()

    scratch = [
        pltpu.VMEM((H + 2, D // 2, LANE), U32),
        pltpu.VMEM((H, D // 2, LANE), U32),
        pltpu.VMEM((H, D // 2, LANE), U32),
        pltpu.VMEM((KD, H * DH // 2, LANE), U32),
        pltpu.VMEM((KD, D // 2, LANE), U32),
        pltpu.VMEM((KD, D // 2, LANE), U32),
        pltpu.VMEM((KF, D // 2, LANE), U32),
        pltpu.VMEM((KD, F // 2, LANE), U32),
        pltpu.VMEM((KD, S, LANE), BF16),
        pltpu.VMEM((KD, P, LANE), BF16),
        pltpu.VMEM((NSEG + 1, KD, SEG, LANE), BF16),
        [pltpu.VMEM((NPAIR // 2, 2, R + 16, LANE), BF16) for _ in range(2)],
        [pltpu.VMEM((NPAIR // 2, 2, R + 16, LANE), BF16) for _ in range(2)],
        [pltpu.VMEM((NPAIR // 2, 2, R + 16, LANE), BF16) for _ in range(2)],
        [pltpu.VMEM((NSEG + PT, NPAIR, SEG, LANE), BF16) for _ in range(2)],
        [pltpu.VMEM((2 * (SEG + M), 2 * (SEG + M)), BF16) for _ in range(NPAIR)],
        pltpu.VMEM((KD, SEG, LANE), F32),
        pltpu.VMEM((KD, S, LANE), BF16),
        pltpu.VMEM((KD, S + 2 * HALO, LANE), BF16),
        pltpu.VMEM((KD, TB, LANE), BF16),
        pltpu.VMEM((KD, TB, LANE), BF16),
        pltpu.VMEM((KD, YB * TB, LANE), F32),
        pltpu.VMEM((KD, TB, LANE), F32),
        pltpu.VMEM((KD, TB, LANE), BF16),
        pltpu.VMEM((KF, TB, LANE), BF16),
        pltpu.VMEM((2, TB, D), BF16),
        pltpu.SemaphoreType.DMA((3,)),
        pltpu.SemaphoreType.DMA((3 * NPAIR + 1,)),
        pltpu.SemaphoreType.DMA((5,)),
        pltpu.SemaphoreType.DMA((2,)),
    ]
    return kernel, scratch


@functools.partial(jax.jit, static_argnames=("A_seg_len",))
def pallas_sequential_preLN__memory_aug_recurrent_mem_tr__mixer_s_mlp__prompt_kernel(
    A_x, A_mem0, A_Wq, A_Wk, A_Wv, A_Wo, A_seg_len, B_x, B_w1, B_w2, B_w3, B_w4,
):
    del B_x
    B, S, D = A_x.shape
    M = A_mem0.shape[1]
    H, DH = A_Wq.shape[1], A_Wq.shape[2]
    F = B_w3.shape[1]
    SEG = int(A_seg_len)
    assert B == 1 and DH == LANE and M == 8 and SEG == 32 and H % 8 == 0 and D == 4 * 2 * LANE
    kernel, scratch = _make_kernel(S, D, H, DH, M, SEG, F, TB=CFG["TB"])
    any_spec = pl.BlockSpec(memory_space=pl.ANY)
    out = pl.pallas_call(
        kernel,
        out_shape=jax.ShapeDtypeStruct((S, D), A_x.dtype),
        in_specs=[pl.BlockSpec(memory_space=pltpu.SMEM), any_spec, pl.BlockSpec()] + [any_spec] * 8,
        out_specs=any_spec,
        scratch_shapes=scratch,
        compiler_params=pltpu.CompilerParams(vmem_limit_bytes=120 * 1024 * 1024, flags=CFG["FLAGS"]),
    )(
        jnp.zeros((1,), jnp.int32),
        A_x.reshape(S, D),
        A_mem0.reshape(M, D),
        A_Wq.reshape(D // 2, 2, H, DH),
        A_Wk.reshape(D // 2, 2, H, DH),
        A_Wv.reshape(D // 2, 2, H, DH),
        A_Wo.reshape(H * DH, D),
        B_w1, B_w2, B_w3, B_w4,
    )
    return out.reshape(B, S, D)
```
